```python
import os as _os
_os.environ.setdefault("JAX_PLATFORMS", "cpu")
import jax
import jax.numpy as jnp

def _softmax(x, axis=-1):
    return jax.nn.softmax(x, axis=axis)
def _gelu(x):
    return jax.nn.gelu(x, approximate=True)
def _silu(x):
    return jax.nn.silu(x)
def _sigmoid(x):
    return jax.nn.sigmoid(x)
def _layernorm(x, axis=-1, eps=1e-5):
    m = jnp.mean(x, axis=axis, keepdims=True)
    v = jnp.var(x, axis=axis, keepdims=True)
    return (x - m) / jnp.sqrt(v + eps)
def _scatter_add(tgt, idx, src, axis=0):
    return tgt.at[idx].add(src)
def _segment_sum(src, seg, n):
    return jax.ops.segment_sum(src, seg, n)
class _Rng:
    def __init__(self, key):
        self._k = key
    def _next(self):
        self._k, sub = jax.random.split(self._k)
        return sub
    def normal(self, shape):
        return jax.random.normal(self._next(), shape, dtype=jnp.bfloat16)
    def randint(self, lo, hi, shape):
        return jax.random.randint(self._next(), shape, lo, hi, dtype=jnp.int32)
    def uniform(self, shape, lo=0.0, hi=1.0):
        return jax.random.uniform(self._next(), shape, jnp.bfloat16, lo, hi)
    def permutation(self, n):
        return jax.random.permutation(self._next(), n)


kernel_name = 'interleave_layers__linear_attn_block__mha_block__prompt'

def setup_inputs():
    _rng = _Rng(jax.random.key(int.from_bytes(__import__("os").urandom(4), "little")))
    _w = (lambda a: (lambda t: t.astype(jnp.bfloat16) if jnp.issubdtype(t.dtype, jnp.floating) else t)(jnp.asarray(a)))
    def _A_setup():
        B, S, D = 1, 2048, 640
        return {
            "x": _w((lambda *s: _rng.normal(s) * 0.05)(B, S, D)),
            "wqkv": _w((lambda *s: _rng.normal(s) * 0.1)(D, 3 * D)),
            "wo": _w((lambda *s: _rng.normal(s) * 0.05)(D, D)),
        }
    _A_in = _A_setup()

    def _B_setup():
        B, S, D, H = 1, 2048, 640, 32
        return {
            "x": _w((lambda *s: _rng.normal(s) * 0.05)(B, S, D)),
            "wqkv": _w((lambda *s: _rng.normal(s) * 0.1)(D, 3 * D)),
            "wo": _w((lambda *s: _rng.normal(s) * 0.05)(D, D)),
        }
    _B_in = _B_setup()

    return {
        "A_x": _A_in["x"],
        "A_wqkv": _A_in["wqkv"],
        "A_wo": _A_in["wo"],
        "B_x": _B_in["x"],
        "B_wqkv": _B_in["wqkv"],
        "B_wo": _B_in["wo"],
    }

def reference(A_x, A_wqkv, A_wo, B_x, B_wqkv, B_wo):
    def _A_ref(x, wqkv, wo):
        B, S, D = x.shape
        H = 32; Dh = D // H
        qkv = (lambda x, *d: x.transpose(*d))((x @ wqkv).reshape(B, S, 3, H, Dh), 2, 0, 3, 1, 4)
        q, k, v = qkv[0], qkv[1], qkv[2]
        phi = lambda t: jnp.where(t > 0, t + 1, jnp.exp(t)) + 1e-6
        pq, pk = phi(q), phi(k)
        kv = jnp.einsum("bhsd,bhse->bhde", pk, v)
        z = jnp.einsum("bhsd->bhd", pk)
        num = jnp.einsum("bhqd,bhde->bhqe", pq, kv)
        den = jnp.einsum("bhqd,bhd->bhq", pq, z)[..., None] + 1e-6
        o = num / den
        return (lambda x, *d: x.transpose(*d))(o, 0, 2, 1, 3).reshape(B, S, D) @ wo

    def _B_ref(x, wqkv, wo):
        B, S, D = x.shape
        H = 32
        Dh = D // H
        qkv = (lambda x, *d: x.transpose(*d))((x @ wqkv).reshape(B, S, 3, H, Dh), 2, 0, 3, 1, 4)
        q, k, v = qkv[0], qkv[1], qkv[2]
        scores = jnp.einsum("bhqd,bhkd->bhqk", q, k) * (Dh ** -0.5)
        p = _softmax(scores, axis=-1)
        o = jnp.einsum("bhqk,bhkd->bhqd", p, v)
        return (lambda x, *d: x.transpose(*d))(o, 0, 2, 1, 3).reshape(B, S, D) @ wo

    x = A_x
    x = x + _A_ref(_layernorm(x, axis=-1), A_wqkv, A_wo)
    x = x + _B_ref(_layernorm(x, axis=-1), B_wqkv, B_wo)
    x = x + _A_ref(_layernorm(x, axis=-1), A_wqkv, A_wo)
    x = x + _B_ref(_layernorm(x, axis=-1), B_wqkv, B_wo)
    return x
```

```python
import math

import jax
import jax.numpy as jnp
from jax import lax
import jax.experimental.pallas as pl
import jax.experimental.pallas.tpu as pltpu

S = 2048
D = 640
H = 32
DH = 20
NG = 6
GW = 120
TB = 512
NB = S // TB
CK = 128
NC = S // CK
QPI = 2
LAG = 1
NSB = 4
LN_EPS = 1e-5
QSCALE = (DH ** -0.5) * math.log2(math.e)

F32 = jnp.float32
BF16 = jnp.bfloat16
NN = (((1,), (0,)), ((), ()))
NT = (((1,), (1,)), ((), ()))
TN = (((0,), (0,)), ((), ()))


def _dot(a, b, dims=NN):
    return lax.dot_general(a, b, dims, preferred_element_type=F32)


def _phi(t):
    return jnp.where(t > 0, t + 1.0, jnp.exp(jnp.minimum(t, 0.0))) + 1e-6


def _layernorm(x):
    m = jnp.mean(x, axis=-1, keepdims=True)
    xc = x - m
    v = jnp.mean(xc * xc, axis=-1, keepdims=True)
    return xc * lax.rsqrt(v + LN_EPS)


def _kernel(x_in, awqkv, awo, bwqkv, bwo, out_ref,
            x_ref, wkt_a, wqvt_b, wk_b,
            pq_ref, v_ref, pkt_ref, m_ref, zm_ref,
            k_ref, qt_ref, vt_ref, ot_ref, *s_refs):
    x_ref[...] = x_in[...].astype(F32)
    wkt_a[...] = awqkv[:, D:2 * D].astype(F32).T.astype(BF16)
    wqvt_b[0:D, :] = bwqkv[:, 0:D].astype(F32).T.astype(BF16)
    wqvt_b[D:2 * D, :] = bwqkv[:, 2 * D:3 * D].astype(F32).T.astype(BF16)
    wk_b[...] = jnp.zeros(wk_b.shape, BF16)
    for g in range(NG):
        w = min(GW, D - g * GW)
        wk_b[:, g * 128:g * 128 + w] = bwqkv[:, D + g * GW:D + g * GW + w]

    def rows(i):
        return pl.ds(pl.multiple_of(i * TB, TB), TB)

    def linear_layer():
        def proj(i, c):
            xn = _layernorm(x_ref[rows(i), :]).astype(BF16)
            pq_ref[rows(i), :] = _phi(_dot(xn, awqkv[:, 0:D])).astype(BF16)
            v_ref[rows(i), :] = _dot(xn, awqkv[:, 2 * D:3 * D]).astype(BF16)
            pkt_ref[i] = _phi(_dot(wkt_a[...], xn, NT))
            return c
        lax.fori_loop(0, NB, proj, 0)

        kv = None
        zs = None
        for i in range(NB):
            pkt = pkt_ref[i]
            t = _dot(pkt, v_ref[i * TB:(i + 1) * TB, :])
            kv = t if kv is None else t + kv
            zs = pkt if zs is None else zs + pkt
        z = jnp.sum(zs, axis=-1, keepdims=True)
        hr = lax.broadcasted_iota(jnp.int32, (D, D), 0) // DH
        hc = lax.broadcasted_iota(jnp.int32, (D, D), 1) // DH
        kv = jnp.where(hr == hc, kv, 0.0)
        m_ref[...] = _dot(kv, awo[...]).astype(BF16)
        hr2 = lax.broadcasted_iota(jnp.int32, (D, 128), 0) // DH
        hc2 = lax.broadcasted_iota(jnp.int32, (D, 128), 1)
        zm_ref[...] = jnp.where((hr2 == hc2) | (hr2 + H == hc2), z, 0.0).astype(BF16)

        er = lax.broadcasted_iota(jnp.int32, (128, D), 0)
        ec = lax.broadcasted_iota(jnp.int32, (128, D), 1) // DH
        expand = jnp.where((er == ec) | (er == ec + H), 1.0, 0.0).astype(BF16)
        lane = lax.broadcasted_iota(jnp.int32, (TB, 128), 1)

        def outp(i, c):
            pq = pq_ref[rows(i), :]
            den = _dot(pq, zm_ref[...]) + 1e-6
            r = 1.0 / den
            r_hi = r.astype(BF16).astype(F32)
            r2 = jnp.where(lane < H, r_hi, r - r_hi)
            rf = _dot(r2, expand)
            pqn = (pq.astype(F32) * rf).astype(BF16)
            x_ref[rows(i), :] += _dot(pqn, m_ref[...])
            return c
        lax.fori_loop(0, NB, outp, 0)

    def mha_layer():
        def proj(i, c):
            xn = _layernorm(x_ref[rows(i), :]).astype(BF16)
            k = _dot(xn, wk_b[...]).astype(BF16)
            for g in range(NG):
                k_ref[g, rows(i), :] = k[:, g * 128:(g + 1) * 128]
            qt = _dot(wqvt_b[0:D, :], xn, NT) * QSCALE
            for g in range(NG):
                w = min(GW, D - g * GW)
                blk = qt[g * GW:g * GW + w]
                blk = jnp.concatenate([blk, jnp.zeros((128 - w, TB), F32)], axis=0)
                qt_ref[g, i] = blk.astype(BF16)
            vt_ref[i] = _dot(wqvt_b[D:2 * D, :], xn, NT)
            return c
        lax.fori_loop(0, NB, proj, 0)

        NQG = NB // QPI
        NP = (H // 2) * NQG
        P = 2 * QPI
        row_c = lax.broadcasted_iota(jnp.int32, (8, CK), 0)
        row_q = lax.broadcasted_iota(jnp.int32, (8, TB), 0)

        def get_qm(g, j, q):
            row = lax.broadcasted_iota(jnp.int32, (128, TB), 0)
            qm = qt_ref[g, q]
            return jnp.where((row >= j * DH) & (row < j * DH + DH), qm, jnp.zeros_like(qm))

        def qk(g, qm, c, s_ref, mx):
            s = _dot(k_ref[g, c * CK:(c + 1) * CK, :], qm)
            s_ref[c * CK:(c + 1) * CK, :] = s
            cm = jnp.max(s.reshape(CK // 8, 8, TB), axis=0)
            return cm if mx is None else jnp.maximum(mx, cm)

        def pv(a, odd, c, s_ref, m, acc, zero):
            sc = s_ref[pl.ds(pl.multiple_of(zero + c * CK, CK), CK), :]
            p = jnp.exp2(sc - m).astype(BF16)
            base = pl.multiple_of(a * 40 + (16 if odd else 0), 8)
            cb, co = (c * CK) // TB, (c * CK) % TB
            v = vt_ref[cb, pl.ds(base, 24), co:co + CK]
            if odd:
                v = jnp.concatenate([jnp.where(row_c < 4, 1.0, v[0:8]), v[8:24]], axis=0)
            else:
                v = jnp.concatenate([v[0:16], jnp.where(row_c >= 4, 1.0, v[16:24])], axis=0)
            o = _dot(v, p)
            return o if acc is None else o + acc

        def finish(a, q, odd, acc, oe):
            if not odd:
                return acc * (1.0 / acc[20:21])
            oo = acc * (1.0 / acc[0:1])
            mid = jnp.where(row_q < 4, oe[16:24], oo[0:8])
            ot_ref[q, pl.ds(pl.multiple_of(a * 40, 8), 40), :] = jnp.concatenate(
                [oe[0:16], mid, oo[8:24]], axis=0)
            return None

        qm0 = get_qm(0, 0, 0)
        mx0 = None
        for c in range(NC):
            mx0 = qk(0, qm0, c, s_refs[0], mx0)
        m0 = jnp.max(mx0, axis=0, keepdims=True)
        for c in range(NC - LAG, NC):
            s_refs[NSB - 1][c * CK:(c + 1) * CK, :] = jnp.zeros((CK, TB), F32)
        ones24 = jnp.ones((24, TB), F32)
        sh = NQG.bit_length() - 1

        def body(t, carry):
            m_prev, m_cur, acc_prev, oe_prev, g, j3 = carry
            zero = jnp.minimum(t, 0)
            tp = jnp.maximum(t - 1, 0)
            if NQG == 1:
                a, qg = t, 0
                a_prev, q_prev = tp, QPI - 1
            else:
                a = lax.shift_right_logical(t, sh)
                qg = t & (NQG - 1)
                a_prev = lax.shift_right_logical(tp, sh)
                q_prev = (tp & (NQG - 1)) * QPI + QPI - 1
            last_in_pair = (qg == NQG - 1)
            j3n = jnp.where(j3 == 2, 0, j3 + 1)
            gn = jnp.where(j3 == 2, g + 1, g)
            gn = jnp.where(t == NP - 1, g, gn)
            j3n = jnp.where(last_in_pair, j3n, j3)
            gn = jnp.where(last_in_pair, gn, g)
            qgn = jnp.where(last_in_pair, 0, qg + 1)
            ms = {-1: m_prev, 0: m_cur}
            accs = {-1: acc_prev}
            oes = {-1: oe_prev}
            mx = None
            for n in range(P * NC):
                i = n // NC + 1
                c = n % NC
                if c == 0:
                    if i < P:
                        gq = g
                        qm = get_qm(g, 2 * j3 + (i % 2), qg * QPI + i // 2)
                    else:
                        gq = gn
                        qm = get_qm(gn, 2 * j3n, qgn * QPI)
                    mx = None
                mx = qk(gq, qm, c, s_refs[i % NSB], mx)
                if c == NC - 1:
                    ms[i] = jnp.max(mx, axis=0, keepdims=True)
                n2 = n - LAG
                i2 = n2 // NC
                c2 = n2 % NC
                a2 = a_prev if i2 < 0 else a
                q2 = q_prev if i2 < 0 else qg * QPI + i2 // 2
                accs[i2] = pv(a2, i2 % 2, c2, s_refs[i2 % NSB], ms[i2], accs.get(i2), zero)
                if c2 == NC - 1:
                    r = finish(a2, q2, i2 % 2, accs[i2], oes.get(i2 if i2 < 0 else i2 - 1))
                    if i2 % 2 == 0:
                        oes[i2] = r
            return ms[P - 1], ms[P], accs[P - 1], oes[P - 2], gn, j3n

        zero_row = jnp.zeros((1, TB), F32)
        carry = lax.fori_loop(
            0, NP, body, (zero_row, m0, ones24, ones24, jnp.int32(0), jnp.int32(0)))
        m_prev, _, acc, oe, _, _ = carry
        for c2 in range(NC - LAG, NC):
            acc = pv(H // 2 - 1, 1, c2, s_refs[NSB - 1], m_prev, acc, 0)
        finish(H // 2 - 1, NB - 1, 1, acc, oe)

        def outp(i, c):
            o = ot_ref[i].T.astype(BF16)
            x_ref[rows(i), :] += _dot(o, bwo[...])
            return c
        lax.fori_loop(0, NB, outp, 0)

    def round_(r, c):
        linear_layer()
        mha_layer()
        return c
    lax.fori_loop(0, 2, round_, 0)

    out_ref[...] = x_ref[...].astype(out_ref.dtype)


@jax.jit
def pallas_interleave_layers__linear_attn_block__mha_block__prompt_kernel(
    A_x: jax.Array,
    A_wqkv: jax.Array,
    A_wo: jax.Array,
    B_x: jax.Array,
    B_wqkv: jax.Array,
    B_wo: jax.Array,
):
    x = A_x.reshape(S, D)
    scratch = [
        pltpu.VMEM((S, D), F32),
        pltpu.VMEM((D, D), BF16),
        pltpu.VMEM((2 * D, D), BF16),
        pltpu.VMEM((D, NG * 128), BF16),
        pltpu.VMEM((S, D), BF16),
        pltpu.VMEM((S, D), BF16),
        pltpu.VMEM((NB, D, TB), F32),
        pltpu.VMEM((D, D), BF16),
        pltpu.VMEM((D, 128), BF16),
        pltpu.VMEM((NG, S, 128), BF16),
        pltpu.VMEM((NG, NB, 128, TB), BF16),
        pltpu.VMEM((NB, D, TB), F32),
        pltpu.VMEM((NB, D, TB), F32),
    ] + [pltpu.VMEM((S, TB), F32) for _ in range(NSB)]
    out = pl.pallas_call(
        _kernel,
        out_shape=jax.ShapeDtypeStruct((S, D), A_x.dtype),
        scratch_shapes=scratch,
        compiler_params=pltpu.CompilerParams(vmem_limit_bytes=110 * 1024 * 1024),
    )(x, A_wqkv, A_wo, B_wqkv, B_wo)
    return out.reshape(A_x.shape)
```

```python
import math

import jax
import jax.numpy as jnp
from jax import lax
import jax.experimental.pallas as pl
import jax.experimental.pallas.tpu as pltpu

S = 2048
D = 640
H = 32
DH = 20
NG = 8
TB = 512
NB = S // TB
SB = 128
NS = TB // SB
CK = 128
NC = S // CK
QPI = 2
LAG = 1
NSB = 4
LN_EPS = 1e-5
QSCALE = (DH ** -0.5) * math.log2(math.e)
KV_ROWS = [(0, 144), (120, 264), (240, 400), (376, 520), (496, 640)]
AQ, AV, BQ, BK, BV, AO, BO, AK = range(8)

F32 = jnp.float32
BF16 = jnp.bfloat16
NN = (((1,), (0,)), ((), ()))
NT = (((1,), (1,)), ((), ()))


def SCOPE(name, f, *args):
    del name
    return f(*args)


def _dot(a, b, dims=NN):
    return lax.dot_general(a, b, dims, preferred_element_type=F32)


def _phi(t):
    return jnp.where(t > 0, t + 1.0, jnp.exp(jnp.minimum(t, 0.0))) + 1e-6


def _layernorm(x):
    m = jnp.mean(x, axis=-1, keepdims=True)
    xc = x - m
    v = jnp.mean(xc * xc, axis=-1, keepdims=True)
    return xc * lax.rsqrt(v + LN_EPS)


def _kernel(x_hbm, awqkv_hbm, awo_hbm, bwqkv_hbm, bwo_hbm, out_hbm,
            xin, wsrc, obuf, sems,
            x_ref, xn_ref, wt,
            pqt_ref, kv_ref, z_ref, mt_ref, zm_ref,
            k_ref, qt_ref, vt_ref, ot_ref, *s_refs):
    def rows(i):
        return pl.ds(pl.multiple_of(i * TB, TB), TB)

    def srows(i, s):
        return pl.ds(pl.multiple_of(i * TB + s * SB, SB), SB)

    def cols(c):
        return pl.ds(c * D, D)

    def cp_x(i):
        return pltpu.make_async_copy(x_hbm.at[rows(i), :], xin.at[rows(i), :], sems.at[i])

    w_srcs = {AQ: awqkv_hbm.at[:, cols(0)], AV: awqkv_hbm.at[:, cols(2)],
              BQ: bwqkv_hbm.at[:, cols(0)], BK: bwqkv_hbm.at[:, cols(1)],
              BV: bwqkv_hbm.at[:, cols(2)], AO: awo_hbm, BO: bwo_hbm,
              AK: awqkv_hbm.at[:, cols(1)]}

    def cp_w(m, src=None):
        src = awo_hbm if src is None else src
        return pltpu.make_async_copy(src, wsrc.at[m], sems.at[NB + m])

    def transpose_w(m):
        wt[pl.ds(pl.multiple_of(m * D, D), D), :] = wsrc[m].astype(F32).T.astype(BF16)

    def resid(i, s):
        return xin[srows(i, s), :].astype(F32) + x_ref[srows(i, s), :]

    def ln_sub(i, s):
        return _layernorm(resid(i, s)).astype(BF16)

    def a_proj_k(xns):
        pk = jnp.concatenate([_phi(_dot(xn, wsrc[AK])) for xn in xns], axis=0)
        z_ref[...] += jnp.sum(pk.reshape(TB // 8, 8, D), axis=0)
        return pk

    def a_proj_qv(i, xns, pk):
        vts = []
        for s in range(NS):
            vts.append(_dot(wt[AV * D:(AV + 1) * D, :], xns[s], NT))
        vt = jnp.concatenate(vts, axis=1)
        for s in range(NS):
            if s == NS // 2:
                for j, (r0, r1) in enumerate(KV_ROWS):
                    kv_ref[j, 0:r1 - r0, :] += _dot(vt[r0:r1], pk[:, j * 128:(j + 1) * 128])
            qt = _dot(wt[AQ * D:(AQ + 1) * D, :], xns[s], NT)
            pqt_ref[i, :, s * SB:(s + 1) * SB] = _phi(qt).astype(BF16)

    def zero_kv():
        kv_ref[...] = jnp.zeros(kv_ref.shape, F32)
        z_ref[...] = jnp.zeros(z_ref.shape, F32)

    cp_x(0).start()
    for m in (AK, AV, AQ):
        cp_w(m, w_srcs[m]).start()
    for i in range(1, NB):
        cp_x(i).start()
    for m in (BQ, BK, BV, AO, BO):
        cp_w(m, w_srcs[m]).start()
    x_ref[...] = jnp.zeros(x_ref.shape, F32)
    cp_x(0).wait()
    xn_ref[...] = ln_sub(0, 0)
    cp_w(AK).wait()

    def stage_a(r):
        def body(i, xn0):
            @pl.when(r == 0)
            def _():
                cp_w(2 * i).wait()

                @pl.when(i < NB - 1)
                def _():
                    cp_w(2 * i + 1).wait()
                    cp_x(i + 1).wait()

            xns = [xn0] + [ln_sub(i, s) for s in range(1, NS)]
            pk = a_proj_k(xns)
            transpose_w(2 * i)
            transpose_w(jnp.minimum(2 * i + 1, BO))
            nxt = ln_sub(jnp.minimum(i + 1, NB - 1), 0)
            a_proj_qv(i, xns, pk)
            return nxt
        zero_kv()
        lax.fori_loop(0, NB, body, xn_ref[...])

    def a_mid():
        z = jnp.sum(z_ref[...], axis=0, keepdims=True)
        hr2 = lax.broadcasted_iota(jnp.int32, (H, D), 0)
        hc2 = lax.broadcasted_iota(jnp.int32, (H, D), 1) // DH
        zm_ref[...] = jnp.where(hr2 == hc2, z, 0.0)
        for j, (r0, r1) in enumerate(KV_ROWS):
            k0 = (r0 // 128) * 128
            k1 = -(-r1 // 128) * 128
            hr = (lax.broadcasted_iota(jnp.int32, (r1 - r0, 128), 0) + r0) // DH
            hc = (lax.broadcasted_iota(jnp.int32, (r1 - r0, 128), 1) + j * 128) // DH
            kvj = jnp.where(hr == hc, kv_ref[j, 0:r1 - r0, :], 0.0)
            pads = []
            if r0 > k0:
                pads.append(jnp.zeros((r0 - k0, 128), F32))
            pads.append(kvj)
            if k1 > r1:
                pads.append(jnp.zeros((k1 - r1, 128), F32))
            kvj = jnp.concatenate(pads, axis=0)
            mt_ref[:, j * 128:(j + 1) * 128] = _dot(
                wt[AO * D:(AO + 1) * D, k0:k1], kvj).astype(BF16)

    row8 = lax.broadcasted_iota(jnp.int32, (8, SB), 0)

    def stage_l2(i, c):
        pqns = []
        for s in range(NS):
            pq = pqt_ref[i, :, s * SB:(s + 1) * SB]
            r = 1.0 / (_dot(zm_ref[...], pq) + 1e-6)
            parts = []
            for a in range(H // 2):
                re = jnp.broadcast_to(r[2 * a:2 * a + 1], (8, SB))
                ro = jnp.broadcast_to(r[2 * a + 1:2 * a + 2], (8, SB))
                parts += [re, re, jnp.where(row8 < 4, re, ro), ro, ro]
            pqns.append((pq.astype(F32) * jnp.concatenate(parts, axis=0)).astype(BF16))
        xns = []
        for s in range(NS):
            y = x_ref[srows(i, s), :] + _dot(mt_ref[...], pqns[s]).T
            x_ref[srows(i, s), :] = y
            xns.append(_layernorm(xin[srows(i, s), :].astype(F32) + y).astype(BF16))
        for s in range(NS):
            kt = _dot(wt[BK * D:(BK + 1) * D, :], xns[s], NT)
            qt = _dot(wt[BQ * D:(BQ + 1) * D, :], xns[s], NT) * QSCALE
            zpad = jnp.zeros((8, SB), F32)
            for g in range(NG):
                kparts = []
                for j in range(4):
                    r0 = (2 * g + j // 2) * 40 + (16 if j % 2 else 0)
                    kparts += [kt[r0:r0 + 24], zpad]
                    if j % 2:
                        qb = [jnp.where(row8 < 4, 0.0, qt[r0:r0 + 8]), qt[r0 + 8:r0 + 24], zpad]
                    else:
                        qb = [qt[r0:r0 + 16], jnp.where(row8 < 4, qt[r0 + 16:r0 + 24], 0.0), zpad]
                    qt_ref[4 * g + j, i, :, s * SB:(s + 1) * SB] = pltpu.bitcast(
                        jnp.concatenate(qb, axis=0).astype(BF16), jnp.uint32)
                kb = jnp.concatenate(kparts, axis=0)
                k_ref[g, pl.ds(pl.multiple_of((i * TB + s * SB) // 2, SB // 2), SB // 2), :] = (
                    pltpu.bitcast(kb.T.astype(BF16), jnp.uint32))
            vt_ref[i, :, s * SB:(s + 1) * SB] = _dot(wt[BV * D:(BV + 1) * D, :], xns[s], NT)
        return c

    def attention():
        NQG = NB // QPI
        NP = NG * NQG
        P = 4 * QPI
        row_c = lax.broadcasted_iota(jnp.int32, (8, CK), 0)
        row_q = lax.broadcasted_iota(jnp.int32, (8, TB), 0)

        def get_qm(g, j, q):
            parts = []
            if j > 0:
                parts.append(jnp.zeros((32 * j, TB), BF16))
            parts.append(pltpu.bitcast(qt_ref[4 * g + j, q], BF16))
            if j < 3:
                parts.append(jnp.zeros((96 - 32 * j, TB), BF16))
            return jnp.concatenate(parts, axis=0)

        def qk(g, qm, c, s_ref, mx):
            s = _dot(pltpu.bitcast(k_ref[g, c * CK // 2:(c + 1) * CK // 2, :], BF16), qm)
            s_ref[c * CK:(c + 1) * CK, :] = s
            cm = jnp.max(s.reshape(CK // 8, 8, TB), axis=0)
            return cm if mx is None else jnp.maximum(mx, cm)

        def pv(a, odd, c, s_ref, m, acc, zero):
            sc = s_ref[pl.ds(pl.multiple_of(zero + c * CK, CK), CK), :]
            p = jnp.exp2(sc - m).astype(BF16)
            base = pl.multiple_of(a * 40 + (16 if odd else 0), 8)
            cb, co = (c * CK) // TB, (c * CK) % TB
            v = vt_ref[cb, pl.ds(base, 24), co:co + CK]
            if odd:
                v = jnp.concatenate([jnp.where(row_c < 4, 1.0, v[0:8]), v[8:24]], axis=0)
            else:
                v = jnp.concatenate([v[0:16], jnp.where(row_c >= 4, 1.0, v[16:24])], axis=0)
            o = _dot(v, p)
            return o if acc is None else o + acc

        def finish(a, q, odd, acc, oe):
            if not odd:
                oe = acc * (1.0 / acc[20:21])
                ot_ref[q, pl.ds(pl.multiple_of(a * 40, 8), 16), :] = oe[0:16]
                return oe[16:24]
            oo = acc * (1.0 / acc[0:1])
            mid = jnp.where(row_q < 4, oe, oo[0:8])
            ot_ref[q, pl.ds(pl.multiple_of(a * 40 + 16, 8), 24), :] = jnp.concatenate(
                [mid, oo[8:24]], axis=0)
            return None

        qm0 = get_qm(0, 0, 0)
        mx0 = None
        for c in range(NC):
            mx0 = qk(0, qm0, c, s_refs[0], mx0)
        m0 = jnp.max(mx0, axis=0, keepdims=True)
        for c in range(NC - LAG, NC):
            s_refs[NSB - 1][c * CK:(c + 1) * CK, :] = jnp.zeros((CK, TB), F32)
        ones24 = jnp.ones((24, TB), F32)
        sh = NQG.bit_length() - 1

        def body(t, carry):
            m_prev, m_cur, acc_prev, oe_prev = carry
            zero = jnp.minimum(t, 0)
            tp = jnp.maximum(t - 1, 0)
            tn = jnp.minimum(t + 1, NP - 1)
            g = lax.shift_right_logical(t, sh)
            q0 = (t & (NQG - 1)) * QPI
            a_prev = 2 * lax.shift_right_logical(tp, sh) + 1
            q_prev = (tp & (NQG - 1)) * QPI + QPI - 1
            gn = lax.shift_right_logical(tn, sh)
            qn = (tn & (NQG - 1)) * QPI
            ms = {-1: m_prev, 0: m_cur}
            accs = {-1: acc_prev}
            oes = {-1: oe_prev}
            mx = None
            for n in range(P * NC):
                i = n // NC + 1
                c = n % NC
                if c == 0:
                    if i < P:
                        gq = g
                        qm = get_qm(g, i % 4, q0 + i // 4)
                    else:
                        gq = gn
                        qm = get_qm(gn, 0, qn)
                    mx = None
                mx = qk(gq, qm, c, s_refs[i % NSB], mx)
                if c == NC - 1:
                    ms[i] = jnp.max(mx, axis=0, keepdims=True)
                n2 = n - LAG
                i2 = n2 // NC
                c2 = n2 % NC
                a2 = a_prev if i2 < 0 else 2 * g + (i2 % 4) // 2
                q2 = q_prev if i2 < 0 else q0 + i2 // 4
                accs[i2] = pv(a2, i2 % 2, c2, s_refs[i2 % NSB], ms[i2], accs.get(i2), zero)
                if c2 == NC - 1:
                    r = finish(a2, q2, i2 % 2, accs[i2], oes.get(i2 if i2 < 0 else i2 - 1))
                    if i2 % 2 == 0:
                        oes[i2] = r
            return ms[P - 1], ms[P], accs[P - 1], oes[P - 2]

        zero_row = jnp.zeros((1, TB), F32)
        carry = SCOPE('s_attn_loop', lambda: lax.fori_loop(
            0, NP, body, (zero_row, m0, ones24, ones24[0:8])))
        m_prev, _, acc, oe = carry
        for c2 in range(NC - LAG, NC):
            acc = pv(H // 2 - 1, 1, c2, s_refs[NSB - 1], m_prev, acc, 0)
        finish(H // 2 - 1, NB - 1, 1, acc, oe)

    def out_copy(i):
        return pltpu.make_async_copy(obuf.at[rows(i), :], out_hbm.at[rows(i), :], sems.at[i])

    def stage_bout(r):
        def body(i, c):
            xn_ref[...] = ln_sub(0, 0)
            for s in range(NS):
                yt = _dot(wt[BO * D:(BO + 1) * D, :], ot_ref[i, :, s * SB:(s + 1) * SB])
                y = x_ref[srows(i, s), :] + yt.T
                x_ref[srows(i, s), :] = y
                obuf[srows(i, s), :] = (xin[srows(i, s), :].astype(F32) + y).astype(obuf.dtype)

            @pl.when(r == 1)
            def _():
                out_copy(i).start()
            return c
        lax.fori_loop(0, NB, body, 0)

    def round_(r, c):
        SCOPE('s_a', stage_a, r)
        SCOPE('s_amid', a_mid)
        SCOPE('s_l2', lambda: lax.fori_loop(0, NB, stage_l2, 0))
        SCOPE('s_attn', attention)
        SCOPE('s_bout', stage_bout, r)
        return c
    lax.fori_loop(0, 2, round_, 0)
    for i in range(NB):
        out_copy(i).wait()


@jax.jit
def pallas_interleave_layers__linear_attn_block__mha_block__prompt_kernel(
    A_x: jax.Array,
    A_wqkv: jax.Array,
    A_wo: jax.Array,
    B_x: jax.Array,
    B_wqkv: jax.Array,
    B_wo: jax.Array,
):
    x = A_x.reshape(S, D)
    scratch = [
        pltpu.VMEM((S, D), BF16),
        pltpu.VMEM((8, D, D), BF16),
        pltpu.VMEM((S, D), BF16),
        pltpu.SemaphoreType.DMA((NB + 8,)),
        pltpu.VMEM((S, D), F32),
        pltpu.VMEM((SB, D), BF16),
        pltpu.VMEM((7 * D, D), BF16),
        pltpu.VMEM((NB, D, TB), BF16),
        pltpu.VMEM((5, 160, 128), F32),
        pltpu.VMEM((8, D), F32),
        pltpu.VMEM((D, D), BF16),
        pltpu.VMEM((H, D), F32),
        pltpu.VMEM((NG, S // 2, 128), jnp.uint32),
        pltpu.VMEM((H, NB, 16, TB), jnp.uint32),
        pltpu.VMEM((NB, D, TB), F32),
        pltpu.VMEM((NB, D, TB), F32),
    ] + [pltpu.VMEM((S, TB), F32) for _ in range(NSB)]
    out = pl.pallas_call(
        _kernel,
        out_shape=jax.ShapeDtypeStruct((S, D), A_x.dtype),
        in_specs=[pl.BlockSpec(memory_space=pl.ANY)] * 5,
        out_specs=pl.BlockSpec(memory_space=pl.ANY),
        scratch_shapes=scratch,
        compiler_params=pltpu.CompilerParams(vmem_limit_bytes=110 * 1024 * 1024),
    )(x, A_wqkv, A_wo, B_wqkv, B_wo)
    return out.reshape(A_x.shape)
```

```python
import math

import jax
import jax.numpy as jnp
from jax import lax
import jax.experimental.pallas as pl
import jax.experimental.pallas.tpu as pltpu

S = 2048
D = 640
H = 32
DH = 20
NG = 8
TB = 512
NB = S // TB
SB = 128
NS = TB // SB
CK = 128
NC = S // CK
QPI = 2
LAG = 1
NSB = 4
LN_EPS = 1e-5
QSCALE = (DH ** -0.5) * math.log2(math.e)
KV_ROWS = [(0, 144), (120, 264), (240, 400), (376, 520), (496, 640)]
AQ, AV, BQ, BK, BV, AO, BO, AK = range(8)

F32 = jnp.float32
BF16 = jnp.bfloat16
NN = (((1,), (0,)), ((), ()))
NT = (((1,), (1,)), ((), ()))


def SCOPE(name, f, *args):
    del name
    return f(*args)


def _dot(a, b, dims=NN):
    return lax.dot_general(a, b, dims, preferred_element_type=F32)


def _phi(t):
    return jnp.where(t > 0, t + 1.0, jnp.exp(jnp.minimum(t, 0.0))) + 1e-6


def _layernorm(x):
    m = jnp.mean(x, axis=-1, keepdims=True)
    xc = x - m
    v = jnp.mean(xc * xc, axis=-1, keepdims=True)
    return xc * lax.rsqrt(v + LN_EPS)


def _kernel(x_hbm, awqkv_hbm, awo_hbm, bwqkv_hbm, bwo_hbm, out_hbm,
            xin, wsrc, obuf, sems, osems,
            x_ref, xn_ref, wt,
            pqt_ref, kv_ref, z_ref, mt_ref, zm_ref,
            k_ref, qt_ref, vt_ref, ot_ref, *s_refs):
    def rows(i):
        return pl.ds(pl.multiple_of(i * TB, TB), TB)

    def srows(i, s):
        if isinstance(i, int):
            return pl.ds(i * TB + s * SB, SB)
        return pl.ds(pl.multiple_of(i * TB + s * SB, SB), SB)

    def cols(c):
        return pl.ds(c * D, D)

    def cp_x(i):
        lo = 0 if i == 0 else i * TB + SB
        hi = min((i + 1) * TB + SB, S)
        return pltpu.make_async_copy(x_hbm.at[lo:hi, :], xin.at[lo:hi, :], sems.at[i])

    w_srcs = {AQ: awqkv_hbm.at[:, cols(0)], AV: awqkv_hbm.at[:, cols(2)],
              BQ: bwqkv_hbm.at[:, cols(0)], BK: bwqkv_hbm.at[:, cols(1)],
              BV: bwqkv_hbm.at[:, cols(2)], AO: awo_hbm, BO: bwo_hbm,
              AK: awqkv_hbm.at[:, cols(1)]}

    def cp_w(m, src=None):
        src = awo_hbm if src is None else src
        return pltpu.make_async_copy(src, wsrc.at[m], sems.at[NB + m])

    def transpose_w(m):
        wt[pl.ds(pl.multiple_of(m * D, D), D), :] = wsrc[m].astype(F32).T.astype(BF16)

    def resid(i, s):
        return xin[srows(i, s), :].astype(F32) + x_ref[srows(i, s), :]

    def ln_sub(i, s):
        return _layernorm(resid(i, s)).astype(BF16)

    def a_proj_k(xns):
        pk = jnp.concatenate([_phi(_dot(xn, wsrc[AK])) for xn in xns], axis=0)
        z_ref[...] += jnp.sum(pk.reshape(TB // 8, 8, D), axis=0)
        return pk

    def a_proj_qv(i, xns, pk):
        vts = []
        for s in range(NS):
            vts.append(_dot(wt[AV * D:(AV + 1) * D, :], xns[s], NT))
        vt = jnp.concatenate(vts, axis=1)
        for s in range(NS):
            if s == NS // 2:
                for j, (r0, r1) in enumerate(KV_ROWS):
                    kv_ref[j, 0:r1 - r0, :] += _dot(vt[r0:r1], pk[:, j * 128:(j + 1) * 128])
            qt = _dot(wt[AQ * D:(AQ + 1) * D, :], xns[s], NT)
            pqt_ref[i, :, s * SB:(s + 1) * SB] = _phi(qt).astype(BF16)

    def zero_kv():
        kv_ref[...] = jnp.zeros(kv_ref.shape, F32)
        z_ref[...] = jnp.zeros(z_ref.shape, F32)

    cp_x(0).start()
    for m in (AK, AV, AQ):
        cp_w(m, w_srcs[m]).start()
    x_ref[...] = jnp.zeros(x_ref.shape, F32)
    s_refs[NSB - 1][...] = jnp.zeros((S, TB), F32)
    s_refs[NSB - 2][(NC - LAG) * CK:, :] = jnp.zeros((LAG * CK, TB), F32)
    cp_x(0).wait()
    xn_ref[...] = ln_sub(0, 0)
    for m in (AK, AV, AQ):
        cp_w(m).wait()
    for i in range(1, NB):
        cp_x(i).start()
        for m in (2 * i, 2 * i + 1):
            if m != AK:
                cp_w(m, w_srcs[m]).start()

    def stage_a(r):
        def body(i, xn0):
            for i_s in range(1, NB):
                @pl.when((r == 0) & (i == i_s))
                def _():
                    cp_x(i_s).wait()
                    for m in (2 * i_s, 2 * i_s + 1):
                        if m != AK:
                            cp_w(m).wait()

            xns = [xn0] + [ln_sub(i, s) for s in range(1, NS)]
            pk = a_proj_k(xns)
            transpose_w(2 * i)
            transpose_w(jnp.minimum(2 * i + 1, BO))
            nxt = ln_sub(jnp.minimum(i + 1, NB - 1), 0)
            a_proj_qv(i, xns, pk)
            return nxt
        zero_kv()
        lax.fori_loop(0, NB, body, xn_ref[...])

    def a_mid():
        z = jnp.sum(z_ref[...], axis=0, keepdims=True)
        hr2 = lax.broadcasted_iota(jnp.int32, (H, D), 0)
        hc2 = lax.broadcasted_iota(jnp.int32, (H, D), 1) // DH
        zm_ref[...] = jnp.where(hr2 == hc2, z, 0.0)
        for j, (r0, r1) in enumerate(KV_ROWS):
            k0 = (r0 // 128) * 128
            k1 = -(-r1 // 128) * 128
            hr = (lax.broadcasted_iota(jnp.int32, (r1 - r0, 128), 0) + r0) // DH
            hc = (lax.broadcasted_iota(jnp.int32, (r1 - r0, 128), 1) + j * 128) // DH
            kvj = jnp.where(hr == hc, kv_ref[j, 0:r1 - r0, :], 0.0)
            pads = []
            if r0 > k0:
                pads.append(jnp.zeros((r0 - k0, 128), F32))
            pads.append(kvj)
            if k1 > r1:
                pads.append(jnp.zeros((k1 - r1, 128), F32))
            kvj = jnp.concatenate(pads, axis=0)
            mt_ref[:, j * 128:(j + 1) * 128] = _dot(
                wt[AO * D:(AO + 1) * D, k0:k1], kvj).astype(BF16)

    row8 = lax.broadcasted_iota(jnp.int32, (8, SB), 0)

    def stage_l2(i, c):
        pqns = []
        for s in range(NS):
            pq = pqt_ref[i, :, s * SB:(s + 1) * SB]
            r = 1.0 / (_dot(zm_ref[...], pq) + 1e-6)
            parts = []
            for a in range(H // 2):
                re = jnp.broadcast_to(r[2 * a:2 * a + 1], (8, SB))
                ro = jnp.broadcast_to(r[2 * a + 1:2 * a + 2], (8, SB))
                parts += [re, re, jnp.where(row8 < 4, re, ro), ro, ro]
            pqns.append((pq.astype(F32) * jnp.concatenate(parts, axis=0)).astype(BF16))
        xns = []
        for s in range(NS):
            y = x_ref[srows(i, s), :] + _dot(mt_ref[...], pqns[s]).T
            x_ref[srows(i, s), :] = y
            xns.append(_layernorm(xin[srows(i, s), :].astype(F32) + y).astype(BF16))
        for s in range(NS):
            kt = _dot(wt[BK * D:(BK + 1) * D, :], xns[s], NT)
            qt = _dot(wt[BQ * D:(BQ + 1) * D, :], xns[s], NT) * QSCALE
            zpad = jnp.zeros((8, SB), F32)
            for g in range(NG):
                kparts = []
                for j in range(4):
                    r0 = (2 * g + j // 2) * 40 + (16 if j % 2 else 0)
                    kparts += [kt[r0:r0 + 24], zpad]
                    if j % 2:
                        qb = [jnp.where(row8 < 4, 0.0, qt[r0:r0 + 8]), qt[r0 + 8:r0 + 24], zpad]
                    else:
                        qb = [qt[r0:r0 + 16], jnp.where(row8 < 4, qt[r0 + 16:r0 + 24], 0.0), zpad]
                    qt_ref[4 * g + j, i, :, s * SB:(s + 1) * SB] = pltpu.bitcast(
                        jnp.concatenate(qb, axis=0).astype(BF16), jnp.uint32)
                kb = jnp.concatenate(kparts, axis=0)
                k_ref[g, pl.ds(pl.multiple_of((i * TB + s * SB) // 2, SB // 2), SB // 2), :] = (
                    pltpu.bitcast(kb.T.astype(BF16), jnp.uint32))
            vt_ref[i, :, s * SB:(s + 1) * SB] = _dot(wt[BV * D:(BV + 1) * D, :], xns[s], NT)
        return c

    def attention():
        NQG = NB // QPI
        NP = NG * NQG
        P = 4 * QPI
        row_c = lax.broadcasted_iota(jnp.int32, (8, CK), 0)
        row_q = lax.broadcasted_iota(jnp.int32, (8, TB), 0)

        def get_qm(g, j, q):
            parts = []
            if j > 0:
                parts.append(jnp.zeros((32 * j, TB), BF16))
            parts.append(pltpu.bitcast(qt_ref[4 * g + j, q], BF16))
            if j < 3:
                parts.append(jnp.zeros((96 - 32 * j, TB), BF16))
            return jnp.concatenate(parts, axis=0)

        def qk(g, qm, c, s_ref, mx):
            s = _dot(pltpu.bitcast(k_ref[g, c * CK // 2:(c + 1) * CK // 2, :], BF16), qm)
            s_ref[c * CK:(c + 1) * CK, :] = s
            cm = jnp.max(s.reshape(CK // 8, 8, TB), axis=0)
            return cm if mx is None else jnp.maximum(mx, cm)

        def pv(a, odd, c, s_ref, m, acc, zero):
            sc = s_ref[pl.ds(pl.multiple_of(zero + c * CK, CK), CK), :]
            p = jnp.exp2(sc - m).astype(BF16)
            base = pl.multiple_of(a * 40 + (16 if odd else 0), 8)
            cb, co = (c * CK) // TB, (c * CK) % TB
            v = vt_ref[cb, pl.ds(base, 24), co:co + CK]
            if odd:
                v = jnp.concatenate([jnp.where(row_c < 4, 1.0, v[0:8]), v[8:24]], axis=0)
            else:
                v = jnp.concatenate([v[0:16], jnp.where(row_c >= 4, 1.0, v[16:24])], axis=0)
            o = _dot(v, p)
            return o if acc is None else o + acc

        def finish(a, q, odd, acc, oe):
            if not odd:
                oe = acc * (1.0 / acc[20:21])
                ot_ref[q, pl.ds(pl.multiple_of(a * 40, 8), 16), :] = oe[0:16]
                return oe[16:24]
            oo = acc * (1.0 / acc[0:1])
            mid = jnp.where(row_q < 4, oe, oo[0:8])
            ot_ref[q, pl.ds(pl.multiple_of(a * 40 + 16, 8), 24), :] = jnp.concatenate(
                [mid, oo[8:24]], axis=0)
            return None

        ones24 = jnp.ones((24, TB), F32)
        zero_row = jnp.zeros((1, TB), F32)
        sh = NQG.bit_length() - 1
        LG = NC + LAG

        def body(t, carry):
            m2, m1, acc2 = carry
            zero = jnp.minimum(t, 0)
            tp = jnp.maximum(t - 1, 0)
            g = lax.shift_right_logical(t, sh)
            q0 = (t & (NQG - 1)) * QPI
            a_prev = 2 * lax.shift_right_logical(tp, sh) + 1
            q_prev = (tp & (NQG - 1)) * QPI + QPI - 1
            ms = {-2: m2, -1: m1}
            accs = {-2: acc2}
            oes = {}
            mx = None
            for n in range(P * NC):
                i = n // NC
                c = n % NC
                if c == 0:
                    qm = get_qm(g, i % 4, q0 + i // 4)
                    mx = None
                mx = qk(g, qm, c, s_refs[i % NSB], mx)
                if c == NC - 1:
                    ms[i] = jnp.max(mx, axis=0, keepdims=True)
                n2 = n - LG
                i2 = n2 // NC
                c2 = n2 % NC
                a2 = a_prev if i2 < 0 else 2 * g + (i2 % 4) // 2
                q2 = q_prev if i2 < 0 else q0 + i2 // 4
                accs[i2] = pv(a2, i2 % 2, c2, s_refs[i2 % NSB], ms[i2], accs.get(i2), zero)
                if c2 == NC - 1:
                    oes[i2] = finish(a2, q2, i2 % 2, accs[i2], oes.get(i2 - 1))
            return ms[P - 2], ms[P - 1], accs[P - 2]

        m2, m1, acc = SCOPE('s_attn_loop', lambda: lax.fori_loop(
            0, NP, body, (zero_row, zero_row, ones24)))

        def epilogue():
            acc2 = acc
            for c2 in range(NC - LAG, NC):
                acc2 = pv(H // 2 - 1, 0, c2, s_refs[NSB - 2], m2, acc2, 0)
            oe = finish(H // 2 - 1, NB - 1, 0, acc2, None)
            yield
            acc1 = None
            for c2 in range(NC):
                acc1 = pv(H // 2 - 1, 1, c2, s_refs[NSB - 1], m1, acc1, 0)
                yield
            finish(H // 2 - 1, NB - 1, 1, acc1, oe)
            yield
        return epilogue()

    def out_copy(i, s):
        k = i * NS + s
        return pltpu.make_async_copy(obuf.at[k * SB:(k + 1) * SB, :],
                                     out_hbm.at[k * SB:(k + 1) * SB, :], osems.at[k])

    def stage_bout(r, epi):
        @pl.when(r == 1)
        def _():
            for i in range(NB):
                for s in range(NS):
                    out_copy(i, s).wait()
        def blk(i):
            for s in range(NS):
                if i < NB - 1:
                    for _ in range(2):
                        next(epi, None)
                yt = _dot(wt[BO * D:(BO + 1) * D, :], ot_ref[i, :, s * SB:(s + 1) * SB])
                y = x_ref[srows(i, s), :] + yt.T
                x_ref[srows(i, s), :] = y
                x = xin[srows(i, s), :].astype(F32) + y
                obuf[srows(i, s), :] = x.astype(obuf.dtype)
                out_copy(i, s).start()
                if i == 0 and s == 0:
                    xn_ref[...] = _layernorm(x).astype(BF16)
        for i in range(NB - 1):
            blk(i)

        @pl.when(r >= 0)
        def _():
            blk(NB - 1)

    def round_(r, c):
        SCOPE('s_a', stage_a, r)
        SCOPE('s_amid', a_mid)
        SCOPE('s_l2', lambda: lax.fori_loop(0, NB, stage_l2, 0))
        epi = attention()
        SCOPE('s_bout', stage_bout, r, epi)
        return c
    lax.fori_loop(0, 2, round_, 0)
    for i in range(NB):
        for s in range(NS):
            out_copy(i, s).wait()


@jax.jit
def pallas_interleave_layers__linear_attn_block__mha_block__prompt_kernel(
    A_x: jax.Array,
    A_wqkv: jax.Array,
    A_wo: jax.Array,
    B_x: jax.Array,
    B_wqkv: jax.Array,
    B_wo: jax.Array,
):
    x = A_x.reshape(S, D)
    scratch = [
        pltpu.VMEM((S, D), BF16),
        pltpu.VMEM((8, D, D), BF16),
        pltpu.VMEM((S, D), BF16),
        pltpu.SemaphoreType.DMA((NB + 8,)),
        pltpu.SemaphoreType.DMA((NB * NS,)),
        pltpu.VMEM((S, D), F32),
        pltpu.VMEM((SB, D), BF16),
        pltpu.VMEM((7 * D, D), BF16),
        pltpu.VMEM((NB, D, TB), BF16),
        pltpu.VMEM((5, 160, 128), F32),
        pltpu.VMEM((8, D), F32),
        pltpu.VMEM((D, D), BF16),
        pltpu.VMEM((H, D), F32),
        pltpu.VMEM((NG, S // 2, 128), jnp.uint32),
        pltpu.VMEM((H, NB, 16, TB), jnp.uint32),
        pltpu.VMEM((NB, D, TB), F32),
        pltpu.VMEM((NB, D, TB), F32),
    ] + [pltpu.VMEM((S, TB), F32) for _ in range(NSB)]
    out = pl.pallas_call(
        _kernel,
        out_shape=jax.ShapeDtypeStruct((S, D), A_x.dtype),
        in_specs=[pl.BlockSpec(memory_space=pl.ANY)] * 5,
        out_specs=pl.BlockSpec(memory_space=pl.ANY),
        scratch_shapes=scratch,
        compiler_params=pltpu.CompilerParams(vmem_limit_bytes=110 * 1024 * 1024),
    )(x, A_wqkv, A_wo, B_wqkv, B_wo)
    return out.reshape(A_x.shape)
```

```python
import math

import jax
import jax.numpy as jnp
from jax import lax
import jax.experimental.pallas as pl
import jax.experimental.pallas.tpu as pltpu

S = 2048
D = 640
H = 32
DH = 20
NG = 8
TB = 512
NB = S // TB
SB = 128
NS = TB // SB
CK = 128
NC = S // CK
QPI = 2
LAG = 1
NSB = 4
GPOS = 2
LN_EPS = 1e-5
QSCALE = (DH ** -0.5) * math.log2(math.e)
KV_ROWS = [(0, 144), (120, 264), (240, 400), (376, 520), (496, 640)]
AQ, AV, BQ, BK, BV, AO, BO, AK = range(8)

F32 = jnp.float32
BF16 = jnp.bfloat16
NN = (((1,), (0,)), ((), ()))
NT = (((1,), (1,)), ((), ()))


def SCOPE(name, f, *args):
    del name
    return f(*args)


def _dot(a, b, dims=NN):
    return lax.dot_general(a, b, dims, preferred_element_type=F32)


def _phi(t):
    return jnp.where(t > 0, t + 1.0, jnp.exp(jnp.minimum(t, 0.0))) + 1e-6


def _layernorm(x):
    m = jnp.mean(x, axis=-1, keepdims=True)
    xc = x - m
    v = jnp.mean(xc * xc, axis=-1, keepdims=True)
    return xc * lax.rsqrt(v + LN_EPS)


def _kernel(x_hbm, awqkv_hbm, awo_hbm, bwqkv_hbm, bwo_hbm, out_hbm,
            xin, wsrc, obuf, sems, osems,
            x_ref, xn_ref, wt, wkt_a,
            pqt_ref, gt_ref, z_ref, mt_ref, r_ref, zmask_ref, kvmask_ref,
            k_ref, qt_ref, vt_ref, ot_ref, *s_refs):
    def rows(i):
        return pl.ds(pl.multiple_of(i * TB, TB), TB)

    def srows(i, s):
        if isinstance(i, int):
            return pl.ds(i * TB + s * SB, SB)
        return pl.ds(pl.multiple_of(i * TB + s * SB, SB), SB)

    def cols(c):
        return pl.ds(c * D, D)

    def cp_x(i):
        lo = 0 if i == 0 else i * TB + SB
        hi = min((i + 1) * TB + SB, S)
        return pltpu.make_async_copy(x_hbm.at[lo:hi, :], xin.at[lo:hi, :], sems.at[i])

    w_srcs = {AQ: awqkv_hbm.at[:, cols(0)], AV: awqkv_hbm.at[:, cols(2)],
              BQ: bwqkv_hbm.at[:, cols(0)], BK: bwqkv_hbm.at[:, cols(1)],
              BV: bwqkv_hbm.at[:, cols(2)], AO: awo_hbm, BO: bwo_hbm,
              AK: awqkv_hbm.at[:, cols(1)]}

    def cp_w(m, src=None):
        src = awo_hbm if src is None else src
        return pltpu.make_async_copy(src, wsrc.at[m], sems.at[NB + m])

    def transpose_w(m):
        wt[pl.ds(pl.multiple_of(m * D, D), D), :] = wsrc[m].astype(F32).T.astype(BF16)

    def resid(i, s):
        return xin[srows(i, s), :].astype(F32) + x_ref[srows(i, s), :]

    def ln_sub(i, s):
        return _layernorm(resid(i, s)).astype(BF16)

    cp_w(AK, w_srcs[AK]).start()
    x_ref[...] = jnp.zeros(x_ref.shape, F32)
    cp_x(0).start()
    cp_w(AQ, w_srcs[AQ]).start()
    hr2 = lax.broadcasted_iota(jnp.int32, (H, D), 0)
    hc2 = lax.broadcasted_iota(jnp.int32, (H, D), 1) // DH
    zmask_ref[...] = (hr2 == hc2).astype(jnp.int32)
    for j, (r0, r1) in enumerate(KV_ROWS):
        hr = (lax.broadcasted_iota(jnp.int32, (160, 128), 0) + r0) // DH
        hc = (lax.broadcasted_iota(jnp.int32, (160, 128), 1) + j * 128) // DH
        kvmask_ref[j] = (hr == hc).astype(jnp.int32)
    cp_w(AK).wait()
    wkt_a[...] = wsrc[AK].astype(F32).T.astype(BF16)
    s_refs[NSB - 1][...] = jnp.zeros((S, TB), F32)
    s_refs[NSB - 2][(NC - LAG) * CK:, :] = jnp.zeros((LAG * CK, TB), F32)
    cp_x(0).wait()
    xn_ref[0] = ln_sub(0, 0)
    cp_w(AQ).wait()
    for i in range(1, NB):
        cp_x(i).start()
        for m in (2 * i - 1, 2 * i):
            cp_w(m, w_srcs[m]).start()

    def stage_a(r):
        def body(i, c):
            for i_s in range(1, NB):
                @pl.when((r == 0) & (i == i_s))
                def _():
                    cp_x(i_s).wait()
                    for m in (2 * i_s - 1, 2 * i_s):
                        cp_w(m).wait()

            xns = [xn_ref[i & 1]] + [ln_sub(i, s) for s in range(1, NS)]
            pkts = [_phi(_dot(wkt_a[...], xn, NT)) for xn in xns]
            transpose_w(jnp.maximum(2 * i - 1, 0))
            transpose_w(2 * i)
            xn_ref[(i + 1) & 1] = ln_sub(jnp.minimum(i + 1, NB - 1), 0)
            xn0_late = xn_ref[i & 1]
            z_ref[...] = (jnp.where(i > 0, z_ref[...], 0.0)
                          + (pkts[0] + pkts[1]) + (pkts[2] + pkts[3]))
            for s in range(NS):
                if s == GPOS:
                    gt_ref[...] = _dot(
                        jnp.concatenate(pkts, axis=1),
                        jnp.concatenate([xn0_late] + xns[1:], axis=0)
                    ) + jnp.where(i > 0, gt_ref[...], 0.0)
                qt = _dot(wt[AQ * D:(AQ + 1) * D, :], xns[s], NT)
                pqt_ref[i, :, s * SB:(s + 1) * SB] = _phi(qt).astype(BF16)
            return c
        lax.fori_loop(0, NB, body, 0)

    def a_mid():
        z = _dot(jnp.ones((8, 128), F32), z_ref[...], NT)[0:1]
        zm = jnp.where(zmask_ref[...] > 0, z, 0.0)
        kvs = []
        for j, (r0, r1) in enumerate(KV_ROWS):
            kvj = _dot(wt[AV * D + r0:AV * D + r1, :], gt_ref[j * 128:(j + 1) * 128, :], NT)
            kvs.append(jnp.where(kvmask_ref[j, 0:r1 - r0, :] > 0, kvj, 0.0))
        for j, (r0, r1) in enumerate(KV_ROWS):
            if j < NB:
                r_ref[j] = 1.0 / (_dot(zm, pqt_ref[j]) + 1e-6)
            k0 = (r0 // 128) * 128
            k1 = -(-r1 // 128) * 128
            pads = []
            if r0 > k0:
                pads.append(jnp.zeros((r0 - k0, 128), F32))
            pads.append(kvs[j])
            if k1 > r1:
                pads.append(jnp.zeros((k1 - r1, 128), F32))
            kvj = jnp.concatenate(pads, axis=0)
            mt_ref[:, j * 128:(j + 1) * 128] = _dot(
                wt[AO * D:(AO + 1) * D, k0:k1], kvj).astype(BF16)

    row8 = lax.broadcasted_iota(jnp.int32, (8, SB), 0)

    def stage_l2(i, c):
        pqns = []
        for s in range(NS):
            pq = pqt_ref[i, :, s * SB:(s + 1) * SB]
            r = r_ref[i, :, s * SB:(s + 1) * SB]
            parts = []
            for a in range(H // 2):
                re = jnp.broadcast_to(r[2 * a:2 * a + 1], (8, SB))
                ro = jnp.broadcast_to(r[2 * a + 1:2 * a + 2], (8, SB))
                parts += [re, re, jnp.where(row8 < 4, re, ro), ro, ro]
            pqns.append((pq.astype(F32) * jnp.concatenate(parts, axis=0)).astype(BF16))
        xns = []
        for s in range(NS):
            y = x_ref[srows(i, s), :] + _dot(mt_ref[...], pqns[s]).T
            x_ref[srows(i, s), :] = y
            xns.append(_layernorm(xin[srows(i, s), :].astype(F32) + y).astype(BF16))
        for s in range(NS):
            kt = _dot(wt[BK * D:(BK + 1) * D, :], xns[s], NT)
            qt = _dot(wt[BQ * D:(BQ + 1) * D, :], xns[s], NT) * QSCALE
            zpad = jnp.zeros((8, SB), F32)
            for g in range(NG):
                kparts = []
                for j in range(4):
                    r0 = (2 * g + j // 2) * 40 + (16 if j % 2 else 0)
                    kparts += [kt[r0:r0 + 24], zpad]
                    if j % 2:
                        qb = [jnp.where(row8 < 4, 0.0, qt[r0:r0 + 8]), qt[r0 + 8:r0 + 24], zpad]
                    else:
                        qb = [qt[r0:r0 + 16], jnp.where(row8 < 4, qt[r0 + 16:r0 + 24], 0.0), zpad]
                    qt_ref[4 * g + j, i, :, s * SB:(s + 1) * SB] = pltpu.bitcast(
                        jnp.concatenate(qb, axis=0).astype(BF16), jnp.uint32)
                kb = jnp.concatenate(kparts, axis=0)
                k_ref[g, pl.ds(pl.multiple_of((i * TB + s * SB) // 2, SB // 2), SB // 2), :] = (
                    pltpu.bitcast(kb.T.astype(BF16), jnp.uint32))
            vt_ref[i, :, s * SB:(s + 1) * SB] = _dot(wt[BV * D:(BV + 1) * D, :], xns[s], NT)
        return c

    def attention():
        NQG = NB // QPI
        NP = NG * NQG
        P = 4 * QPI
        row_c = lax.broadcasted_iota(jnp.int32, (8, CK), 0)
        row_q = lax.broadcasted_iota(jnp.int32, (8, TB), 0)

        def get_qm(g, j, q):
            parts = []
            if j > 0:
                parts.append(jnp.zeros((32 * j, TB), BF16))
            parts.append(pltpu.bitcast(qt_ref[4 * g + j, q], BF16))
            if j < 3:
                parts.append(jnp.zeros((96 - 32 * j, TB), BF16))
            return jnp.concatenate(parts, axis=0)

        def qk(g, qm, c, s_ref, mx):
            s = _dot(pltpu.bitcast(k_ref[g, c * CK // 2:(c + 1) * CK // 2, :], BF16), qm)
            s_ref[c * CK:(c + 1) * CK, :] = s
            cm = jnp.max(s.reshape(CK // 8, 8, TB), axis=0)
            return cm if mx is None else jnp.maximum(mx, cm)

        def pv(a, odd, c, s_ref, m, acc, zero):
            sc = s_ref[pl.ds(pl.multiple_of(zero + c * CK, CK), CK), :]
            p = jnp.exp2(sc - m).astype(BF16)
            base = pl.multiple_of(a * 40 + (16 if odd else 0), 8)
            cb, co = (c * CK) // TB, (c * CK) % TB
            v = vt_ref[cb, pl.ds(base, 24), co:co + CK]
            if odd:
                v = jnp.concatenate([jnp.where(row_c < 4, 1.0, v[0:8]), v[8:24]], axis=0)
            else:
                v = jnp.concatenate([v[0:16], jnp.where(row_c >= 4, 1.0, v[16:24])], axis=0)
            o = _dot(v, p)
            return o if acc is None else o + acc

        def finish(a, q, odd, acc, oe):
            if not odd:
                oe = acc * (1.0 / acc[20:21])
                ot_ref[q, pl.ds(pl.multiple_of(a * 40, 8), 16), :] = oe[0:16]
                return oe[16:24]
            oo = acc * (1.0 / acc[0:1])
            mid = jnp.where(row_q < 4, oe, oo[0:8])
            ot_ref[q, pl.ds(pl.multiple_of(a * 40 + 16, 8), 24), :] = jnp.concatenate(
                [mid, oo[8:24]], axis=0)
            return None

        ones24 = jnp.ones((24, TB), F32)
        zero_row = jnp.zeros((1, TB), F32)
        sh = NQG.bit_length() - 1
        LG = NC + LAG

        def body(t, carry):
            m2, m1, acc2 = carry
            zero = jnp.minimum(t, 0)
            tp = jnp.maximum(t - 1, 0)
            g = lax.shift_right_logical(t, sh)
            q0 = (t & (NQG - 1)) * QPI
            a_prev = 2 * lax.shift_right_logical(tp, sh) + 1
            q_prev = (tp & (NQG - 1)) * QPI + QPI - 1
            ms = {-2: m2, -1: m1}
            accs = {-2: acc2}
            oes = {}
            mx = None
            for n in range(P * NC):
                i = n // NC
                c = n % NC
                if c == 0:
                    qm = get_qm(g, i % 4, q0 + i // 4)
                    mx = None
                mx = qk(g, qm, c, s_refs[i % NSB], mx)
                if c == NC - 1:
                    ms[i] = jnp.max(mx, axis=0, keepdims=True)
                n2 = n - LG
                i2 = n2 // NC
                c2 = n2 % NC
                a2 = a_prev if i2 < 0 else 2 * g + (i2 % 4) // 2
                q2 = q_prev if i2 < 0 else q0 + i2 // 4
                accs[i2] = pv(a2, i2 % 2, c2, s_refs[i2 % NSB], ms[i2], accs.get(i2), zero)
                if c2 == NC - 1:
                    oes[i2] = finish(a2, q2, i2 % 2, accs[i2], oes.get(i2 - 1))
            return ms[P - 2], ms[P - 1], accs[P - 2]

        m2, m1, acc = SCOPE('s_attn_loop', lambda: lax.fori_loop(
            0, NP, body, (zero_row, zero_row, ones24)))

        def epilogue():
            acc2 = acc
            for c2 in range(NC - LAG, NC):
                acc2 = pv(H // 2 - 1, 0, c2, s_refs[NSB - 2], m2, acc2, 0)
            oe = finish(H // 2 - 1, NB - 1, 0, acc2, None)
            yield
            acc1 = None
            for c2 in range(NC):
                acc1 = pv(H // 2 - 1, 1, c2, s_refs[NSB - 1], m1, acc1, 0)
                yield
            finish(H // 2 - 1, NB - 1, 1, acc1, oe)
            yield
        return epilogue()

    def out_copy(i, s):
        k = i * NS + s
        return pltpu.make_async_copy(obuf.at[k * SB:(k + 1) * SB, :],
                                     out_hbm.at[k * SB:(k + 1) * SB, :], osems.at[k])

    def stage_bout(r, epi):
        @pl.when(r == 1)
        def _():
            for i in range(NB):
                for s in range(NS):
                    out_copy(i, s).wait()
        def blk(i):
            for s in range(NS):
                if i < NB - 1:
                    for _ in range(2):
                        next(epi, None)
                yt = _dot(wt[BO * D:(BO + 1) * D, :], ot_ref[i, :, s * SB:(s + 1) * SB])
                y = x_ref[srows(i, s), :] + yt.T
                x_ref[srows(i, s), :] = y
                x = xin[srows(i, s), :].astype(F32) + y
                obuf[srows(i, s), :] = x.astype(obuf.dtype)
                out_copy(i, s).start()
                if i == 0 and s == 0:
                    xn_ref[0] = _layernorm(x).astype(BF16)
        for i in range(NB - 1):
            blk(i)

        @pl.when(r >= 0)
        def _():
            blk(NB - 1)

    def round_(r, c):
        SCOPE('s_a', stage_a, r)
        SCOPE('s_amid', a_mid)
        SCOPE('s_l2', lambda: lax.fori_loop(0, NB, stage_l2, 0))
        epi = attention()
        SCOPE('s_bout', stage_bout, r, epi)
        return c
    lax.fori_loop(0, 2, round_, 0)
    for i in range(NB):
        for s in range(NS):
            out_copy(i, s).wait()


@jax.jit
def pallas_interleave_layers__linear_attn_block__mha_block__prompt_kernel(
    A_x: jax.Array,
    A_wqkv: jax.Array,
    A_wo: jax.Array,
    B_x: jax.Array,
    B_wqkv: jax.Array,
    B_wo: jax.Array,
):
    x = A_x.reshape(S, D)
    scratch = [
        pltpu.VMEM((S, D), BF16),
        pltpu.VMEM((8, D, D), BF16),
        pltpu.VMEM((S, D), BF16),
        pltpu.SemaphoreType.DMA((NB + 8,)),
        pltpu.SemaphoreType.DMA((NB * NS,)),
        pltpu.VMEM((S, D), F32),
        pltpu.VMEM((2, SB, D), BF16),
        pltpu.VMEM((7 * D, D), BF16),
        pltpu.VMEM((D, D), BF16),
        pltpu.VMEM((NB, D, TB), BF16),
        pltpu.VMEM((D, D), F32),
        pltpu.VMEM((D, 128), F32),
        pltpu.VMEM((D, D), BF16),
        pltpu.VMEM((NB, H, TB), F32),
        pltpu.VMEM((H, D), jnp.int32),
        pltpu.VMEM((5, 160, 128), jnp.int32),
        pltpu.VMEM((NG, S // 2, 128), jnp.uint32),
        pltpu.VMEM((H, NB, 16, TB), jnp.uint32),
        pltpu.VMEM((NB, D, TB), F32),
        pltpu.VMEM((NB, D, TB), F32),
    ] + [pltpu.VMEM((S, TB), F32) for _ in range(NSB)]
    out = pl.pallas_call(
        _kernel,
        out_shape=jax.ShapeDtypeStruct((S, D), A_x.dtype),
        in_specs=[pl.BlockSpec(memory_space=pl.ANY)] * 5,
        out_specs=pl.BlockSpec(memory_space=pl.ANY),
        scratch_shapes=scratch,
        compiler_params=pltpu.CompilerParams(vmem_limit_bytes=110 * 1024 * 1024),
    )(x, A_wqkv, A_wo, B_wqkv, B_wo)
    return out.reshape(A_x.shape)
```

```python
import math

import jax
import jax.numpy as jnp
from jax import lax
import jax.experimental.pallas as pl
import jax.experimental.pallas.tpu as pltpu

S = 2048
D = 640
H = 32
DH = 20
NG = 8
TB = 512
NB = S // TB
SB = 128
NS = TB // SB
CK = 128
NC = S // CK
QPI = 2
LAG = 1
NSB = 4
GPOS = 2
FORMB = 1
LN_EPS = 1e-5
QSCALE = (DH ** -0.5) * math.log2(math.e)
KV_ROWS = [(0, 144), (112, 272), (240, 400), (368, 528), (496, 640)]
AQ, AV, BQ, BK, BV, AO, BO, AK = range(8)

F32 = jnp.float32
BF16 = jnp.bfloat16
U32 = jnp.uint32
NN = (((1,), (0,)), ((), ()))
NT = (((1,), (1,)), ((), ()))


def SCOPE(name, f, *args):
    del name
    return f(*args)


def _dot(a, b, dims=NN):
    return lax.dot_general(a, b, dims, preferred_element_type=F32)


def _pk(x):
    return pltpu.bitcast(x, jnp.uint32)


def _up(x):
    return pltpu.bitcast(x, BF16)


def _phi(t):
    return jnp.where(t > 0, t + 1.0, jnp.exp(jnp.minimum(t, 0.0))) + 1e-6


def _layernorm(x):
    m = jnp.mean(x, axis=-1, keepdims=True)
    xc = x - m
    v = jnp.mean(xc * xc, axis=-1, keepdims=True)
    return xc * lax.rsqrt(v + LN_EPS)


def _kernel(x_hbm, awqkv_hbm, awo_hbm, bwqkv_hbm, bwo_hbm, out_hbm,
            xin, wsrc, obuf, sems, osems,
            x_ref, xn_ref, wt, wkt_a,
            pqt_ref, gt_ref, z_ref, mt_ref, r_ref, zmask_ref, kvmask_ref,
            k_ref, qt_ref, vt_ref, ot_ref, *s_refs):
    def rows(i):
        return pl.ds(pl.multiple_of(i * TB, TB), TB)

    def srows(i, s):
        if isinstance(i, int):
            return pl.ds(i * TB + s * SB, SB)
        return pl.ds(pl.multiple_of(i * TB + s * SB, SB), SB)

    def cols(c):
        return pl.ds(c * D, D)

    def cp_x(i):
        lo = 0 if i == 0 else i * TB + SB
        hi = min((i + 1) * TB + SB, S)
        return pltpu.make_async_copy(x_hbm.at[lo:hi, :], xin.at[lo:hi, :], sems.at[i])

    w_srcs = {AQ: awqkv_hbm.at[:, cols(0)], AV: awqkv_hbm.at[:, cols(2)],
              BQ: bwqkv_hbm.at[:, cols(0)], BK: bwqkv_hbm.at[:, cols(1)],
              BV: bwqkv_hbm.at[:, cols(2)], AO: awo_hbm, BO: bwo_hbm,
              AK: awqkv_hbm.at[:, cols(1)]}

    def cp_w(m, src=None):
        src = awo_hbm if src is None else src
        return pltpu.make_async_copy(src, wsrc.at[m], sems.at[NB + m])

    def transpose_w(m):
        wt[m] = _pk(wsrc[m].T)

    def resid(i, s):
        return xin[srows(i, s), :].astype(F32) + x_ref[srows(i, s), :]

    def ln_sub(i, s):
        return _layernorm(resid(i, s)).astype(BF16)

    cp_w(AK, w_srcs[AK]).start()
    x_ref[...] = jnp.zeros(x_ref.shape, F32)
    cp_x(0).start()
    cp_w(AQ, w_srcs[AQ]).start()
    hr2 = lax.broadcasted_iota(jnp.int32, (H, D), 0)
    hc2 = lax.broadcasted_iota(jnp.int32, (H, D), 1) // DH
    zmask_ref[...] = (hr2 == hc2).astype(jnp.int32)
    for j, (r0, r1) in enumerate(KV_ROWS):
        hr = (lax.broadcasted_iota(jnp.int32, (160, 128), 0) + r0) // DH
        hc = (lax.broadcasted_iota(jnp.int32, (160, 128), 1) + j * 128) // DH
        kvmask_ref[j] = (hr == hc).astype(jnp.int32)
    cp_w(AK).wait()
    wkt_a[...] = _pk(wsrc[AK].T)
    s_refs[NSB - 1][...] = jnp.zeros((S, TB), F32)
    s_refs[NSB - 2][(NC - LAG) * CK:, :] = jnp.zeros((LAG * CK, TB), F32)
    cp_x(0).wait()
    xn_ref[0] = _pk(ln_sub(0, 0))
    cp_w(AQ).wait()
    for i in range(1, NB):
        cp_x(i).start()
        for m in (2 * i - 1, 2 * i):
            cp_w(m, w_srcs[m]).start()

    def stage_a(r):
        def body(i, c):
            for i_s in range(1, NB):
                @pl.when((r == 0) & (i == i_s))
                def _():
                    cp_x(i_s).wait()
                    for m in (2 * i_s - 1, 2 * i_s):
                        cp_w(m).wait()

            xns = [_up(xn_ref[i & 1])] + [ln_sub(i, s) for s in range(1, NS)]
            pkts = [_phi(_dot(_up(wkt_a[...]), xn, NT)) for xn in xns]
            transpose_w(jnp.maximum(2 * i - 1, 0))
            transpose_w(2 * i)
            xn_ref[(i + 1) & 1] = _pk(ln_sub(jnp.minimum(i + 1, NB - 1), 0))
            xn0_late = _up(xn_ref[i & 1])
            z_ref[...] = (jnp.where(i > 0, z_ref[...], 0.0)
                          + (pkts[0] + pkts[1]) + (pkts[2] + pkts[3]))
            for s in range(NS):
                if s == GPOS:
                    gt_ref[...] = _dot(
                        jnp.concatenate(pkts, axis=1),
                        jnp.concatenate([xn0_late] + xns[1:], axis=0)
                    ) + jnp.where(i > 0, gt_ref[...], 0.0)
                qt = _dot(_up(wt[AQ]), xns[s], NT)
                pqt_ref[i, :, s * SB:(s + 1) * SB] = _pk(_phi(qt).astype(BF16))
            return c
        lax.fori_loop(0, NB, body, 0)

    def a_mid():
        z = _dot(jnp.ones((8, 128), F32), z_ref[...], NT)[0:1]
        zm = jnp.where(zmask_ref[...] > 0, z, 0.0)
        kvs = []
        for j, (r0, r1) in enumerate(KV_ROWS):
            kvj = _dot(_up(wt[AV, r0 // 2:r1 // 2, :]), gt_ref[j * 128:(j + 1) * 128, :], NT)
            kvs.append(jnp.where(kvmask_ref[j, 0:r1 - r0, :] > 0, kvj, 0.0))
        for j, (r0, r1) in enumerate(KV_ROWS):
            if j < NB:
                r_ref[j] = 1.0 / (_dot(zm, _up(pqt_ref[j])) + 1e-6)
            k0 = (r0 // 128) * 128
            k1 = -(-r1 // 128) * 128
            pads = []
            if r0 > k0:
                pads.append(jnp.zeros((r0 - k0, 128), F32))
            pads.append(kvs[j])
            if k1 > r1:
                pads.append(jnp.zeros((k1 - r1, 128), F32))
            kvj = jnp.concatenate(pads, axis=0)
            mt_ref[:, j * 128:(j + 1) * 128] = _pk(_dot(
                _up(wt[AO, :, k0:k1]), kvj).astype(BF16))

    row8 = lax.broadcasted_iota(jnp.int32, (8, SB), 0)

    def stage_l2(i, c):
        pqns = []
        for s in range(NS):
            pq = _up(pqt_ref[i, :, s * SB:(s + 1) * SB])
            r = r_ref[i, :, s * SB:(s + 1) * SB]
            parts = []
            for a in range(H // 2):
                re = jnp.broadcast_to(r[2 * a:2 * a + 1], (8, SB))
                ro = jnp.broadcast_to(r[2 * a + 1:2 * a + 2], (8, SB))
                parts += [re, re, jnp.where(row8 < 4, re, ro), ro, ro]
            pqns.append((pq.astype(F32) * jnp.concatenate(parts, axis=0)).astype(BF16))
        xns = []
        for s in range(NS):
            y = x_ref[srows(i, s), :] + _dot(_up(mt_ref[...]), pqns[s]).T
            x_ref[srows(i, s), :] = y
            xns.append(_layernorm(xin[srows(i, s), :].astype(F32) + y).astype(BF16))
        for s in range(NS):
            kt = _dot(_up(wt[BK]), xns[s], NT)
            qt = _dot(_up(wt[BQ]), xns[s], NT) * QSCALE
            zpad = jnp.zeros((8, SB), F32)
            for g in range(NG):
                kparts = []
                for j in range(4):
                    r0 = (2 * g + j // 2) * 40 + (16 if j % 2 else 0)
                    kparts += [kt[r0:r0 + 24], zpad]
                    if j % 2:
                        qb = [jnp.where(row8 < 4, 0.0, qt[r0:r0 + 8]), qt[r0 + 8:r0 + 24], zpad]
                    else:
                        qb = [qt[r0:r0 + 16], jnp.where(row8 < 4, qt[r0 + 16:r0 + 24], 0.0), zpad]
                    qt_ref[4 * g + j, i, :, s * SB:(s + 1) * SB] = pltpu.bitcast(
                        jnp.concatenate(qb, axis=0).astype(BF16), jnp.uint32)
                kb = jnp.concatenate(kparts, axis=0)
                k_ref[g, pl.ds(pl.multiple_of((i * TB + s * SB) // 2, SB // 2), SB // 2), :] = (
                    pltpu.bitcast(kb.T.astype(BF16), jnp.uint32))
            vt_ref[i, :, s * SB:(s + 1) * SB] = _dot(_up(wt[BV]), xns[s], NT)
        return c

    def attention():
        NQG = NB // QPI
        NP = NG * NQG
        P = 4 * QPI
        row_c = lax.broadcasted_iota(jnp.int32, (8, CK), 0)
        row_q = lax.broadcasted_iota(jnp.int32, (8, TB), 0)

        def get_qm(g, j, q):
            parts = []
            if j > 0:
                parts.append(jnp.zeros((32 * j, TB), BF16))
            parts.append(pltpu.bitcast(qt_ref[4 * g + j, q], BF16))
            if j < 3:
                parts.append(jnp.zeros((96 - 32 * j, TB), BF16))
            return jnp.concatenate(parts, axis=0)

        def qk(g, qm, c, s_ref, mx):
            s = _dot(pltpu.bitcast(k_ref[g, c * CK // 2:(c + 1) * CK // 2, :], BF16), qm)
            s_ref[c * CK:(c + 1) * CK, :] = s
            cm = jnp.max(s.reshape(CK // 8, 8, TB), axis=0)
            return cm if mx is None else jnp.maximum(mx, cm)

        def pv(a, odd, c, s_ref, m, acc, zero):
            sc = s_ref[pl.ds(pl.multiple_of(zero + c * CK, CK), CK), :]
            p = jnp.exp2(sc - m).astype(BF16)
            base = pl.multiple_of(a * 40 + (16 if odd else 0), 8)
            cb, co = (c * CK) // TB, (c * CK) % TB
            v = vt_ref[cb, pl.ds(base, 24), co:co + CK]
            if odd:
                v = jnp.concatenate([jnp.where(row_c < 4, 1.0, v[0:8]), v[8:24]], axis=0)
            else:
                v = jnp.concatenate([v[0:16], jnp.where(row_c >= 4, 1.0, v[16:24])], axis=0)
            o = _dot(v, p)
            return o if acc is None else o + acc

        def finish(a, q, odd, acc, oe):
            if not odd:
                oe = acc * (1.0 / acc[20:21])
                ot_ref[q, pl.ds(pl.multiple_of(a * 40, 8), 16), :] = oe[0:16]
                return oe[16:24]
            oo = acc * (1.0 / acc[0:1])
            mid = jnp.where(row_q < 4, oe, oo[0:8])
            ot_ref[q, pl.ds(pl.multiple_of(a * 40 + 16, 8), 24), :] = jnp.concatenate(
                [mid, oo[8:24]], axis=0)
            return None

        ones24 = jnp.ones((24, TB), F32)
        zero_row = jnp.zeros((1, TB), F32)
        sh = NQG.bit_length() - 1
        LG = NC + LAG

        def body(t, carry):
            m2, m1, acc2 = carry
            zero = jnp.minimum(t, 0)
            tp = jnp.maximum(t - 1, 0)
            g = lax.shift_right_logical(t, sh)
            q0 = (t & (NQG - 1)) * QPI
            a_prev = 2 * lax.shift_right_logical(tp, sh) + 1
            q_prev = (tp & (NQG - 1)) * QPI + QPI - 1
            ms = {-2: m2, -1: m1}
            accs = {-2: acc2}
            oes = {}
            mx = None
            for n in range(P * NC):
                i = n // NC
                c = n % NC
                if c == 0:
                    qm = get_qm(g, i % 4, q0 + i // 4)
                    mx = None
                mx = qk(g, qm, c, s_refs[i % NSB], mx)
                if c == NC - 1:
                    ms[i] = jnp.max(mx, axis=0, keepdims=True)
                n2 = n - LG
                i2 = n2 // NC
                c2 = n2 % NC
                a2 = a_prev if i2 < 0 else 2 * g + (i2 % 4) // 2
                q2 = q_prev if i2 < 0 else q0 + i2 // 4
                accs[i2] = pv(a2, i2 % 2, c2, s_refs[i2 % NSB], ms[i2], accs.get(i2), zero)
                if c2 == NC - 1:
                    oes[i2] = finish(a2, q2, i2 % 2, accs[i2], oes.get(i2 - 1))
            return ms[P - 2], ms[P - 1], accs[P - 2]

        m2, m1, acc = SCOPE('s_attn_loop', lambda: lax.fori_loop(
            0, NP, body, (zero_row, zero_row, ones24)))

        def epilogue():
            acc2 = acc
            for c2 in range(NC - LAG, NC):
                acc2 = pv(H // 2 - 1, 0, c2, s_refs[NSB - 2], m2, acc2, 0)
            oe = finish(H // 2 - 1, NB - 1, 0, acc2, None)
            yield
            acc1 = None
            for c2 in range(NC):
                acc1 = pv(H // 2 - 1, 1, c2, s_refs[NSB - 1], m1, acc1, 0)
                yield
            finish(H // 2 - 1, NB - 1, 1, acc1, oe)
            yield
        return epilogue()

    def out_copy(i, s):
        k = i * NS + s
        return pltpu.make_async_copy(obuf.at[k * SB:(k + 1) * SB, :],
                                     out_hbm.at[k * SB:(k + 1) * SB, :], osems.at[k])

    def stage_bout(r, epi):
        @pl.when(r == 1)
        def _():
            for i in range(NB):
                for s in range(NS):
                    out_copy(i, s).wait()
        def blk(i):
            for s in range(NS):
                ot = ot_ref[i, :, s * SB:(s + 1) * SB]
                if s < FORMB and i in (0, NB - 1):
                    yy = _dot(_up(wt[BO]), ot).T
                else:
                    yy = _dot(ot.T.astype(BF16), wsrc[BO])
                if i < NB - 1:
                    for _ in range(2):
                        next(epi, None)
                y = x_ref[srows(i, s), :] + yy
                x_ref[srows(i, s), :] = y
                x = xin[srows(i, s), :].astype(F32) + y
                obuf[srows(i, s), :] = x.astype(obuf.dtype)
                out_copy(i, s).start()
                if i == 0 and s == 0:
                    xn_ref[0] = _pk(_layernorm(x).astype(BF16))
        for i in range(NB - 1):
            blk(i)

        @pl.when(r >= 0)
        def _():
            blk(NB - 1)

    def round_(r, c):
        SCOPE('s_a', stage_a, r)
        SCOPE('s_amid', a_mid)
        SCOPE('s_l2', lambda: lax.fori_loop(0, NB, stage_l2, 0))
        epi = attention()
        SCOPE('s_bout', stage_bout, r, epi)
        return c
    lax.fori_loop(0, 2, round_, 0)
    for i in range(NB):
        for s in range(NS):
            out_copy(i, s).wait()


@jax.jit
def pallas_interleave_layers__linear_attn_block__mha_block__prompt_kernel(
    A_x: jax.Array,
    A_wqkv: jax.Array,
    A_wo: jax.Array,
    B_x: jax.Array,
    B_wqkv: jax.Array,
    B_wo: jax.Array,
):
    x = A_x.reshape(S, D)
    scratch = [
        pltpu.VMEM((S, D), BF16),
        pltpu.VMEM((8, D, D), BF16),
        pltpu.VMEM((S, D), BF16),
        pltpu.SemaphoreType.DMA((NB + 8,)),
        pltpu.SemaphoreType.DMA((NB * NS,)),
        pltpu.VMEM((S, D), F32),
        pltpu.VMEM((2, SB // 2, D), U32),
        pltpu.VMEM((7, D // 2, D), U32),
        pltpu.VMEM((D // 2, D), U32),
        pltpu.VMEM((NB, D // 2, TB), U32),
        pltpu.VMEM((D, D), F32),
        pltpu.VMEM((D, 128), F32),
        pltpu.VMEM((D // 2, D), U32),
        pltpu.VMEM((NB, H, TB), F32),
        pltpu.VMEM((H, D), jnp.int32),
        pltpu.VMEM((5, 160, 128), jnp.int32),
        pltpu.VMEM((NG, S // 2, 128), jnp.uint32),
        pltpu.VMEM((H, NB, 16, TB), jnp.uint32),
        pltpu.VMEM((NB, D, TB), F32),
        pltpu.VMEM((NB, D, TB), F32),
    ] + [pltpu.VMEM((S, TB), F32) for _ in range(NSB)]
    out = pl.pallas_call(
        _kernel,
        out_shape=jax.ShapeDtypeStruct((S, D), A_x.dtype),
        in_specs=[pl.BlockSpec(memory_space=pl.ANY)] * 5,
        out_specs=pl.BlockSpec(memory_space=pl.ANY),
        scratch_shapes=scratch,
        compiler_params=pltpu.CompilerParams(vmem_limit_bytes=110 * 1024 * 1024),
    )(x, A_wqkv, A_wo, B_wqkv, B_wo)
    return out.reshape(A_x.shape)
```

```python
import math

import jax
import jax.numpy as jnp
from jax import lax
import jax.experimental.pallas as pl
import jax.experimental.pallas.tpu as pltpu

S = 2048
D = 640
H = 32
DH = 20
NG = 8
TB = 512
NB = S // TB
SB = 128
NS = TB // SB
CK = 128
NC = S // CK
QPI = 2
LAG = 2
NSB = 4
GPOS = 2
FORMB = 1
KV = 128
SM = S - KV
STAG = (16, 48, 80, 112)
LN_EPS = 1e-5
QSCALE = (DH ** -0.5) * math.log2(math.e)
KV_ROWS = [(0, 144), (112, 272), (240, 400), (368, 528), (496, 640)]
AQ, AV, BQ, BK, BV, AO, BO, AK = range(8)

F32 = jnp.float32
BF16 = jnp.bfloat16
U32 = jnp.uint32
NN = (((1,), (0,)), ((), ()))
NT = (((1,), (1,)), ((), ()))


def SCOPE(name, f, *args):
    del name
    return f(*args)


def _dot(a, b, dims=NN):
    return lax.dot_general(a, b, dims, preferred_element_type=F32)


def _pk(x):
    return pltpu.bitcast(x, jnp.uint32)


def _up(x):
    return pltpu.bitcast(x, BF16)


def _phi(t):
    return jnp.where(t > 0, t + 1.0, jnp.exp(jnp.minimum(t, 0.0))) + 1e-6


def _layernorm(x):
    m = jnp.mean(x, axis=-1, keepdims=True)
    xc = x - m
    v = jnp.mean(xc * xc, axis=-1, keepdims=True)
    return xc * lax.rsqrt(v + LN_EPS)


def _kernel(x_hbm, awqkv_hbm, awo_hbm, bwqkv_hbm, bwo_hbm, out_hbm,
            xin, wsrc, obuf, sems, osems,
            x_ref, xn_ref, wt, wkt_a,
            pqt_ref, gt_ref, z_ref, mt_ref, r_ref, zmask_ref, kvmask_ref,
            k_ref, qt_ref, vt_ref, ot_ref, qf_ref, kf_ref, kb0, kb1, *s_refs):
    kbufs = (kb0, kb1)

    def rows(i):
        return pl.ds(pl.multiple_of(i * TB, TB), TB)

    def srows(i, s):
        if isinstance(i, int):
            return pl.ds(i * TB + s * SB, SB)
        return pl.ds(pl.multiple_of(i * TB + s * SB, SB), SB)

    def cols(c):
        return pl.ds(c * D, D)

    def cp_x(i):
        lo = 0 if i == 0 else i * TB + SB
        hi = min((i + 1) * TB + SB, S)
        return pltpu.make_async_copy(x_hbm.at[lo:hi, :], xin.at[lo:hi, :], sems.at[i])

    w_srcs = {AQ: awqkv_hbm.at[:, cols(0)], AV: awqkv_hbm.at[:, cols(2)],
              BQ: bwqkv_hbm.at[:, cols(0)], BK: bwqkv_hbm.at[:, cols(1)],
              BV: bwqkv_hbm.at[:, cols(2)], AO: awo_hbm, BO: bwo_hbm,
              AK: awqkv_hbm.at[:, cols(1)]}

    def cp_w(m, src=None):
        src = awo_hbm if src is None else src
        return pltpu.make_async_copy(src, wsrc.at[m], sems.at[NB + m])

    def transpose_w(m):
        wt[m] = _pk(wsrc[m].T)

    def resid(i, s):
        return xin[srows(i, s), :].astype(F32) + x_ref[srows(i, s), :]

    def ln_sub(i, s):
        return _layernorm(resid(i, s)).astype(BF16)

    cp_w(AK, w_srcs[AK]).start()
    x_ref[...] = jnp.zeros(x_ref.shape, F32)
    cp_x(0).start()
    cp_w(AQ, w_srcs[AQ]).start()
    hr2 = lax.broadcasted_iota(jnp.int32, (H, D), 0)
    hc2 = lax.broadcasted_iota(jnp.int32, (H, D), 1) // DH
    zmask_ref[...] = (hr2 == hc2).astype(jnp.int32)
    for j, (r0, r1) in enumerate(KV_ROWS):
        hr = (lax.broadcasted_iota(jnp.int32, (160, 128), 0) + r0) // DH
        hc = (lax.broadcasted_iota(jnp.int32, (160, 128), 1) + j * 128) // DH
        kvmask_ref[j] = (hr == hc).astype(jnp.int32)
    cp_w(AK).wait()
    wkt_a[...] = _pk(wsrc[AK].T)
    s_refs[NSB - 1][...] = jnp.zeros((TB // 128, S, 128), F32)
    s_refs[NSB - 2][:, (NC - LAG) * CK:, :] = jnp.zeros((TB // 128, LAG * CK, 128), F32)
    ot_ref[0:QPI, 56:64, :] = jnp.zeros((QPI, 8, TB), F32)
    cp_x(0).wait()
    xn_ref[0] = _pk(ln_sub(0, 0))
    cp_w(AQ).wait()
    for i in range(1, NB):
        cp_x(i).start()
        for m in (2 * i - 1, 2 * i):
            cp_w(m, w_srcs[m]).start()

    def stage_a(r):
        def body(i, c):
            for i_s in range(1, NB):
                @pl.when((r == 0) & (i == i_s))
                def _():
                    cp_x(i_s).wait()
                    for m in (2 * i_s - 1, 2 * i_s):
                        cp_w(m).wait()

            xns = [_up(xn_ref[i & 1])] + [ln_sub(i, s) for s in range(1, NS)]
            pkts = [_phi(_dot(_up(wkt_a[...]), xn, NT)) for xn in xns]
            transpose_w(jnp.maximum(2 * i - 1, 0))
            transpose_w(2 * i)
            xn_ref[(i + 1) & 1] = _pk(ln_sub(jnp.minimum(i + 1, NB - 1), 0))
            xn0_late = _up(xn_ref[i & 1])
            z_ref[...] = (jnp.where(i > 0, z_ref[...], 0.0)
                          + (pkts[0] + pkts[1]) + (pkts[2] + pkts[3]))
            for s in range(NS):
                if s == GPOS:
                    gt_ref[...] = _dot(
                        jnp.concatenate(pkts, axis=1),
                        jnp.concatenate([xn0_late] + xns[1:], axis=0)
                    ) + jnp.where(i > 0, gt_ref[...], 0.0)
                qt = _dot(_up(wt[AQ]), xns[s], NT)
                pqt_ref[i, :, s * SB:(s + 1) * SB] = _pk(_phi(qt).astype(BF16))
            return c
        lax.fori_loop(0, NB, body, 0)

    def a_mid():
        z = _dot(jnp.ones((8, 128), F32), z_ref[...], NT)[0:1]
        zm = jnp.where(zmask_ref[...] > 0, z, 0.0)
        kvs = []
        for j, (r0, r1) in enumerate(KV_ROWS):
            kvj = _dot(_up(wt[AV, r0 // 2:r1 // 2, :]), gt_ref[j * 128:(j + 1) * 128, :], NT)
            kvs.append(jnp.where(kvmask_ref[j, 0:r1 - r0, :] > 0, kvj, 0.0))
        for j, (r0, r1) in enumerate(KV_ROWS):
            if j < NB:
                r_ref[j] = 1.0 / (_dot(zm, _up(pqt_ref[j])) + 1e-6)
            k0 = (r0 // 128) * 128
            k1 = -(-r1 // 128) * 128
            pads = []
            if r0 > k0:
                pads.append(jnp.zeros((r0 - k0, 128), F32))
            pads.append(kvs[j])
            if k1 > r1:
                pads.append(jnp.zeros((k1 - r1, 128), F32))
            kvj = jnp.concatenate(pads, axis=0)
            mt_ref[:, j * 128:(j + 1) * 128] = _pk(_dot(
                _up(wt[AO, :, k0:k1]), kvj).astype(BF16))

    row8 = lax.broadcasted_iota(jnp.int32, (8, SB), 0)

    def stage_l2(i, c):
        pqns = []
        for s in range(NS):
            pq = _up(pqt_ref[i, :, s * SB:(s + 1) * SB])
            r = r_ref[i, :, s * SB:(s + 1) * SB]
            parts = []
            for a in range(H // 2):
                re = jnp.broadcast_to(r[2 * a:2 * a + 1], (8, SB))
                ro = jnp.broadcast_to(r[2 * a + 1:2 * a + 2], (8, SB))
                parts += [re, re, jnp.where(row8 < 4, re, ro), ro, ro]
            pqns.append((pq.astype(F32) * jnp.concatenate(parts, axis=0)).astype(BF16))
        xns = []
        for s in range(NS):
            y = x_ref[srows(i, s), :] + _dot(_up(mt_ref[...]), pqns[s]).T
            x_ref[srows(i, s), :] = y
            xns.append(_layernorm(xin[srows(i, s), :].astype(F32) + y).astype(BF16))
        for s in range(NS):
            ps = (s + NS - 1) % NS
            kt = _dot(_up(wt[BK]), xns[s], NT)
            qt = _dot(_up(wt[BQ]), xns[s], NT) * QSCALE
            zpad = jnp.zeros((8, SB), F32)
            for g in range(NG):
                kparts = []
                for j in range(4):
                    r0 = (2 * g + j // 2) * 40 + (16 if j % 2 else 0)
                    kparts += [kt[r0:r0 + 24], zpad]
                    if j % 2:
                        qb = [jnp.where(row8 < 4, 0.0, qt[r0:r0 + 8]), qt[r0 + 8:r0 + 24], zpad]
                    else:
                        qb = [qt[r0:r0 + 16], jnp.where(row8 < 4, qt[r0 + 16:r0 + 24], 0.0), zpad]
                    qt_ref[4 * g + j, i, :, s * SB:(s + 1) * SB] = pltpu.bitcast(
                        jnp.concatenate(qb, axis=0).astype(BF16), jnp.uint32)
                kb = jnp.concatenate(kparts, axis=0).T
                k_ref[g, pl.ds(pl.multiple_of((i * TB + ps * SB) // 2, SB // 2), SB // 2), :] = (
                    _pk(kb.astype(BF16)))
                if ps == NS - 1:
                    kf_ref[g] = kb[SB - KV:]
                    if g == 0:
                        for d in range(DH):
                            kbufs[0][d] = jnp.broadcast_to(kb[SB - KV:, d:d + 1], (KV, 128))
            for g in range(NG):
                qf_ref[i * NS + s, g, 0:4 * DH, :] = qt[g * 4 * DH:(g + 1) * 4 * DH]
            vt_ref[i, :, ps * SB:(ps + 1) * SB] = _dot(_up(wt[BV]), xns[s], NT)
        return c

    def attention():
        NQG = NB // QPI
        NP = NG * NQG
        P = 4 * QPI
        NL = TB // 128
        LG = NC + LAG
        sh = NQG.bit_length() - 1
        nv = KV // 8
        units = SM // 16
        bounds = [16 * ((c * units + NC - 1) // NC) for c in range(NC + 1)]
        pieces = [[0] + [x - (bounds[1] - STAG[lt]) for x in bounds[1:]] + [SM]
                  for lt in range(NL)]

        def lanes(lt):
            return slice(lt * 128, (lt + 1) * 128)

        def get_qm(g, j, q, lt):
            parts = []
            if j > 0:
                parts.append(jnp.zeros((32 * j, 128), BF16))
            parts.append(_up(qt_ref[4 * g + j, q, :, lanes(lt)]))
            if j < 3:
                parts.append(jnp.zeros((96 - 32 * j, 128), BF16))
            return jnp.concatenate(parts, axis=0)

        def upd(s, mx):
            cm = jnp.max(s.reshape(s.shape[0] // 8, 8, 128), axis=0)
            return cm if mx is None else jnp.maximum(mx, cm)

        def qk(g, qm, lt, r0, r1, s_ref, mx):
            s = _dot(_up(k_ref[g, r0 // 2:r1 // 2, :]), qm)
            s_ref[lt, r0:r1, :] = s
            return upd(s, mx)

        def build(g, j, d, kb):
            l = 32 * j + (4 if j % 2 else 0) + d
            kb[d] = jnp.broadcast_to(kf_ref[g, :, l:l + 1], (KV, 128))

        def qk_vpu(g, j, q, lt, vi, s_ref, mx, kb, zero):
            s = None
            for d in range(DH):
                t = (kb[d, pl.ds(pl.multiple_of(zero + vi * 8, 8), 8), :]
                     * qf_ref[q * NL + lt, g, pl.ds(j * DH + d, 8, stride=0), :])
                s = t if s is None else s + t
            s_ref[lt, SM + vi * 8:SM + vi * 8 + 8, :] = s
            return upd(s, mx)

        def getv(a, odd, c):
            base = pl.multiple_of(a * 40 + (16 if odd else 0), 8)
            cb, co = (c * CK) // TB, (c * CK) % TB
            v = vt_ref[cb, pl.ds(base, 24), co:co + CK]
            if odd:
                return jnp.concatenate([jnp.where(row8 < 4, 1.0, v[0:8]), v[8:24]], axis=0)
            return jnp.concatenate([v[0:16], jnp.where(row8 >= 4, 1.0, v[16:24])], axis=0)

        def pv(v, lt, c, s_ref, m, acc, zero):
            sc = s_ref[lt, pl.ds(pl.multiple_of(zero + c * CK, CK), CK), :]
            p = jnp.exp2(sc - m).astype(BF16)
            o = _dot(v, p)
            return o if acc is None else o + acc

        def finish(a, q, lt, odd, acc):
            if not odd:
                ot_ref[q, pl.ds(pl.multiple_of(a * 40, 8), 24), lanes(lt)] = (
                    acc * (1.0 / acc[20:21]))
                return
            oo = acc * (1.0 / acc[0:1])
            r0 = pl.multiple_of(a * 40 + 16, 8)
            mid = jnp.where(row8 < 4, ot_ref[q, pl.ds(r0, 8), lanes(lt)], oo[0:8])
            ot_ref[q, pl.ds(r0, 24), lanes(lt)] = jnp.concatenate([mid, oo[8:24]], axis=0)

        def body(t, carry):
            m2, m1, acc2 = carry
            zero = jnp.minimum(t, 0)
            tp = jnp.maximum(t - 1, 0)
            g = lax.shift_right_logical(t, sh)
            gn = lax.shift_right_logical(jnp.minimum(t + 1, NP - 1), sh)
            q0 = (t & (NQG - 1)) * QPI
            g_prev = lax.shift_right_logical(tp, sh)
            q0_prev = (tp & (NQG - 1)) * QPI
            ms = {-2: list(m2), -1: list(m1)}
            accs = {-2: list(acc2)}
            for n in range(P * NC):
                i = n // NC
                c = n % NC
                j, q = i // QPI, q0 + i % QPI
                s_ref = s_refs[i % NSB]
                if c == 0:
                    qms = [get_qm(g, j, q, lt) for lt in range(NL)]
                    mx = [None] * NL
                for lt in range(NL):
                    mx[lt] = qk(g, qms[lt], lt, pieces[lt][c], pieces[lt][c + 1], s_ref, mx[lt])
                for u in range((c * nv * NL) // NC, ((c + 1) * nv * NL) // NC):
                    vi, lt = u // NL, u % NL
                    mx[lt] = qk_vpu(g, j, q, lt, vi, s_ref, mx[lt], kbufs[j % 2], zero)
                nb = (i % QPI) * NC + c
                for d in range((nb * DH) // (QPI * NC), ((nb + 1) * DH) // (QPI * NC)):
                    build(g if j < 3 else gn, (j + 1) % 4, d, kbufs[(j + 1) % 2])
                n2 = n - LG
                i2 = n2 // NC
                c2 = n2 % NC
                j2 = (i2 % P) // QPI
                a2 = 2 * (g_prev if i2 < 0 else g) + j2 // 2
                q2 = (q0_prev if i2 < 0 else q0) + i2 % QPI
                v = getv(a2, j2 % 2, c2)
                acc = accs.setdefault(i2, [None] * NL)
                for lt in range(NL):
                    acc[lt] = pv(v, lt, c2, s_refs[i2 % NSB], ms[i2][lt], acc[lt], zero)
                if c2 == NC - 1:
                    for lt in range(NL):
                        finish(a2, q2, lt, j2 % 2, acc[lt])
                if c == NC - 1:
                    for lt in range(NL):
                        mx[lt] = qk(g, qms[lt], lt, pieces[lt][NC], pieces[lt][NC + 1], s_ref, mx[lt])
                    ms[i] = [jnp.max(mx[lt], axis=0, keepdims=True) for lt in range(NL)]
            return tuple(ms[P - 2]), tuple(ms[P - 1]), tuple(accs[P - 2])

        zr = tuple(jnp.zeros((1, 128), F32) for _ in range(NL))
        ones24 = tuple(jnp.ones((24, 128), F32) for _ in range(NL))
        m2, m1, acc2 = SCOPE('s_attn_loop', lambda: lax.fori_loop(0, NP, body, (zr, zr, ones24)))

        def epilogue():
            for (i2, m, acc, c0) in ((P - 2, m2, list(acc2), NC - LAG), (P - 1, m1, [None] * NL, 0)):
                j2 = i2 // QPI
                a2 = 2 * (NG - 1) + j2 // 2
                q2 = NB - QPI + i2 % QPI
                for c2 in range(c0, NC):
                    v = getv(a2, j2 % 2, c2)
                    for lt in range(NL):
                        acc[lt] = pv(v, lt, c2, s_refs[i2 % NSB], m[lt], acc[lt], 0)
                    if c2 == NC - 1:
                        for lt in range(NL):
                            finish(a2, q2, lt, j2 % 2, acc[lt])
                    yield
        return epilogue()

    def out_copy(i, s):
        k = i * NS + s
        return pltpu.make_async_copy(obuf.at[k * SB:(k + 1) * SB, :],
                                     out_hbm.at[k * SB:(k + 1) * SB, :], osems.at[k])

    def stage_bout(r, epi):
        @pl.when(r == 1)
        def _():
            for i in range(NB):
                for s in range(NS):
                    out_copy(i, s).wait()
        def blk(i):
            for s in range(NS):
                ot = ot_ref[i, :, s * SB:(s + 1) * SB]
                if s < FORMB and i in (0, NB - 1):
                    yy = _dot(_up(wt[BO]), ot).T
                else:
                    yy = _dot(ot.T.astype(BF16), wsrc[BO])
                if i < NB - 1:
                    for _ in range(2):
                        next(epi, None)
                y = x_ref[srows(i, s), :] + yy
                x_ref[srows(i, s), :] = y
                x = xin[srows(i, s), :].astype(F32) + y
                obuf[srows(i, s), :] = x.astype(obuf.dtype)
                out_copy(i, s).start()
                if i == 0 and s == 0:
                    xn_ref[0] = _pk(_layernorm(x).astype(BF16))
        for i in range(NB - 1):
            blk(i)

        @pl.when(r >= 0)
        def _():
            blk(NB - 1)

    def round_(r, c):
        SCOPE('s_a', stage_a, r)
        SCOPE('s_amid', a_mid)
        SCOPE('s_l2', lambda: lax.fori_loop(0, NB, stage_l2, 0))
        epi = attention()
        SCOPE('s_bout', stage_bout, r, epi)
        return c
    lax.fori_loop(0, 2, round_, 0)
    for i in range(NB):
        for s in range(NS):
            out_copy(i, s).wait()


@jax.jit
def pallas_interleave_layers__linear_attn_block__mha_block__prompt_kernel(
    A_x: jax.Array,
    A_wqkv: jax.Array,
    A_wo: jax.Array,
    B_x: jax.Array,
    B_wqkv: jax.Array,
    B_wo: jax.Array,
):
    x = A_x.reshape(S, D)
    scratch = [
        pltpu.VMEM((S, D), BF16),
        pltpu.VMEM((8, D, D), BF16),
        pltpu.VMEM((S, D), BF16),
        pltpu.SemaphoreType.DMA((NB + 8,)),
        pltpu.SemaphoreType.DMA((NB * NS,)),
        pltpu.VMEM((S, D), F32),
        pltpu.VMEM((2, SB // 2, D), U32),
        pltpu.VMEM((7, D // 2, D), U32),
        pltpu.VMEM((D // 2, D), U32),
        pltpu.VMEM((NB, D // 2, TB), U32),
        pltpu.VMEM((D, D), F32),
        pltpu.VMEM((D, 128), F32),
        pltpu.VMEM((D // 2, D), U32),
        pltpu.VMEM((NB, H, TB), F32),
        pltpu.VMEM((H, D), jnp.int32),
        pltpu.VMEM((5, 160, 128), jnp.int32),
        pltpu.VMEM((NG, S // 2, 128), jnp.uint32),
        pltpu.VMEM((H, NB, 16, TB), jnp.uint32),
        pltpu.VMEM((NB, D, TB), F32),
        pltpu.VMEM((NB, D, TB), F32),
        pltpu.VMEM((S // 128, NG, 96, 128), F32),
        pltpu.VMEM((NG, KV, 128), F32),
        pltpu.VMEM((DH, KV, 128), F32),
        pltpu.VMEM((DH, KV, 128), F32),
    ] + [pltpu.VMEM((TB // 128, S, 128), F32) for _ in range(NSB)]
    out = pl.pallas_call(
        _kernel,
        out_shape=jax.ShapeDtypeStruct((S, D), A_x.dtype),
        in_specs=[pl.BlockSpec(memory_space=pl.ANY)] * 5,
        out_specs=pl.BlockSpec(memory_space=pl.ANY),
        scratch_shapes=scratch,
        compiler_params=pltpu.CompilerParams(vmem_limit_bytes=110 * 1024 * 1024),
    )(x, A_wqkv, A_wo, B_wqkv, B_wo)
    return out.reshape(A_x.shape)
```

```python
import math

import jax
import jax.numpy as jnp
from jax import lax
import jax.experimental.pallas as pl
import jax.experimental.pallas.tpu as pltpu

S = 2048
D = 640
H = 32
DH = 20
NG = 8
TB = 512
NB = S // TB
SB = 128
NS = TB // SB
CK = 128
NC = S // CK
QPI = 2
LAG = 2
NSB = 4
GPOS = 2
FORMB = 1
KV = 128
SM = S - KV
STAG = (16, 48, 80, 112)
NSPLIT = 1
LN_EPS = 1e-5
QSCALE = (DH ** -0.5) * math.log2(math.e)
KV_ROWS = [(0, 144), (112, 272), (240, 400), (368, 528), (496, 640)]
AQ, AV, BQ, BK, BV, AO, BO, AK = range(8)

F32 = jnp.float32
BF16 = jnp.bfloat16
U32 = jnp.uint32
NN = (((1,), (0,)), ((), ()))
NT = (((1,), (1,)), ((), ()))


def SCOPE(name, f, *args):
    del name
    return f(*args)


def _dot(a, b, dims=NN):
    return lax.dot_general(a, b, dims, preferred_element_type=F32)


def _pk(x):
    return pltpu.bitcast(x, jnp.uint32)


def _up(x):
    return pltpu.bitcast(x, BF16)


def _phi(t):
    return jnp.where(t > 0, t + 1.0, jnp.exp(jnp.minimum(t, 0.0))) + 1e-6


def _layernorm(x):
    m = jnp.mean(x, axis=-1, keepdims=True)
    xc = x - m
    v = jnp.mean(xc * xc, axis=-1, keepdims=True)
    return xc * lax.rsqrt(v + LN_EPS)


def _kernel(x_hbm, awqkv_hbm, awo_hbm, bwqkv_hbm, bwo_hbm, out_hbm,
            xin, wsrc, obuf, sems, osems,
            x_ref, xn_ref, wt, wkt_a,
            pqt_ref, gt_ref, z_ref, mt_ref, r_ref, zmask_ref, kvmask_ref,
            k_ref, qt_ref, vt_ref, ot_ref, qf_ref, kf_ref, kb0, kb1, *s_refs):
    kbufs = (kb0, kb1)

    def rows(i):
        return pl.ds(pl.multiple_of(i * TB, TB), TB)

    def srows(i, s):
        if isinstance(i, int):
            return pl.ds(i * TB + s * SB, SB)
        return pl.ds(pl.multiple_of(i * TB + s * SB, SB), SB)

    def cols(c):
        return pl.ds(c * D, D)

    def cp_x(i):
        lo = 0 if i == 0 else i * TB + SB
        hi = min((i + 1) * TB + SB, S)
        return pltpu.make_async_copy(x_hbm.at[lo:hi, :], xin.at[lo:hi, :], sems.at[i])

    w_srcs = {AQ: awqkv_hbm.at[:, cols(0)], AV: awqkv_hbm.at[:, cols(2)],
              BQ: bwqkv_hbm.at[:, cols(0)], BK: bwqkv_hbm.at[:, cols(1)],
              BV: bwqkv_hbm.at[:, cols(2)], AO: awo_hbm, BO: bwo_hbm,
              AK: awqkv_hbm.at[:, cols(1)]}

    def cp_w(m, src=None):
        src = awo_hbm if src is None else src
        return pltpu.make_async_copy(src, wsrc.at[m], sems.at[NB + m])

    def transpose_w(m):
        wt[m] = _pk(wsrc[m].T)

    def resid(i, s):
        return xin[srows(i, s), :].astype(F32) + x_ref[srows(i, s), :]

    def ln_sub(i, s):
        return _layernorm(resid(i, s)).astype(BF16)

    cp_w(AK, w_srcs[AK]).start()
    x_ref[...] = jnp.zeros(x_ref.shape, F32)
    cp_x(0).start()
    cp_w(AQ, w_srcs[AQ]).start()
    hr2 = lax.broadcasted_iota(jnp.int32, (H, D), 0)
    hc2 = lax.broadcasted_iota(jnp.int32, (H, D), 1) // DH
    zmask_ref[...] = (hr2 == hc2).astype(jnp.int32)
    for j, (r0, r1) in enumerate(KV_ROWS):
        hr = (lax.broadcasted_iota(jnp.int32, (160, 128), 0) + r0) // DH
        hc = (lax.broadcasted_iota(jnp.int32, (160, 128), 1) + j * 128) // DH
        kvmask_ref[j] = (hr == hc).astype(jnp.int32)
    cp_w(AK).wait()
    wkt_a[...] = _pk(wsrc[AK].T)
    s_refs[NSB - 1][...] = jnp.zeros((TB // 128, S, 128), F32)
    s_refs[NSB - 2][:, (NC - LAG) * CK:, :] = jnp.zeros((TB // 128, LAG * CK, 128), F32)
    ot_ref[0:QPI, 56:64, :] = jnp.zeros((QPI, 8, TB), F32)
    cp_x(0).wait()
    xn_ref[0] = _pk(ln_sub(0, 0))
    cp_w(AQ).wait()
    for i in range(1, NB):
        cp_x(i).start()
        for m in (2 * i - 1, 2 * i):
            cp_w(m, w_srcs[m]).start()

    def stage_a(r):
        def body(i, c):
            for i_s in range(1, NB):
                @pl.when((r == 0) & (i == i_s))
                def _():
                    cp_x(i_s).wait()
                    for m in (2 * i_s - 1, 2 * i_s):
                        cp_w(m).wait()

            xns = [_up(xn_ref[i & 1])] + [ln_sub(i, s) for s in range(1, NS)]
            pkts = [_phi(_dot(_up(wkt_a[...]), xn, NT)) for xn in xns]
            transpose_w(jnp.maximum(2 * i - 1, 0))
            transpose_w(2 * i)
            xn_ref[(i + 1) & 1] = _pk(ln_sub(jnp.minimum(i + 1, NB - 1), 0))
            xn0_late = _up(xn_ref[i & 1])
            z_ref[...] = (jnp.where(i > 0, z_ref[...], 0.0)
                          + (pkts[0] + pkts[1]) + (pkts[2] + pkts[3]))
            for s in range(NS):
                if s == GPOS:
                    gt_ref[...] = _dot(
                        jnp.concatenate(pkts, axis=1),
                        jnp.concatenate([xn0_late] + xns[1:], axis=0)
                    ) + jnp.where(i > 0, gt_ref[...], 0.0)
                qt = _dot(_up(wt[AQ]), xns[s], NT)
                pqt_ref[i, :, s * SB:(s + 1) * SB] = _pk(_phi(qt).astype(BF16))
            return c
        lax.fori_loop(0, NB, body, 0)

    def a_mid():
        z = _dot(jnp.ones((8, 128), F32), z_ref[...], NT)[0:1]
        zm = jnp.where(zmask_ref[...] > 0, z, 0.0)
        kvs = []
        for j, (r0, r1) in enumerate(KV_ROWS):
            kvj = _dot(_up(wt[AV, r0 // 2:r1 // 2, :]), gt_ref[j * 128:(j + 1) * 128, :], NT)
            kvs.append(jnp.where(kvmask_ref[j, 0:r1 - r0, :] > 0, kvj, 0.0))
        for j, (r0, r1) in enumerate(KV_ROWS):
            if j < NB:
                r_ref[j] = 1.0 / (_dot(zm, _up(pqt_ref[j])) + 1e-6)
            k0 = (r0 // 128) * 128
            k1 = -(-r1 // 128) * 128
            pads = []
            if r0 > k0:
                pads.append(jnp.zeros((r0 - k0, 128), F32))
            pads.append(kvs[j])
            if k1 > r1:
                pads.append(jnp.zeros((k1 - r1, 128), F32))
            kvj = jnp.concatenate(pads, axis=0)
            mt_ref[:, j * 128:(j + 1) * 128] = _pk(_dot(
                _up(wt[AO, :, k0:k1]), kvj).astype(BF16))

    row8 = lax.broadcasted_iota(jnp.int32, (8, SB), 0)

    def stage_l2(i, c):
        pqns = []
        for s in range(NS):
            pq = _up(pqt_ref[i, :, s * SB:(s + 1) * SB])
            r = r_ref[i, :, s * SB:(s + 1) * SB]
            parts = []
            for a in range(H // 2):
                re = jnp.broadcast_to(r[2 * a:2 * a + 1], (8, SB))
                ro = jnp.broadcast_to(r[2 * a + 1:2 * a + 2], (8, SB))
                parts += [re, re, jnp.where(row8 < 4, re, ro), ro, ro]
            pqns.append((pq.astype(F32) * jnp.concatenate(parts, axis=0)).astype(BF16))
        xns = []
        for s in range(NS):
            y = x_ref[srows(i, s), :] + _dot(_up(mt_ref[...]), pqns[s]).T
            x_ref[srows(i, s), :] = y
            xns.append(_layernorm(xin[srows(i, s), :].astype(F32) + y).astype(BF16))
        for s in range(NS):
            ps = (s + NS - 1) % NS
            gw = 4 * DH // 2
            nsp = NSPLIT
            kts, qts, vts = [], [], []
            for sp in range(nsp):
                gs = range(sp * NG // nsp, (sp + 1) * NG // nsp)
                wl = jnp.concatenate(
                    [wt[m, g * gw:(g + 1) * gw, :] for g in gs for m in (BK, BQ, BV)], axis=0)
                res = _dot(_up(wl), xns[s], NT)
                for n_, g in enumerate(gs):
                    o = n_ * 3 * 4 * DH
                    kts.append(res[o:o + 4 * DH])
                    qts.append(res[o + 4 * DH:o + 8 * DH])
                    vts.append(res[o + 8 * DH:o + 12 * DH])
            kt = jnp.concatenate(kts, axis=0)
            qt = jnp.concatenate(qts, axis=0) * QSCALE
            zpad = jnp.zeros((8, SB), F32)
            for g in range(NG):
                kparts = []
                for j in range(4):
                    r0 = (2 * g + j // 2) * 40 + (16 if j % 2 else 0)
                    kparts += [kt[r0:r0 + 24], zpad]
                    if j % 2:
                        qb = [jnp.where(row8 < 4, 0.0, qt[r0:r0 + 8]), qt[r0 + 8:r0 + 24], zpad]
                    else:
                        qb = [qt[r0:r0 + 16], jnp.where(row8 < 4, qt[r0 + 16:r0 + 24], 0.0), zpad]
                    qt_ref[4 * g + j, i, :, s * SB:(s + 1) * SB] = pltpu.bitcast(
                        jnp.concatenate(qb, axis=0).astype(BF16), jnp.uint32)
                kb = jnp.concatenate(kparts, axis=0).T
                k_ref[g, pl.ds(pl.multiple_of((i * TB + ps * SB) // 2, SB // 2), SB // 2), :] = (
                    _pk(kb.astype(BF16)))
                if ps == NS - 1:
                    kf_ref[g] = kb[SB - KV:]
                    if g == 0:
                        for d in range(DH):
                            kbufs[0][d] = jnp.broadcast_to(kb[SB - KV:, d:d + 1], (KV, 128))
            for g in range(NG):
                for r in range(4 * DH):
                    rr = g * 4 * DH + r
                    qf_ref[i * NS + s, g, r] = jnp.broadcast_to(qt[rr:rr + 1], (8, SB))
            vt_ref[i, :, ps * SB:(ps + 1) * SB] = jnp.concatenate(vts, axis=0)
        return c

    def attention():
        NQG = NB // QPI
        NP = NG * NQG
        P = 4 * QPI
        NL = TB // 128
        LG = NC + LAG
        sh = NQG.bit_length() - 1
        nv = KV // 8
        units = SM // 16
        bounds = [16 * ((c * units + NC - 1) // NC) for c in range(NC + 1)]
        pieces = [[0] + [x - (bounds[1] - STAG[lt]) for x in bounds[1:]] + [SM]
                  for lt in range(NL)]

        def lanes(lt):
            return slice(lt * 128, (lt + 1) * 128)

        def get_qm(g, j, q, lt):
            parts = []
            if j > 0:
                parts.append(jnp.zeros((32 * j, 128), BF16))
            parts.append(_up(qt_ref[4 * g + j, q, :, lanes(lt)]))
            if j < 3:
                parts.append(jnp.zeros((96 - 32 * j, 128), BF16))
            return jnp.concatenate(parts, axis=0)

        def upd(s, mx):
            cm = jnp.max(s.reshape(s.shape[0] // 8, 8, 128), axis=0)
            return cm if mx is None else jnp.maximum(mx, cm)

        def qk(g, qm, lt, r0, r1, s_ref, mx):
            s = _dot(_up(k_ref[g, r0 // 2:r1 // 2, :]), qm)
            s_ref[lt, r0:r1, :] = s
            return upd(s, mx)

        def build(g, j, d, kb):
            l = 32 * j + (4 if j % 2 else 0) + d
            kb[d] = jnp.broadcast_to(kf_ref[g, :, l:l + 1], (KV, 128))

        def qk_vpu(g, j, q, lt, vi, s_ref, mx, kb, zero):
            s = None
            for d in range(DH):
                t = (kb[d, pl.ds(pl.multiple_of(zero + vi * 8, 8), 8), :]
                     * qf_ref[q * NL + lt, g, j * DH + d])
                s = t if s is None else s + t
            s_ref[lt, SM + vi * 8:SM + vi * 8 + 8, :] = s
            return upd(s, mx)

        def getv(a, odd, c):
            base = pl.multiple_of(a * 40 + (16 if odd else 0), 8)
            cb, co = (c * CK) // TB, (c * CK) % TB
            v = vt_ref[cb, pl.ds(base, 24), co:co + CK]
            if odd:
                return jnp.concatenate([jnp.where(row8 < 4, 1.0, v[0:8]), v[8:24]], axis=0)
            return jnp.concatenate([v[0:16], jnp.where(row8 >= 4, 1.0, v[16:24])], axis=0)

        def pv(v, lt, c, s_ref, m, acc, zero):
            sc = s_ref[lt, pl.ds(pl.multiple_of(zero + c * CK, CK), CK), :]
            p = jnp.exp2(sc - m).astype(BF16)
            o = _dot(v, p)
            return o if acc is None else o + acc

        def finish(a, q, lt, odd, acc):
            if not odd:
                ot_ref[q, pl.ds(pl.multiple_of(a * 40, 8), 24), lanes(lt)] = (
                    acc * (1.0 / acc[20:21]))
                return
            oo = acc * (1.0 / acc[0:1])
            r0 = pl.multiple_of(a * 40 + 16, 8)
            mid = jnp.where(row8 < 4, ot_ref[q, pl.ds(r0, 8), lanes(lt)], oo[0:8])
            ot_ref[q, pl.ds(r0, 24), lanes(lt)] = jnp.concatenate([mid, oo[8:24]], axis=0)

        def body(t, carry):
            m2, m1, acc2 = carry
            zero = jnp.minimum(t, 0)
            tp = jnp.maximum(t - 1, 0)
            g = lax.shift_right_logical(t, sh)
            gn = lax.shift_right_logical(jnp.minimum(t + 1, NP - 1), sh)
            q0 = (t & (NQG - 1)) * QPI
            g_prev = lax.shift_right_logical(tp, sh)
            q0_prev = (tp & (NQG - 1)) * QPI
            ms = {-2: list(m2), -1: list(m1)}
            accs = {-2: list(acc2)}
            for n in range(P * NC):
                i = n // NC
                c = n % NC
                j, q = i // QPI, q0 + i % QPI
                s_ref = s_refs[i % NSB]
                if c == 0:
                    qms = [get_qm(g, j, q, lt) for lt in range(NL)]
                    mx = [None] * NL
                for lt in range(NL):
                    mx[lt] = qk(g, qms[lt], lt, pieces[lt][c], pieces[lt][c + 1], s_ref, mx[lt])
                for u in range((c * nv * NL) // NC, ((c + 1) * nv * NL) // NC):
                    vi, lt = u // NL, u % NL
                    mx[lt] = qk_vpu(g, j, q, lt, vi, s_ref, mx[lt], kbufs[j % 2], zero)
                nb = (i % QPI) * NC + c
                for d in range((nb * DH) // (QPI * NC), ((nb + 1) * DH) // (QPI * NC)):
                    build(g if j < 3 else gn, (j + 1) % 4, d, kbufs[(j + 1) % 2])
                n2 = n - LG
                i2 = n2 // NC
                c2 = n2 % NC
                j2 = (i2 % P) // QPI
                a2 = 2 * (g_prev if i2 < 0 else g) + j2 // 2
                q2 = (q0_prev if i2 < 0 else q0) + i2 % QPI
                v = getv(a2, j2 % 2, c2)
                acc = accs.setdefault(i2, [None] * NL)
                for lt in range(NL):
                    acc[lt] = pv(v, lt, c2, s_refs[i2 % NSB], ms[i2][lt], acc[lt], zero)
                if c2 == NC - 1:
                    for lt in range(NL):
                        finish(a2, q2, lt, j2 % 2, acc[lt])
                if c == NC - 1:
                    for lt in range(NL):
                        mx[lt] = qk(g, qms[lt], lt, pieces[lt][NC], pieces[lt][NC + 1], s_ref, mx[lt])
                    ms[i] = [jnp.max(mx[lt], axis=0, keepdims=True) for lt in range(NL)]
            return tuple(ms[P - 2]), tuple(ms[P - 1]), tuple(accs[P - 2])

        zr = tuple(jnp.zeros((1, 128), F32) for _ in range(NL))
        ones24 = tuple(jnp.ones((24, 128), F32) for _ in range(NL))
        m2, m1, acc2 = SCOPE('s_attn_loop', lambda: lax.fori_loop(0, NP, body, (zr, zr, ones24)))

        def epilogue():
            for (i2, m, acc, c0) in ((P - 2, m2, list(acc2), NC - LAG), (P - 1, m1, [None] * NL, 0)):
                j2 = i2 // QPI
                a2 = 2 * (NG - 1) + j2 // 2
                q2 = NB - QPI + i2 % QPI
                for c2 in range(c0, NC):
                    v = getv(a2, j2 % 2, c2)
                    for lt in range(NL):
                        acc[lt] = pv(v, lt, c2, s_refs[i2 % NSB], m[lt], acc[lt], 0)
                    if c2 == NC - 1:
                        for lt in range(NL):
                            finish(a2, q2, lt, j2 % 2, acc[lt])
                    yield
        return epilogue()

    def out_copy(i, s):
        k = i * NS + s
        return pltpu.make_async_copy(obuf.at[k * SB:(k + 1) * SB, :],
                                     out_hbm.at[k * SB:(k + 1) * SB, :], osems.at[k])

    def stage_bout(r, epi):
        @pl.when(r == 1)
        def _():
            for i in range(NB):
                for s in range(NS):
                    out_copy(i, s).wait()
        def blk(i):
            for s in range(NS):
                ot = ot_ref[i, :, s * SB:(s + 1) * SB]
                if s < FORMB and i in (0, NB - 1):
                    yy = _dot(_up(wt[BO]), ot).T
                else:
                    yy = _dot(ot.T.astype(BF16), wsrc[BO])
                if i < NB - 1:
                    for _ in range(2):
                        next(epi, None)
                y = x_ref[srows(i, s), :] + yy
                x_ref[srows(i, s), :] = y
                x = xin[srows(i, s), :].astype(F32) + y
                obuf[srows(i, s), :] = x.astype(obuf.dtype)
                out_copy(i, s).start()
                if i == 0 and s == 0:
                    xn_ref[0] = _pk(_layernorm(x).astype(BF16))
        for i in range(NB - 1):
            blk(i)

        @pl.when(r >= 0)
        def _():
            blk(NB - 1)

    def round_(r, c):
        SCOPE('s_a', stage_a, r)
        SCOPE('s_amid', a_mid)
        SCOPE('s_l2', lambda: lax.fori_loop(0, NB, stage_l2, 0))
        epi = attention()
        SCOPE('s_bout', stage_bout, r, epi)
        return c
    lax.fori_loop(0, 2, round_, 0)
    for i in range(NB):
        for s in range(NS):
            out_copy(i, s).wait()


@jax.jit
def pallas_interleave_layers__linear_attn_block__mha_block__prompt_kernel(
    A_x: jax.Array,
    A_wqkv: jax.Array,
    A_wo: jax.Array,
    B_x: jax.Array,
    B_wqkv: jax.Array,
    B_wo: jax.Array,
):
    x = A_x.reshape(S, D)
    scratch = [
        pltpu.VMEM((S, D), BF16),
        pltpu.VMEM((8, D, D), BF16),
        pltpu.VMEM((S, D), BF16),
        pltpu.SemaphoreType.DMA((NB + 8,)),
        pltpu.SemaphoreType.DMA((NB * NS,)),
        pltpu.VMEM((S, D), F32),
        pltpu.VMEM((2, SB // 2, D), U32),
        pltpu.VMEM((7, D // 2, D), U32),
        pltpu.VMEM((D // 2, D), U32),
        pltpu.VMEM((NB, D // 2, TB), U32),
        pltpu.VMEM((D, D), F32),
        pltpu.VMEM((D, 128), F32),
        pltpu.VMEM((D // 2, D), U32),
        pltpu.VMEM((NB, H, TB), F32),
        pltpu.VMEM((H, D), jnp.int32),
        pltpu.VMEM((5, 160, 128), jnp.int32),
        pltpu.VMEM((NG, S // 2, 128), jnp.uint32),
        pltpu.VMEM((H, NB, 16, TB), jnp.uint32),
        pltpu.VMEM((NB, D, TB), F32),
        pltpu.VMEM((NB, D, TB), F32),
        pltpu.VMEM((S // 128, NG, 4 * DH, 8, 128), F32),
        pltpu.VMEM((NG, KV, 128), F32),
        pltpu.VMEM((DH, KV, 128), F32),
        pltpu.VMEM((DH, KV, 128), F32),
    ] + [pltpu.VMEM((TB // 128, S, 128), F32) for _ in range(NSB)]
    out = pl.pallas_call(
        _kernel,
        out_shape=jax.ShapeDtypeStruct((S, D), A_x.dtype),
        in_specs=[pl.BlockSpec(memory_space=pl.ANY)] * 5,
        out_specs=pl.BlockSpec(memory_space=pl.ANY),
        scratch_shapes=scratch,
        compiler_params=pltpu.CompilerParams(vmem_limit_bytes=124 * 1024 * 1024),
    )(x, A_wqkv, A_wo, B_wqkv, B_wo)
    return out.reshape(A_x.shape)
```

```python
import math

import jax
import jax.numpy as jnp
from jax import lax
import jax.experimental.pallas as pl
import jax.experimental.pallas.tpu as pltpu

S = 2048
D = 640
H = 32
DH = 20
NG = 8
TB = 512
NB = S // TB
SB = 128
NS = TB // SB
CK = 128
NC = S // CK
QPI = 2
LAG = 2
NSB = 4
GPOS = 2
FORMB = 1
KV = 128
SM = S - KV
STAG = (16, 48, 80, 112)
NSPLIT = 1
PF32 = 0
NST = 16
LN_EPS = 1e-5
QSCALE = (DH ** -0.5) * math.log2(math.e)
KV_ROWS = [(0, 144), (112, 272), (240, 400), (368, 528), (496, 640)]
AQ, AV, BQ, BK, BV, AO, BO, AK = range(8)

F32 = jnp.float32
BF16 = jnp.bfloat16
U32 = jnp.uint32
NN = (((1,), (0,)), ((), ()))
NT = (((1,), (1,)), ((), ()))


def SCOPE(name, f, *args):
    del name
    return f(*args)


def _dot(a, b, dims=NN):
    return lax.dot_general(a, b, dims, preferred_element_type=F32)


def _pk(x):
    return pltpu.bitcast(x, jnp.uint32)


def _up(x):
    return pltpu.bitcast(x, BF16)


def _phi(t):
    return jnp.where(t > 0, t + 1.0, jnp.exp(jnp.minimum(t, 0.0))) + 1e-6


def _layernorm(x):
    m = jnp.mean(x, axis=-1, keepdims=True)
    xc = x - m
    v = jnp.mean(xc * xc, axis=-1, keepdims=True)
    return xc * lax.rsqrt(v + LN_EPS)


def _kernel(x_hbm, awqkv_hbm, awo_hbm, bwqkv_hbm, bwo_hbm, out_hbm,
            xin, wsrc, obuf, sems, osems,
            x_ref, xn_ref, wt, wkt_a,
            pqt_ref, gt_ref, z_ref, mt_ref, r_ref, zmask_ref, kvmask_ref,
            k_ref, qt_ref, vt_ref, ot_ref, qf_ref, kf_ref, kb0, kb1, *s_refs):
    kbufs = (kb0, kb1)

    def rows(i):
        return pl.ds(pl.multiple_of(i * TB, TB), TB)

    def srows(i, s):
        if isinstance(i, int):
            return pl.ds(i * TB + s * SB, SB)
        return pl.ds(pl.multiple_of(i * TB + s * SB, SB), SB)

    def cols(c):
        return pl.ds(c * D, D)

    def cp_x(i):
        lo = 0 if i == 0 else i * TB + SB
        hi = min((i + 1) * TB + SB, S)
        return pltpu.make_async_copy(x_hbm.at[lo:hi, :], xin.at[lo:hi, :], sems.at[i])

    w_srcs = {AQ: awqkv_hbm.at[:, cols(0)], AV: awqkv_hbm.at[:, cols(2)],
              BQ: bwqkv_hbm.at[:, cols(0)], BK: bwqkv_hbm.at[:, cols(1)],
              BV: bwqkv_hbm.at[:, cols(2)], AO: awo_hbm, BO: bwo_hbm,
              AK: awqkv_hbm.at[:, cols(1)]}

    def cp_w(m, src=None):
        src = awo_hbm if src is None else src
        return pltpu.make_async_copy(src, wsrc.at[m], sems.at[NB + m])

    def transpose_w(m):
        wt[m] = _pk(wsrc[m].T)

    def resid(i, s):
        return xin[srows(i, s), :].astype(F32) + x_ref[srows(i, s), :]

    def ln_sub(i, s):
        return _layernorm(resid(i, s)).astype(BF16)

    cp_w(AK, w_srcs[AK]).start()
    x_ref[...] = jnp.zeros(x_ref.shape, F32)
    cp_x(0).start()
    cp_w(AQ, w_srcs[AQ]).start()
    hr2 = lax.broadcasted_iota(jnp.int32, (H, D), 0)
    hc2 = lax.broadcasted_iota(jnp.int32, (H, D), 1) // DH
    zmask_ref[...] = (hr2 == hc2).astype(jnp.int32)
    for j, (r0, r1) in enumerate(KV_ROWS):
        hr = (lax.broadcasted_iota(jnp.int32, (160, 128), 0) + r0) // DH
        hc = (lax.broadcasted_iota(jnp.int32, (160, 128), 1) + j * 128) // DH
        kvmask_ref[j] = (hr == hc).astype(jnp.int32)
    cp_w(AK).wait()
    wkt_a[...] = _pk(wsrc[AK].T)
    s_refs[NSB - 1][...] = jnp.zeros((TB // 128, S, 128), F32)
    s_refs[NSB - 2][:, (NC - LAG) * CK:, :] = jnp.zeros((TB // 128, LAG * CK, 128), F32)
    ot_ref[0:QPI, 56:64, :] = jnp.zeros((QPI, 8, TB), F32)
    cp_x(0).wait()
    xn_ref[0] = _pk(ln_sub(0, 0))
    cp_w(AQ).wait()
    for i in range(1, NB):
        cp_x(i).start()
        for m in (2 * i - 1, 2 * i):
            cp_w(m, w_srcs[m]).start()

    def stage_a(r):
        def body(i, c):
            for i_s in range(1, NB):
                @pl.when((r == 0) & (i == i_s))
                def _():
                    cp_x(i_s).wait()
                    for m in (2 * i_s - 1, 2 * i_s):
                        cp_w(m).wait()

            xns = [_up(xn_ref[i & 1])] + [ln_sub(i, s) for s in range(1, NS)]
            pkts = [_phi(_dot(_up(wkt_a[...]), xn, NT)) for xn in xns]
            transpose_w(jnp.maximum(2 * i - 1, 0))
            transpose_w(2 * i)
            xn_ref[(i + 1) & 1] = _pk(ln_sub(jnp.minimum(i + 1, NB - 1), 0))
            xn0_late = _up(xn_ref[i & 1])
            z_ref[...] = (jnp.where(i > 0, z_ref[...], 0.0)
                          + (pkts[0] + pkts[1]) + (pkts[2] + pkts[3]))
            for s in range(NS):
                if s == GPOS:
                    gt_ref[...] = _dot(
                        jnp.concatenate(pkts, axis=1),
                        jnp.concatenate([xn0_late] + xns[1:], axis=0)
                    ) + jnp.where(i > 0, gt_ref[...], 0.0)
                qt = _dot(_up(wt[AQ]), xns[s], NT)
                pqt_ref[i, :, s * SB:(s + 1) * SB] = _pk(_phi(qt).astype(BF16))
            return c
        lax.fori_loop(0, NB, body, 0)

    def a_mid():
        z = _dot(jnp.ones((8, 128), F32), z_ref[...], NT)[0:1]
        zm = jnp.where(zmask_ref[...] > 0, z, 0.0)
        kvs = []
        for j, (r0, r1) in enumerate(KV_ROWS):
            kvj = _dot(_up(wt[AV, r0 // 2:r1 // 2, :]), gt_ref[j * 128:(j + 1) * 128, :], NT)
            kvs.append(jnp.where(kvmask_ref[j, 0:r1 - r0, :] > 0, kvj, 0.0))
        for j, (r0, r1) in enumerate(KV_ROWS):
            if j < NB:
                r_ref[j] = 1.0 / (_dot(zm, _up(pqt_ref[j])) + 1e-6)
            k0 = (r0 // 128) * 128
            k1 = -(-r1 // 128) * 128
            pads = []
            if r0 > k0:
                pads.append(jnp.zeros((r0 - k0, 128), F32))
            pads.append(kvs[j])
            if k1 > r1:
                pads.append(jnp.zeros((k1 - r1, 128), F32))
            kvj = jnp.concatenate(pads, axis=0)
            mt_ref[:, j * 128:(j + 1) * 128] = _pk(_dot(
                _up(wt[AO, :, k0:k1]), kvj).astype(BF16))

    row8 = lax.broadcasted_iota(jnp.int32, (8, SB), 0)

    def stage_l2(i, c):
        pqns = []
        for s in range(NS):
            pq = _up(pqt_ref[i, :, s * SB:(s + 1) * SB])
            r = r_ref[i, :, s * SB:(s + 1) * SB]
            parts = []
            for a in range(H // 2):
                re = jnp.broadcast_to(r[2 * a:2 * a + 1], (8, SB))
                ro = jnp.broadcast_to(r[2 * a + 1:2 * a + 2], (8, SB))
                parts += [re, re, jnp.where(row8 < 4, re, ro), ro, ro]
            pqns.append((pq.astype(F32) * jnp.concatenate(parts, axis=0)).astype(BF16))
        xns = []
        for s in range(NS):
            y = x_ref[srows(i, s), :] + _dot(_up(mt_ref[...]), pqns[s]).T
            x_ref[srows(i, s), :] = y
            xns.append(_layernorm(xin[srows(i, s), :].astype(F32) + y).astype(BF16))
        for s in range(NS):
            ps = (s + NS - 1) % NS
            gw = 4 * DH // 2
            nsp = NSPLIT
            kts, qts, vts = [], [], []
            for sp in range(nsp):
                gs = range(sp * NG // nsp, (sp + 1) * NG // nsp)
                wl = jnp.concatenate(
                    [wt[m, g * gw:(g + 1) * gw, :] for g in gs for m in (BK, BQ, BV)], axis=0)
                res = _dot(_up(wl), xns[s], NT)
                for n_, g in enumerate(gs):
                    o = n_ * 3 * 4 * DH
                    kts.append(res[o:o + 4 * DH])
                    qts.append(res[o + 4 * DH:o + 8 * DH])
                    vts.append(res[o + 8 * DH:o + 12 * DH])
            kt = jnp.concatenate(kts, axis=0)
            qt = jnp.concatenate(qts, axis=0) * QSCALE
            zpad = jnp.zeros((8, SB), F32)
            for g in range(NG):
                kparts = []
                for j in range(4):
                    r0 = (2 * g + j // 2) * 40 + (16 if j % 2 else 0)
                    kparts += [kt[r0:r0 + 24], zpad]
                    if j % 2:
                        qb = [jnp.where(row8 < 4, 0.0, qt[r0:r0 + 8]), qt[r0 + 8:r0 + 24], zpad]
                    else:
                        qb = [qt[r0:r0 + 16], jnp.where(row8 < 4, qt[r0 + 16:r0 + 24], 0.0), zpad]
                    qt_ref[4 * g + j, i, :, s * SB:(s + 1) * SB] = pltpu.bitcast(
                        jnp.concatenate(qb, axis=0).astype(BF16), jnp.uint32)
                kb = jnp.concatenate(kparts, axis=0).T
                k_ref[g, pl.ds(pl.multiple_of((i * TB + ps * SB) // 2, SB // 2), SB // 2), :] = (
                    _pk(kb.astype(BF16)))
                lo = max(TB - KV, ps * SB)
                hi = (ps + 1) * SB
                if lo < hi:
                    kpart = kb[lo - ps * SB:]
                    o0, o1 = lo - (TB - KV), hi - (TB - KV)
                    kf_ref[g, o0:o1, :] = kpart
                    if g == 0:
                        for d in range(DH):
                            kbufs[0][d, o0:o1, :] = jnp.broadcast_to(
                                kpart[:, d:d + 1], (o1 - o0, 128))
            for g in range(NG):
                for r in range(4 * DH):
                    rr = g * 4 * DH + r
                    qf_ref[i * NS + s, g, r] = jnp.broadcast_to(qt[rr:rr + 1], (8, SB))
            vt_ref[i, :, ps * SB:(ps + 1) * SB] = jnp.concatenate(vts, axis=0)
        return c

    def attention():
        NQG = NB // QPI
        NP = NG * NQG
        P = 4 * QPI
        NL = TB // 128
        LG = NC + LAG
        sh = NQG.bit_length() - 1
        nv = KV // 8
        units = SM // 16
        bounds = [16 * ((c * units + NC - 1) // NC) for c in range(NC + 1)]
        pieces = [[0] + [x - (bounds[1] - STAG[lt]) for x in bounds[1:]] + [SM]
                  for lt in range(NL)]

        def lanes(lt):
            return slice(lt * 128, (lt + 1) * 128)

        def get_qm(g, j, q, lt):
            parts = []
            if j > 0:
                parts.append(jnp.zeros((32 * j, 128), BF16))
            parts.append(_up(qt_ref[4 * g + j, q, :, lanes(lt)]))
            if j < 3:
                parts.append(jnp.zeros((96 - 32 * j, 128), BF16))
            return jnp.concatenate(parts, axis=0)

        def upd(s, mx):
            cm = jnp.max(s.reshape(s.shape[0] // 8, 8, 128), axis=0)
            return cm if mx is None else jnp.maximum(mx, cm)

        def qk(g, qm, lt, r0, r1, s_ref, mx):
            s = _dot(_up(k_ref[g, r0 // 2:r1 // 2, :]), qm)
            s_ref[lt, r0:r1, :] = s
            return upd(s, mx)

        def build(g, j, d, kb):
            l = 32 * j + (4 if j % 2 else 0) + d
            kb[d] = jnp.broadcast_to(kf_ref[g, 0:KV, l:l + 1], (KV, 128))

        def qk_vpu(g, j, q, lt, vi, s_ref, mx, kb, zero):
            s = None
            for d in range(DH):
                t = (kb[d, pl.ds(zero + vi * 8, 8), :]
                     * qf_ref[q * NL + lt, g, j * DH + d])
                s = t if s is None else s + t
            s_ref[lt, SM + vi * 8:SM + vi * 8 + 8, :] = s
            return upd(s, mx)

        def getv(a, odd, c):
            base = pl.multiple_of(a * 40 + (16 if odd else 0), 8)
            cb, co = (c * CK) // TB, (c * CK) % TB
            v = vt_ref[cb, pl.ds(base, 24), co:co + CK]
            if odd:
                return jnp.concatenate([jnp.where(row8 < 4, 1.0, v[0:8]), v[8:24]], axis=0)
            return jnp.concatenate([v[0:16], jnp.where(row8 >= 4, 1.0, v[16:24])], axis=0)

        def pv(v, lt, c, s_ref, m, acc, zero):
            sc = s_ref[lt, pl.ds(zero + c * CK, CK), :]
            p = jnp.exp2(sc - m)
            if not PF32:
                p = p.astype(BF16)
            o = _dot(v, p)
            return o if acc is None else o + acc

        def finish(a, q, lt, odd, acc):
            if not odd:
                ot_ref[q, pl.ds(pl.multiple_of(a * 40, 8), 24), lanes(lt)] = (
                    acc * (1.0 / acc[20:21]))
                return
            oo = acc * (1.0 / acc[0:1])
            r0 = pl.multiple_of(a * 40 + 16, 8)
            mid = jnp.where(row8 < 4, ot_ref[q, pl.ds(r0, 8), lanes(lt)], oo[0:8])
            ot_ref[q, pl.ds(r0, 24), lanes(lt)] = jnp.concatenate([mid, oo[8:24]], axis=0)

        def body(t, carry):
            m2, m1, acc2 = carry
            zero = pl.multiple_of(jnp.minimum(t, 0), 256)
            tp = jnp.maximum(t - 1, 0)
            g = lax.shift_right_logical(t, sh)
            gn = lax.shift_right_logical(jnp.minimum(t + 1, NP - 1), sh)
            q0 = (t & (NQG - 1)) * QPI
            g_prev = lax.shift_right_logical(tp, sh)
            q0_prev = (tp & (NQG - 1)) * QPI
            ms = {-2: list(m2), -1: list(m1)}
            accs = {-2: list(acc2)}
            for n in range(P * NC):
                i = n // NC
                c = n % NC
                j, q = i // QPI, q0 + i % QPI
                s_ref = s_refs[i % NSB]
                if c == 0:
                    qms = [get_qm(g, j, q, lt) for lt in range(NL)]
                    mx = [None] * NL
                for u in range((c * nv * NL) // NST, ((c + 1) * nv * NL) // NST):
                    vi, lt = u // NL, u % NL
                    mx[lt] = qk_vpu(g, j, q, lt, vi, s_ref, mx[lt], kbufs[j % 2], zero)
                for lt in range(NL):
                    mx[lt] = qk(g, qms[lt], lt, pieces[lt][c], pieces[lt][c + 1], s_ref, mx[lt])
                nb = (i % QPI) * NC + c
                for d in range((nb * DH) // (QPI * NC), ((nb + 1) * DH) // (QPI * NC)):
                    build(g if j < 3 else gn, (j + 1) % 4, d, kbufs[(j + 1) % 2])
                n2 = n - LG
                i2 = n2 // NC
                c2 = n2 % NC
                j2 = (i2 % P) // QPI
                a2 = 2 * (g_prev if i2 < 0 else g) + j2 // 2
                q2 = (q0_prev if i2 < 0 else q0) + i2 % QPI
                v = getv(a2, j2 % 2, c2)
                acc = accs.setdefault(i2, [None] * NL)
                for lt in range(NL):
                    acc[lt] = pv(v, lt, c2, s_refs[i2 % NSB], ms[i2][lt], acc[lt], zero)
                if c2 == NC - 1:
                    for lt in range(NL):
                        finish(a2, q2, lt, j2 % 2, acc[lt])
                if c == NC - 1:
                    for u in range((NC * nv * NL) // NST, nv * NL):
                        vi, lt = u // NL, u % NL
                        mx[lt] = qk_vpu(g, j, q, lt, vi, s_ref, mx[lt], kbufs[j % 2], zero)
                    for lt in range(NL):
                        mx[lt] = qk(g, qms[lt], lt, pieces[lt][NC], pieces[lt][NC + 1], s_ref, mx[lt])
                    ms[i] = [jnp.max(mx[lt], axis=0, keepdims=True) for lt in range(NL)]
            return tuple(ms[P - 2]), tuple(ms[P - 1]), tuple(accs[P - 2])

        zr = tuple(jnp.zeros((1, 128), F32) for _ in range(NL))
        ones24 = tuple(jnp.ones((24, 128), F32) for _ in range(NL))
        m2, m1, acc2 = SCOPE('s_attn_loop', lambda: lax.fori_loop(0, NP, body, (zr, zr, ones24)))

        def epilogue():
            for (i2, m, acc, c0) in ((P - 2, m2, list(acc2), NC - LAG), (P - 1, m1, [None] * NL, 0)):
                j2 = i2 // QPI
                a2 = 2 * (NG - 1) + j2 // 2
                q2 = NB - QPI + i2 % QPI
                for c2 in range(c0, NC):
                    v = getv(a2, j2 % 2, c2)
                    for lt in range(NL):
                        acc[lt] = pv(v, lt, c2, s_refs[i2 % NSB], m[lt], acc[lt], 0)
                    if c2 == NC - 1:
                        for lt in range(NL):
                            finish(a2, q2, lt, j2 % 2, acc[lt])
                    yield
        return epilogue()

    def out_copy(i, s):
        k = i * NS + s
        return pltpu.make_async_copy(obuf.at[k * SB:(k + 1) * SB, :],
                                     out_hbm.at[k * SB:(k + 1) * SB, :], osems.at[k])

    def stage_bout(r, epi):
        @pl.when(r == 1)
        def _():
            for i in range(NB):
                for s in range(NS):
                    out_copy(i, s).wait()
        def blk(i):
            for s in range(NS):
                ot = ot_ref[i, :, s * SB:(s + 1) * SB]
                if s < FORMB and i in (0, NB - 1):
                    yy = _dot(_up(wt[BO]), ot).T
                else:
                    yy = _dot(ot.T.astype(BF16), wsrc[BO])
                if i < NB - 1:
                    for _ in range(2):
                        next(epi, None)
                y = x_ref[srows(i, s), :] + yy
                x_ref[srows(i, s), :] = y
                x = xin[srows(i, s), :].astype(F32) + y
                obuf[srows(i, s), :] = x.astype(obuf.dtype)
                out_copy(i, s).start()
                if i == 0 and s == 0:
                    xn_ref[0] = _pk(_layernorm(x).astype(BF16))
        for i in range(NB - 1):
            blk(i)

        @pl.when(r >= 0)
        def _():
            blk(NB - 1)

    def round_(r, c):
        SCOPE('s_a', stage_a, r)
        SCOPE('s_amid', a_mid)
        SCOPE('s_l2', lambda: lax.fori_loop(0, NB, stage_l2, 0))
        epi = attention()
        SCOPE('s_bout', stage_bout, r, epi)
        return c
    lax.fori_loop(0, 2, round_, 0)
    for i in range(NB):
        for s in range(NS):
            out_copy(i, s).wait()


@jax.jit
def pallas_interleave_layers__linear_attn_block__mha_block__prompt_kernel(
    A_x: jax.Array,
    A_wqkv: jax.Array,
    A_wo: jax.Array,
    B_x: jax.Array,
    B_wqkv: jax.Array,
    B_wo: jax.Array,
):
    x = A_x.reshape(S, D)
    scratch = [
        pltpu.VMEM((S, D), BF16),
        pltpu.VMEM((8, D, D), BF16),
        pltpu.VMEM((S, D), BF16),
        pltpu.SemaphoreType.DMA((NB + 8,)),
        pltpu.SemaphoreType.DMA((NB * NS,)),
        pltpu.VMEM((S, D), F32),
        pltpu.VMEM((2, SB // 2, D), U32),
        pltpu.VMEM((7, D // 2, D), U32),
        pltpu.VMEM((D // 2, D), U32),
        pltpu.VMEM((NB, D // 2, TB), U32),
        pltpu.VMEM((D, D), F32),
        pltpu.VMEM((D, 128), F32),
        pltpu.VMEM((D // 2, D), U32),
        pltpu.VMEM((NB, H, TB), F32),
        pltpu.VMEM((H, D), jnp.int32),
        pltpu.VMEM((5, 160, 128), jnp.int32),
        pltpu.VMEM((NG, S // 2, 128), jnp.uint32),
        pltpu.VMEM((H, NB, 16, TB), jnp.uint32),
        pltpu.VMEM((NB, D, TB), F32),
        pltpu.VMEM((NB, D, TB), F32),
        pltpu.VMEM((S // 128, NG, 4 * DH, 8, 128), F32),
        pltpu.VMEM((NG, 256, 128), F32),
        pltpu.VMEM((DH, KV, 128), F32),
        pltpu.VMEM((DH, KV, 128), F32),
    ] + [pltpu.VMEM((TB // 128, S, 128), F32) for _ in range(NSB)]
    out = pl.pallas_call(
        _kernel,
        out_shape=jax.ShapeDtypeStruct((S, D), A_x.dtype),
        in_specs=[pl.BlockSpec(memory_space=pl.ANY)] * 5,
        out_specs=pl.BlockSpec(memory_space=pl.ANY),
        scratch_shapes=scratch,
        compiler_params=pltpu.CompilerParams(vmem_limit_bytes=124 * 1024 * 1024),
    )(x, A_wqkv, A_wo, B_wqkv, B_wo)
    return out.reshape(A_x.shape)
```

```python
import math

import jax
import jax.numpy as jnp
from jax import lax
import jax.experimental.pallas as pl
import jax.experimental.pallas.tpu as pltpu

S = 2048
D = 640
H = 32
DH = 20
NG = 8
GD = 4 * DH
TB = 512
NB = S // TB
SB = 128
NS = TB // SB
NL = TB // 128
CK = 128
NC = S // CK
QPI = 2
LAG = 2
NSB = 4
KV = 128
SM = S - KV
STAG = (16, 48, 80, 112)
DG = 5
LN_EPS = 1e-5
QSCALE = (DH ** -0.5) * math.log2(math.e)
KV_ROWS = [(0, 144), (112, 272), (240, 400), (368, 528), (496, 640)]
AQ, AV, BQ, BK, BV, AO, BO, AK = range(8)

F32 = jnp.float32
BF16 = jnp.bfloat16
U32 = jnp.uint32
NN = (((1,), (0,)), ((), ()))
NT = (((1,), (1,)), ((), ()))


def SCOPE(name, f, *args):
    del name
    return f(*args)


def _dot(a, b, dims=NN):
    return lax.dot_general(a, b, dims, preferred_element_type=F32)


def _pk(x):
    return pltpu.bitcast(x, U32)


def _up(x):
    return pltpu.bitcast(x, BF16)


def _phi(t):
    return jnp.where(t > 0, t + 1.0, jnp.exp(jnp.minimum(t, 0.0))) + 1e-6


def _layernorm(x):
    m = jnp.mean(x, axis=-1, keepdims=True)
    xc = x - m
    v = jnp.mean(xc * xc, axis=-1, keepdims=True)
    return xc * lax.rsqrt(v + LN_EPS)


def _lanes(k):
    return slice(k * 128, (k + 1) * 128)


def _kernel(x_hbm, awqkv_hbm, awo_hbm, bwqkv_hbm, bwo_hbm, out_hbm,
            xin, wsrc, obuf, sems, osems,
            x_ref, xn_ref, wt, wkt_a,
            pqt_ref, gt_ref, z_ref, mt_ref, r_ref, zmask_ref, kvmask_ref,
            k_ref, qt_ref, vt_ref, ot_ref, qb_ref, kf_ref, kb0, kb1, *s_refs):
    kbufs = (kb0, kb1)
    row8 = lax.broadcasted_iota(jnp.int32, (8, 128), 0)

    def srows(i, s):
        if isinstance(i, int):
            return pl.ds(i * TB + s * SB, SB)
        return pl.ds(pl.multiple_of(i * TB + s * SB, SB), SB)

    def cp_x(i):
        lo = 0 if i == 0 else i * TB + SB
        hi = min((i + 1) * TB + SB, S)
        return pltpu.make_async_copy(x_hbm.at[lo:hi, :], xin.at[lo:hi, :], sems.at[i])

    w_srcs = {AQ: awqkv_hbm.at[:, 0:D], AK: awqkv_hbm.at[:, D:2 * D],
              AV: awqkv_hbm.at[:, 2 * D:3 * D], AO: awo_hbm,
              BQ: bwqkv_hbm.at[:, 0:D], BK: bwqkv_hbm.at[:, D:2 * D],
              BV: bwqkv_hbm.at[:, 2 * D:3 * D], BO: bwo_hbm}

    def cp_w(m):
        return pltpu.make_async_copy(w_srcs[m], wsrc.at[m], sems.at[NB + m])

    def ln_sub(i, s):
        x = xin[srows(i, s), :].astype(F32) + x_ref[srows(i, s), :]
        return _layernorm(x).astype(BF16)

    cp_w(AK).start()
    x_ref[...] = jnp.zeros(x_ref.shape, F32)
    cp_x(0).start()
    cp_w(AQ).start()
    hr2 = lax.broadcasted_iota(jnp.int32, (H, D), 0)
    hc2 = lax.broadcasted_iota(jnp.int32, (H, D), 1) // DH
    zmask_ref[...] = (hr2 == hc2).astype(jnp.int32)
    for j, (r0, r1) in enumerate(KV_ROWS):
        hr = (lax.broadcasted_iota(jnp.int32, (160, 128), 0) + r0) // DH
        hc = (lax.broadcasted_iota(jnp.int32, (160, 128), 1) + j * 128) // DH
        kvmask_ref[j] = (hr == hc).astype(jnp.int32)
    cp_w(AK).wait()
    wkt_a[...] = _pk(wsrc[AK].T)
    gt_ref[...] = jnp.zeros(gt_ref.shape, F32)
    z_ref[...] = jnp.zeros(z_ref.shape, F32)
    s_refs[NSB - 1][...] = jnp.zeros((NL, S, 128), F32)
    s_refs[NSB - 2][:, (NC - LAG) * CK:, :] = jnp.zeros((NL, LAG * CK, 128), F32)
    ot_ref[0:QPI, 56:64, :] = jnp.zeros((QPI, 8, TB), F32)
    cp_x(0).wait()
    xn_ref[0] = _pk(ln_sub(0, 0))
    cp_w(AQ).wait()
    for i in range(1, NB):
        cp_x(i).start()
        cp_w(2 * i - 1).start()
        cp_w(2 * i).start()

    def stage_a(r):
        def body(i, c):
            for i_s in range(1, NB):
                @pl.when((r == 0) & (i == i_s))
                def _():
                    cp_x(i_s).wait()
                    cp_w(2 * i_s - 1).wait()
                    cp_w(2 * i_s).wait()

            xns = [_up(xn_ref[i & 1])] + [ln_sub(i, s) for s in range(1, NS)]
            pkts = [_phi(_dot(_up(wkt_a[...]), xn, NT)) for xn in xns]
            for m in (jnp.maximum(2 * i - 1, 0), 2 * i):
                wt[m] = _pk(wsrc[m].T)
            xn_ref[(i + 1) & 1] = _pk(ln_sub(jnp.minimum(i + 1, NB - 1), 0))
            xn0_late = _up(xn_ref[i & 1])
            z_ref[...] = (jnp.where(i > 0, z_ref[...], 0.0)
                          + (pkts[0] + pkts[1]) + (pkts[2] + pkts[3]))
            for s in range(NS):
                if s == NS // 2:
                    gt_ref[...] = _dot(
                        jnp.concatenate(pkts, axis=1),
                        jnp.concatenate([xn0_late] + xns[1:], axis=0)
                    ) + jnp.where(i > 0, gt_ref[...], 0.0)
                qt = _dot(_up(wt[AQ]), xns[s], NT)
                pqt_ref[i, :, _lanes(s)] = _pk(_phi(qt).astype(BF16))
            return c
        lax.fori_loop(0, NB, body, 0)

    def a_mid():
        z = _dot(jnp.ones((8, 128), F32), z_ref[...], NT)[0:1]
        zm = jnp.where(zmask_ref[...] > 0, z, 0.0)
        kvs = []
        for j, (r0, r1) in enumerate(KV_ROWS):
            kvj = _dot(_up(wt[AV, r0 // 2:r1 // 2, :]), gt_ref[_lanes(j), :], NT)
            kvs.append(jnp.where(kvmask_ref[j, 0:r1 - r0, :] > 0, kvj, 0.0))
        for j, (r0, r1) in enumerate(KV_ROWS):
            if j < NB:
                r_ref[j] = 1.0 / (_dot(zm, _up(pqt_ref[j])) + 1e-6)
            k0 = (r0 // 128) * 128
            k1 = -(-r1 // 128) * 128
            pads = []
            if r0 > k0:
                pads.append(jnp.zeros((r0 - k0, 128), F32))
            pads.append(kvs[j])
            if k1 > r1:
                pads.append(jnp.zeros((k1 - r1, 128), F32))
            kvj = jnp.concatenate(pads, axis=0)
            mt_ref[:, _lanes(j)] = _pk(_dot(_up(wt[AO, :, k0:k1]), kvj).astype(BF16))

    def stage_l2(i, c):
        pqns = []
        for s in range(NS):
            pq = _up(pqt_ref[i, :, _lanes(s)])
            r = r_ref[i, :, _lanes(s)]
            parts = []
            for a in range(H // 2):
                re = jnp.broadcast_to(r[2 * a:2 * a + 1], (8, SB))
                ro = jnp.broadcast_to(r[2 * a + 1:2 * a + 2], (8, SB))
                parts += [re, re, jnp.where(row8 < 4, re, ro), ro, ro]
            pqns.append((pq.astype(F32) * jnp.concatenate(parts, axis=0)).astype(BF16))
        xns = []
        for s in range(NS):
            y = x_ref[srows(i, s), :] + _dot(_up(mt_ref[...]), pqns[s]).T
            x_ref[srows(i, s), :] = y
            xns.append(_layernorm(xin[srows(i, s), :].astype(F32) + y).astype(BF16))
        zpad = jnp.zeros((8, SB), F32)
        for s in range(NS):
            ps = (s + NS - 1) % NS
            wl = jnp.concatenate(
                [wt[m, g * GD // 2:(g + 1) * GD // 2, :]
                 for g in range(NG) for m in (BK, BQ, BV)], axis=0)
            res = _dot(_up(wl), xns[s], NT)
            krow0 = pl.ds(pl.multiple_of((i * TB + ps * SB) // 2, SB // 2), SB // 2)
            for g in range(NG):
                kt = res[3 * g * GD:(3 * g + 1) * GD]
                qt = res[(3 * g + 1) * GD:(3 * g + 2) * GD] * QSCALE
                vt_ref[i, g * GD:(g + 1) * GD, _lanes(ps)] = res[(3 * g + 2) * GD:(3 * g + 3) * GD]
                kparts = []
                for j in range(4):
                    r0 = (j // 2) * 40 + (16 if j % 2 else 0)
                    kparts += [kt[r0:r0 + 24], zpad]
                    if j % 2:
                        qw = [jnp.where(row8 < 4, 0.0, qt[r0:r0 + 8]), qt[r0 + 8:r0 + 24], zpad]
                    else:
                        qw = [qt[r0:r0 + 16], jnp.where(row8 < 4, qt[r0 + 16:r0 + 24], 0.0), zpad]
                    qt_ref[4 * g + j, i, :, _lanes(s)] = _pk(
                        jnp.concatenate(qw, axis=0).astype(BF16))
                kb = jnp.concatenate(kparts, axis=0).T
                k_ref[g, krow0, :] = _pk(kb.astype(BF16))
                if ps == NS - 1:
                    kf_ref[g] = kb
                    if g == 0:
                        for d in range(DH):
                            kbufs[0][d] = jnp.broadcast_to(kb[:, d:d + 1], (KV, 128))
                qb_ref[i * NS + s, g] = jnp.broadcast_to(qt.reshape(GD, 1, SB), (GD, 8, SB))
        return c

    def attention():
        NQG = NB // QPI
        NP = NG * NQG
        P = 4 * QPI
        LG = NC + LAG
        sh = NQG.bit_length() - 1
        units = SM // 16
        bounds = [16 * ((c * units + NC - 1) // NC) for c in range(NC + 1)]
        pieces = [[0] + [x - (bounds[1] - STAG[lt]) for x in bounds[1:]] + [SM]
                  for lt in range(NL)]

        def get_qm(h, j, q, lt):
            parts = []
            if j > 0:
                parts.append(jnp.zeros((32 * j, 128), BF16))
            parts.append(_up(qt_ref[h, q, :, _lanes(lt)]))
            if j < 3:
                parts.append(jnp.zeros((96 - 32 * j, 128), BF16))
            return jnp.concatenate(parts, axis=0)

        def qk(g, qm, lt, r0, r1, s_ref, mx):
            s = _dot(_up(k_ref[g, r0 // 2:r1 // 2, :]), qm)
            s_ref[lt, r0:r1, :] = s
            return jnp.maximum(mx, jnp.max(s.reshape((r1 - r0) // 8, 8, 128), axis=0))

        def build(g, j, d, kb):
            l = 32 * j + (4 if j % 2 else 0) + d
            kb[d] = jnp.broadcast_to(kf_ref[g, :, l:l + 1], (KV, 128))

        def qk_vpu(kbs, g, j, ql, lt, vi, s_ref, mx):
            s = None
            for n, d in enumerate(range(0, DH, DG)):
                t = kbs[n] * qb_ref[ql, g, j * DH + d:j * DH + d + DG]
                if s is not None:
                    t = jnp.concatenate([s[None], t], axis=0)
                s = jnp.sum(t, axis=0)
            s_ref[lt, SM + vi * 8:SM + vi * 8 + 8, :] = s
            return s if mx is None else jnp.maximum(mx, s)

        def getv(base, odd, c):
            cb, co = (c * CK) // TB, (c * CK) % TB
            v = vt_ref[cb, pl.ds(base, 24), co:co + CK]
            if odd:
                return jnp.concatenate([jnp.where(row8 < 4, 1.0, v[0:8]), v[8:24]], axis=0)
            return jnp.concatenate([v[0:16], jnp.where(row8 >= 4, 1.0, v[16:24])], axis=0)

        def pv(v, lt, rows, s_ref, m, acc):
            p = jnp.exp2(s_ref[lt, rows, :] - m).astype(BF16)
            o = _dot(v, p)
            return o if acc is None else o + acc

        def finish(base, q, lt, odd, acc):
            if not odd:
                ot_ref[q, pl.ds(base, 24), _lanes(lt)] = acc * (1.0 / acc[20:21])
                return
            oo = acc * (1.0 / acc[0:1])
            mid = jnp.where(row8 < 4, ot_ref[q, pl.ds(base, 8), _lanes(lt)], oo[0:8])
            ot_ref[q, pl.ds(base, 24), _lanes(lt)] = jnp.concatenate([mid, oo[8:24]], axis=0)

        def vbase(g, j):
            off = (j // 2) * 40 + (16 if j % 2 else 0)
            if isinstance(g, int):
                return g * GD + off
            return pl.multiple_of(g * GD + off, 8)

        def body(t, carry):
            m2, m1, acc2 = carry
            zero = pl.multiple_of(jnp.minimum(t, 0), 256)
            tp = jnp.maximum(t - 1, 0)
            g = lax.shift_right_logical(t, sh)
            gn = lax.shift_right_logical(jnp.minimum(t + 1, NP - 1), sh)
            g_prev = lax.shift_right_logical(tp, sh)
            qs = [(t & (NQG - 1)) * QPI + k for k in range(QPI)]
            qs_prev = [(tp & (NQG - 1)) * QPI + k for k in range(QPI)]
            qls = [[q * NL + lt for lt in range(NL)] for q in qs]
            crows = [pl.ds(zero + c * CK, CK) for c in range(NC)]
            krows = [pl.ds(zero + c * 8, 8) for c in range(NC)]
            ms = {-2: list(m2), -1: list(m1)}
            accs = {-2: list(acc2)}
            for n in range(P * NC):
                i, c = n // NC, n % NC
                j, q = i // QPI, qs[i % QPI]
                s_ref = s_refs[i % NSB]
                if c == 0:
                    qms = [get_qm(4 * g + j, j, q, lt) for lt in range(NL)]
                    mx = [None] * NL
                kbs = [kbufs[j % 2][d:d + DG, krows[c], :] for d in range(0, DH, DG)]
                for lt in range(NL):
                    mx[lt] = qk_vpu(kbs, g, j, qls[i % QPI][lt], lt, c, s_ref, mx[lt])
                for lt in range(NL):
                    mx[lt] = qk(g, qms[lt], lt, pieces[lt][c], pieces[lt][c + 1], s_ref, mx[lt])
                nb = (i % QPI) * NC + c
                for d in range((nb * DH) // (QPI * NC), ((nb + 1) * DH) // (QPI * NC)):
                    build(g if j < 3 else gn, (j + 1) % 4, d, kbufs[(j + 1) % 2])
                n2 = n - LG
                i2, c2 = n2 // NC, n2 % NC
                j2 = (i2 % P) // QPI
                if c2 == 0 or n == 0:
                    base2 = vbase(g_prev if i2 < 0 else g, j2)
                q2 = (qs_prev if i2 < 0 else qs)[i2 % QPI]
                v = getv(base2, j2 % 2, c2)
                acc = accs.setdefault(i2, [None] * NL)
                for lt in range(NL):
                    acc[lt] = pv(v, lt, crows[c2], s_refs[i2 % NSB], ms[i2][lt], acc[lt])
                if c2 == NC - 1:
                    for lt in range(NL):
                        finish(base2, q2, lt, j2 % 2, acc[lt])
                if c == NC - 1:
                    for lt in range(NL):
                        mx[lt] = qk(g, qms[lt], lt, pieces[lt][NC], pieces[lt][NC + 1], s_ref, mx[lt])
                    ms[i] = [jnp.max(mx[lt], axis=0, keepdims=True) for lt in range(NL)]
            return tuple(ms[P - 2]), tuple(ms[P - 1]), tuple(accs[P - 2])

        zr = tuple(jnp.zeros((1, 128), F32) for _ in range(NL))
        ones24 = tuple(jnp.ones((24, 128), F32) for _ in range(NL))
        m2, m1, acc2 = SCOPE('s_attn_loop', lambda: lax.fori_loop(0, NP, body, (zr, zr, ones24)))

        def epilogue():
            for (i2, m, acc, c0) in ((P - 2, m2, list(acc2), NC - LAG), (P - 1, m1, [None] * NL, 0)):
                j2 = i2 // QPI
                base2 = vbase(NG - 1, j2)
                q2 = NB - QPI + i2 % QPI
                for c2 in range(c0, NC):
                    v = getv(base2, j2 % 2, c2)
                    for lt in range(NL):
                        acc[lt] = pv(v, lt, pl.ds(c2 * CK, CK), s_refs[i2 % NSB], m[lt], acc[lt])
                    if c2 == NC - 1:
                        for lt in range(NL):
                            finish(base2, q2, lt, j2 % 2, acc[lt])
                    yield
        return epilogue()

    def out_copy(i, s):
        k = i * NS + s
        return pltpu.make_async_copy(obuf.at[k * SB:(k + 1) * SB, :],
                                     out_hbm.at[k * SB:(k + 1) * SB, :], osems.at[k])

    def stage_bout(r, epi):
        @pl.when(r == 1)
        def _():
            for i in range(NB):
                for s in range(NS):
                    out_copy(i, s).wait()

        def blk(i):
            for s in range(NS):
                ot = ot_ref[i, :, _lanes(s)]
                if s == 0 and i in (0, NB - 1):
                    yy = _dot(_up(wt[BO]), ot).T
                else:
                    yy = _dot(ot.T.astype(BF16), wsrc[BO])
                if i < NB - 1:
                    for _ in range(2):
                        next(epi, None)
                y = x_ref[srows(i, s), :] + yy
                x_ref[srows(i, s), :] = y
                x = xin[srows(i, s), :].astype(F32) + y
                obuf[srows(i, s), :] = x.astype(obuf.dtype)
                out_copy(i, s).start()
                if i == 0 and s == 0:
                    xn_ref[0] = _pk(_layernorm(x).astype(BF16))
        for i in range(NB - 1):
            blk(i)

        @pl.when(r >= 0)
        def _():
            blk(NB - 1)

    def round_(r, c):
        SCOPE('s_a', stage_a, r)
        SCOPE('s_amid', a_mid)
        SCOPE('s_l2', lambda: lax.fori_loop(0, NB, stage_l2, 0))
        epi = attention()
        SCOPE('s_bout', stage_bout, r, epi)
        return c
    lax.fori_loop(0, 2, round_, 0)
    for i in range(NB):
        for s in range(NS):
            out_copy(i, s).wait()


@jax.jit
def pallas_interleave_layers__linear_attn_block__mha_block__prompt_kernel(
    A_x: jax.Array,
    A_wqkv: jax.Array,
    A_wo: jax.Array,
    B_x: jax.Array,
    B_wqkv: jax.Array,
    B_wo: jax.Array,
):
    del B_x
    x = A_x.reshape(S, D)
    scratch = [
        pltpu.VMEM((S, D), BF16),
        pltpu.VMEM((8, D, D), BF16),
        pltpu.VMEM((S, D), BF16),
        pltpu.SemaphoreType.DMA((NB + 8,)),
        pltpu.SemaphoreType.DMA((NB * NS,)),
        pltpu.VMEM((S, D), F32),
        pltpu.VMEM((2, SB // 2, D), U32),
        pltpu.VMEM((7, D // 2, D), U32),
        pltpu.VMEM((D // 2, D), U32),
        pltpu.VMEM((NB, D // 2, TB), U32),
        pltpu.VMEM((D, D), F32),
        pltpu.VMEM((D, 128), F32),
        pltpu.VMEM((D // 2, D), U32),
        pltpu.VMEM((NB, H, TB), F32),
        pltpu.VMEM((H, D), jnp.int32),
        pltpu.VMEM((5, 160, 128), jnp.int32),
        pltpu.VMEM((NG, S // 2, 128), U32),
        pltpu.VMEM((H, NB, 16, TB), U32),
        pltpu.VMEM((NB, D, TB), F32),
        pltpu.VMEM((NB, D, TB), F32),
        pltpu.VMEM((S // 128, NG, GD, 8, 128), F32),
        pltpu.VMEM((NG, KV, 128), F32),
        pltpu.VMEM((DH, KV, 128), F32),
        pltpu.VMEM((DH, KV, 128), F32),
    ] + [pltpu.VMEM((NL, S, 128), F32) for _ in range(NSB)]
    out = pl.pallas_call(
        _kernel,
        out_shape=jax.ShapeDtypeStruct((S, D), A_x.dtype),
        in_specs=[pl.BlockSpec(memory_space=pl.ANY)] * 5,
        out_specs=pl.BlockSpec(memory_space=pl.ANY),
        scratch_shapes=scratch,
        compiler_params=pltpu.CompilerParams(vmem_limit_bytes=124 * 1024 * 1024),
    )(x, A_wqkv, A_wo, B_wqkv, B_wo)
    return out.reshape(A_x.shape)
```

```python
import math

import jax
import jax.numpy as jnp
from jax import lax
import jax.experimental.pallas as pl
import jax.experimental.pallas.tpu as pltpu

S = 2048
D = 640
H = 32
DH = 20
NG = 8
GD = 4 * DH
TB = 512
NB = S // TB
SB = 128
NS = TB // SB
NL = TB // 128
CK = 128
NC = S // CK
QPI = 2
LAG = 2
NSB = 4
KV = 128
SM = S - KV
STAG = (16, 48, 80, 112)
DG = 5
LN_EPS = 1e-5
QSCALE = (DH ** -0.5) * math.log2(math.e)
KV_ROWS = [(0, 144), (112, 272), (240, 400), (368, 528), (496, 640)]
AQ, AV, BQ, BK, BV, AO, BO, AK = range(8)

ORDER = []
for _g in range(NG):
    ORDER += [(BK, _g), (BQ, _g)] + ([(BV, _g - 2)] if _g >= 2 else [])
ORDER += [(BV, NG - 2), (BV, NG - 1)]

F32 = jnp.float32
BF16 = jnp.bfloat16
U32 = jnp.uint32
NN = (((1,), (0,)), ((), ()))
NT = (((1,), (1,)), ((), ()))


def SCOPE(name, f, *args):
    del name
    return f(*args)


def _dot(a, b, dims=NN):
    return lax.dot_general(a, b, dims, preferred_element_type=F32)


def _pk(x):
    return pltpu.bitcast(x, U32)


def _up(x):
    return pltpu.bitcast(x, BF16)


def _phi(t):
    return jnp.where(t > 0, t + 1.0, jnp.exp(jnp.minimum(t, 0.0))) + 1e-6


def _layernorm(x):
    m = jnp.mean(x, axis=-1, keepdims=True)
    xc = x - m
    v = jnp.mean(xc * xc, axis=-1, keepdims=True)
    return xc * lax.rsqrt(v + LN_EPS)


def _lanes(k):
    return slice(k * 128, (k + 1) * 128)


def _kernel(x_hbm, awqkv_hbm, awo_hbm, bwqkv_hbm, bwo_hbm, out_hbm,
            xin, wsrc, obuf, sems, osems,
            x_ref, xn_ref, wt, wkt_a,
            pqt_ref, gt_ref, z_ref, mt_ref, r_ref, zmask_ref, kvmask_ref,
            k_ref, qt_ref, vt_ref, ot_ref, qb_ref, kf_ref, kb0, kb1, *s_refs):
    kbufs = (kb0, kb1)
    row8 = lax.broadcasted_iota(jnp.int32, (8, 128), 0)

    def srows(i, s):
        if isinstance(i, int):
            return pl.ds(i * TB + s * SB, SB)
        return pl.ds(pl.multiple_of(i * TB + s * SB, SB), SB)

    def cp_x(i):
        lo = 0 if i == 0 else i * TB + SB
        hi = min((i + 1) * TB + SB, S)
        return pltpu.make_async_copy(x_hbm.at[lo:hi, :], xin.at[lo:hi, :], sems.at[i])

    w_srcs = {AQ: awqkv_hbm.at[:, 0:D], AK: awqkv_hbm.at[:, D:2 * D],
              AV: awqkv_hbm.at[:, 2 * D:3 * D], AO: awo_hbm,
              BQ: bwqkv_hbm.at[:, 0:D], BK: bwqkv_hbm.at[:, D:2 * D],
              BV: bwqkv_hbm.at[:, 2 * D:3 * D], BO: bwo_hbm}

    def cp_w(m):
        return pltpu.make_async_copy(w_srcs[m], wsrc.at[m], sems.at[NB + m])

    def ln_sub(i, s):
        x = xin[srows(i, s), :].astype(F32) + x_ref[srows(i, s), :]
        return _layernorm(x).astype(BF16)

    cp_w(AK).start()
    x_ref[...] = jnp.zeros(x_ref.shape, F32)
    cp_x(0).start()
    cp_w(AQ).start()
    hr2 = lax.broadcasted_iota(jnp.int32, (H, D), 0)
    hc2 = lax.broadcasted_iota(jnp.int32, (H, D), 1) // DH
    zmask_ref[...] = (hr2 == hc2).astype(jnp.int32)
    for j, (r0, r1) in enumerate(KV_ROWS):
        hr = (lax.broadcasted_iota(jnp.int32, (160, 128), 0) + r0) // DH
        hc = (lax.broadcasted_iota(jnp.int32, (160, 128), 1) + j * 128) // DH
        kvmask_ref[j] = (hr == hc).astype(jnp.int32)
    cp_w(AK).wait()
    wkt_a[...] = _pk(wsrc[AK].T)
    gt_ref[...] = jnp.zeros(gt_ref.shape, F32)
    z_ref[...] = jnp.zeros(z_ref.shape, F32)
    s_refs[NSB - 1][...] = jnp.zeros((NL, S, 128), F32)
    s_refs[NSB - 2][:, (NC - LAG) * CK:, :] = jnp.zeros((NL, LAG * CK, 128), F32)
    ot_ref[0:QPI, 56:64, :] = jnp.zeros((QPI, 8, TB), F32)
    cp_x(0).wait()
    xn_ref[0] = _pk(ln_sub(0, 0))
    cp_w(AQ).wait()
    for i in range(1, NB):
        cp_x(i).start()
        cp_w(2 * i - 1).start()
        cp_w(2 * i).start()

    def stage_a(r):
        def body(i, c):
            for i_s in range(1, NB):
                @pl.when((r == 0) & (i == i_s))
                def _():
                    cp_x(i_s).wait()
                    cp_w(2 * i_s - 1).wait()
                    cp_w(2 * i_s).wait()

            xns = [_up(xn_ref[i & 1])] + [ln_sub(i, s) for s in range(1, NS)]
            pkts = [_phi(_dot(_up(wkt_a[...]), xn, NT)) for xn in xns]
            for m in (jnp.maximum(2 * i - 1, 0), 2 * i):
                wt[m] = _pk(wsrc[m].T)
            xn_ref[(i + 1) & 1] = _pk(ln_sub(jnp.minimum(i + 1, NB - 1), 0))
            xn0_late = _up(xn_ref[i & 1])
            z_ref[...] = (jnp.where(i > 0, z_ref[...], 0.0)
                          + (pkts[0] + pkts[1]) + (pkts[2] + pkts[3]))
            for s in range(NS):
                if s == NS // 2:
                    gt_ref[...] = _dot(
                        jnp.concatenate(pkts, axis=1),
                        jnp.concatenate([xn0_late] + xns[1:], axis=0)
                    ) + jnp.where(i > 0, gt_ref[...], 0.0)
                qt = _dot(_up(wt[AQ]), xns[s], NT)
                pqt_ref[i, :, _lanes(s)] = _pk(_phi(qt).astype(BF16))
            return c
        lax.fori_loop(0, NB, body, 0)

    def a_mid():
        z = _dot(jnp.ones((8, 128), F32), z_ref[...], NT)[0:1]
        zm = jnp.where(zmask_ref[...] > 0, z, 0.0)
        kvs = []
        for j, (r0, r1) in enumerate(KV_ROWS):
            kvj = _dot(_up(wt[AV, r0 // 2:r1 // 2, :]), gt_ref[_lanes(j), :], NT)
            kvs.append(jnp.where(kvmask_ref[j, 0:r1 - r0, :] > 0, kvj, 0.0))
        for j, (r0, r1) in enumerate(KV_ROWS):
            if j < NB:
                r_ref[j] = 1.0 / (_dot(zm, _up(pqt_ref[j])) + 1e-6)
            k0 = (r0 // 128) * 128
            k1 = -(-r1 // 128) * 128
            pads = []
            if r0 > k0:
                pads.append(jnp.zeros((r0 - k0, 128), F32))
            pads.append(kvs[j])
            if k1 > r1:
                pads.append(jnp.zeros((k1 - r1, 128), F32))
            kvj = jnp.concatenate(pads, axis=0)
            mt_ref[:, _lanes(j)] = _pk(_dot(_up(wt[AO, :, k0:k1]), kvj).astype(BF16))

    def stage_l2(i, c):
        pqns = []
        for s in range(NS):
            pq = _up(pqt_ref[i, :, _lanes(s)])
            r = r_ref[i, :, _lanes(s)]
            parts = []
            for a in range(H // 2):
                re = jnp.broadcast_to(r[2 * a:2 * a + 1], (8, SB))
                ro = jnp.broadcast_to(r[2 * a + 1:2 * a + 2], (8, SB))
                parts += [re, re, jnp.where(row8 < 4, re, ro), ro, ro]
            pqns.append((pq.astype(F32) * jnp.concatenate(parts, axis=0)).astype(BF16))
        xns = []
        for s in range(NS):
            y = x_ref[srows(i, s), :] + _dot(_up(mt_ref[...]), pqns[s]).T
            x_ref[srows(i, s), :] = y
            xns.append(_layernorm(xin[srows(i, s), :].astype(F32) + y).astype(BF16))
        zpad = jnp.zeros((8, SB), F32)
        for s in range(NS):
            ps = (s + NS - 1) % NS
            wl = jnp.concatenate(
                [wt[m, g * GD // 2:(g + 1) * GD // 2, :] for (m, g) in ORDER], axis=0)
            res = _dot(_up(wl), xns[s], NT)
            blk = {mg: res[n * GD:(n + 1) * GD] for n, mg in enumerate(ORDER)}
            krow0 = pl.ds(pl.multiple_of((i * TB + ps * SB) // 2, SB // 2), SB // 2)
            for g in range(NG):
                kt = blk[BK, g]
                qt = blk[BQ, g] * QSCALE
                vt_ref[i, g * GD:(g + 1) * GD, _lanes(ps)] = blk[BV, g]
                kparts = []
                for j in range(4):
                    r0 = (j // 2) * 40 + (16 if j % 2 else 0)
                    kparts += [kt[r0:r0 + 24], zpad]
                    if j % 2:
                        qw = [jnp.where(row8 < 4, 0.0, qt[r0:r0 + 8]), qt[r0 + 8:r0 + 24], zpad]
                    else:
                        qw = [qt[r0:r0 + 16], jnp.where(row8 < 4, qt[r0 + 16:r0 + 24], 0.0), zpad]
                    qt_ref[4 * g + j, i, :, _lanes(s)] = _pk(
                        jnp.concatenate(qw, axis=0).astype(BF16))
                kb = jnp.concatenate(kparts, axis=0).T
                k_ref[g, krow0, :] = _pk(kb.astype(BF16))
                if ps == NS - 1:
                    kf_ref[g] = kb
                    if g == 0:
                        for d in range(DH):
                            kbufs[0][d] = jnp.broadcast_to(kb[:, d:d + 1], (KV, 128))
                qb_ref[i * NS + s, g] = jnp.broadcast_to(qt.reshape(GD, 1, SB), (GD, 8, SB))
        return c

    def attention():
        NQG = NB // QPI
        NP = NG * NQG
        P = 4 * QPI
        LG = NC + LAG
        sh = NQG.bit_length() - 1
        units = SM // 16
        bounds = [16 * ((c * units + NC - 1) // NC) for c in range(NC + 1)]
        pieces = [[0] + [x - (bounds[1] - STAG[lt]) for x in bounds[1:]] + [SM]
                  for lt in range(NL)]

        def get_qm(h, j, q, lt):
            parts = []
            if j > 0:
                parts.append(jnp.zeros((32 * j, 128), BF16))
            parts.append(_up(qt_ref[h, q, :, _lanes(lt)]))
            if j < 3:
                parts.append(jnp.zeros((96 - 32 * j, 128), BF16))
            return jnp.concatenate(parts, axis=0)

        def qk(g, qm, lt, r0, r1, s_ref, mx):
            s = _dot(_up(k_ref[g, r0 // 2:r1 // 2, :]), qm)
            s_ref[lt, r0:r1, :] = s
            return jnp.maximum(mx, jnp.max(s.reshape((r1 - r0) // 8, 8, 128), axis=0))

        def build(g, j, d, kb):
            l = 32 * j + (4 if j % 2 else 0) + d
            kb[d] = jnp.broadcast_to(kf_ref[g, :, l:l + 1], (KV, 128))

        def qk_vpu(kbs, g, j, ql, lt, vi, s_ref, mx):
            s = None
            for n, d in enumerate(range(0, DH, DG)):
                t = kbs[n] * qb_ref[ql, g, j * DH + d:j * DH + d + DG]
                if s is not None:
                    t = jnp.concatenate([s[None], t], axis=0)
                s = jnp.sum(t, axis=0)
            s_ref[lt, SM + vi * 8:SM + vi * 8 + 8, :] = s
            return s if mx is None else jnp.maximum(mx, s)

        def getv(base, odd, c):
            cb, co = (c * CK) // TB, (c * CK) % TB
            v = vt_ref[cb, pl.ds(base, 24), co:co + CK]
            if odd:
                return jnp.concatenate([jnp.where(row8 < 4, 1.0, v[0:8]), v[8:24]], axis=0)
            return jnp.concatenate([v[0:16], jnp.where(row8 >= 4, 1.0, v[16:24])], axis=0)

        def pv(v, lt, rows, s_ref, m, acc):
            p = jnp.exp2(s_ref[lt, rows, :] - m).astype(BF16)
            o = _dot(v, p)
            return o if acc is None else o + acc

        def finish(base, q, lt, odd, acc):
            if not odd:
                ot_ref[q, pl.ds(base, 24), _lanes(lt)] = acc * (1.0 / acc[20:21])
                return
            oo = acc * (1.0 / acc[0:1])
            mid = jnp.where(row8 < 4, ot_ref[q, pl.ds(base, 8), _lanes(lt)], oo[0:8])
            ot_ref[q, pl.ds(base, 24), _lanes(lt)] = jnp.concatenate([mid, oo[8:24]], axis=0)

        def vbase(g, j):
            off = (j // 2) * 40 + (16 if j % 2 else 0)
            if isinstance(g, int):
                return g * GD + off
            return pl.multiple_of(g * GD + off, 8)

        def body(t, carry):
            m2, m1, acc2 = carry
            zero = pl.multiple_of(jnp.minimum(t, 0), 256)
            tp = jnp.maximum(t - 1, 0)
            g = lax.shift_right_logical(t, sh)
            gn = lax.shift_right_logical(jnp.minimum(t + 1, NP - 1), sh)
            g_prev = lax.shift_right_logical(tp, sh)
            qs = [(t & (NQG - 1)) * QPI + k for k in range(QPI)]
            qs_prev = [(tp & (NQG - 1)) * QPI + k for k in range(QPI)]
            qls = [[q * NL + lt for lt in range(NL)] for q in qs]
            crows = [pl.ds(zero + c * CK, CK) for c in range(NC)]
            krows = [pl.ds(zero + c * 8, 8) for c in range(NC)]
            ms = {-2: list(m2), -1: list(m1)}
            accs = {-2: list(acc2)}
            for n in range(P * NC):
                i, c = n // NC, n % NC
                j, q = i // QPI, qs[i % QPI]
                s_ref = s_refs[i % NSB]
                if c == 0:
                    qms = [get_qm(4 * g + j, j, q, lt) for lt in range(NL)]
                    mx = [None] * NL
                kbs = [kbufs[j % 2][d:d + DG, krows[c], :] for d in range(0, DH, DG)]
                for lt in range(NL):
                    mx[lt] = qk_vpu(kbs, g, j, qls[i % QPI][lt], lt, c, s_ref, mx[lt])
                for lt in range(NL):
                    mx[lt] = qk(g, qms[lt], lt, pieces[lt][c], pieces[lt][c + 1], s_ref, mx[lt])
                nb = (i % QPI) * NC + c
                for d in range((nb * DH) // (QPI * NC), ((nb + 1) * DH) // (QPI * NC)):
                    build(g if j < 3 else gn, (j + 1) % 4, d, kbufs[(j + 1) % 2])
                n2 = n - LG
                i2, c2 = n2 // NC, n2 % NC
                j2 = (i2 % P) // QPI
                if c2 == 0 or n == 0:
                    base2 = vbase(g_prev if i2 < 0 else g, j2)
                q2 = (qs_prev if i2 < 0 else qs)[i2 % QPI]
                v = getv(base2, j2 % 2, c2)
                acc = accs.setdefault(i2, [None] * NL)
                for lt in range(NL):
                    acc[lt] = pv(v, lt, crows[c2], s_refs[i2 % NSB], ms[i2][lt], acc[lt])
                if c2 == NC - 1:
                    for lt in range(NL):
                        finish(base2, q2, lt, j2 % 2, acc[lt])
                if c == NC - 1:
                    for lt in range(NL):
                        mx[lt] = qk(g, qms[lt], lt, pieces[lt][NC], pieces[lt][NC + 1], s_ref, mx[lt])
                    ms[i] = [jnp.max(mx[lt], axis=0, keepdims=True) for lt in range(NL)]
            return tuple(ms[P - 2]), tuple(ms[P - 1]), tuple(accs[P - 2])

        zr = tuple(jnp.zeros((1, 128), F32) for _ in range(NL))
        ones24 = tuple(jnp.ones((24, 128), F32) for _ in range(NL))
        m2, m1, acc2 = SCOPE('s_attn_loop', lambda: lax.fori_loop(0, NP, body, (zr, zr, ones24)))

        def epilogue():
            for (i2, m, acc, c0) in ((P - 2, m2, list(acc2), NC - LAG), (P - 1, m1, [None] * NL, 0)):
                j2 = i2 // QPI
                base2 = vbase(NG - 1, j2)
                q2 = NB - QPI + i2 % QPI
                for c2 in range(c0, NC):
                    v = getv(base2, j2 % 2, c2)
                    for lt in range(NL):
                        acc[lt] = pv(v, lt, pl.ds(c2 * CK, CK), s_refs[i2 % NSB], m[lt], acc[lt])
                    if c2 == NC - 1:
                        for lt in range(NL):
                            finish(base2, q2, lt, j2 % 2, acc[lt])
                    yield
        return epilogue()

    def out_copy(i, s):
        k = i * NS + s
        return pltpu.make_async_copy(obuf.at[k * SB:(k + 1) * SB, :],
                                     out_hbm.at[k * SB:(k + 1) * SB, :], osems.at[k])

    def stage_bout(r, epi):
        @pl.when(r == 1)
        def _():
            for i in range(NB):
                for s in range(NS):
                    out_copy(i, s).wait()

        def blk(i):
            for s in range(NS):
                ot = ot_ref[i, :, _lanes(s)]
                if s == 0 and i in (0, NB - 1):
                    yy = _dot(_up(wt[BO]), ot).T
                else:
                    yy = _dot(ot.T.astype(BF16), wsrc[BO])
                if i < NB - 1:
                    for _ in range(2):
                        next(epi, None)
                y = x_ref[srows(i, s), :] + yy
                x_ref[srows(i, s), :] = y
                x = xin[srows(i, s), :].astype(F32) + y
                obuf[srows(i, s), :] = x.astype(obuf.dtype)
                out_copy(i, s).start()
                if i == 0 and s == 0:
                    xn_ref[0] = _pk(_layernorm(x).astype(BF16))
        for i in range(NB - 1):
            blk(i)

        @pl.when(r >= 0)
        def _():
            blk(NB - 1)

    def round_(r, c):
        SCOPE('s_a', stage_a, r)
        SCOPE('s_amid', a_mid)
        SCOPE('s_l2', lambda: lax.fori_loop(0, NB, stage_l2, 0))
        epi = attention()
        SCOPE('s_bout', stage_bout, r, epi)
        return c
    lax.fori_loop(0, 2, round_, 0)
    for i in range(NB):
        for s in range(NS):
            out_copy(i, s).wait()


@jax.jit
def pallas_interleave_layers__linear_attn_block__mha_block__prompt_kernel(
    A_x: jax.Array,
    A_wqkv: jax.Array,
    A_wo: jax.Array,
    B_x: jax.Array,
    B_wqkv: jax.Array,
    B_wo: jax.Array,
):
    del B_x
    x = A_x.reshape(S, D)
    scratch = [
        pltpu.VMEM((S, D), BF16),
        pltpu.VMEM((8, D, D), BF16),
        pltpu.VMEM((S, D), BF16),
        pltpu.SemaphoreType.DMA((NB + 8,)),
        pltpu.SemaphoreType.DMA((NB * NS,)),
        pltpu.VMEM((S, D), F32),
        pltpu.VMEM((2, SB // 2, D), U32),
        pltpu.VMEM((7, D // 2, D), U32),
        pltpu.VMEM((D // 2, D), U32),
        pltpu.VMEM((NB, D // 2, TB), U32),
        pltpu.VMEM((D, D), F32),
        pltpu.VMEM((D, 128), F32),
        pltpu.VMEM((D // 2, D), U32),
        pltpu.VMEM((NB, H, TB), F32),
        pltpu.VMEM((H, D), jnp.int32),
        pltpu.VMEM((5, 160, 128), jnp.int32),
        pltpu.VMEM((NG, S // 2, 128), U32),
        pltpu.VMEM((H, NB, 16, TB), U32),
        pltpu.VMEM((NB, D, TB), F32),
        pltpu.VMEM((NB, D, TB), F32),
        pltpu.VMEM((S // 128, NG, GD, 8, 128), F32),
        pltpu.VMEM((NG, KV, 128), F32),
        pltpu.VMEM((DH, KV, 128), F32),
        pltpu.VMEM((DH, KV, 128), F32),
    ] + [pltpu.VMEM((NL, S, 128), F32) for _ in range(NSB)]
    out = pl.pallas_call(
        _kernel,
        out_shape=jax.ShapeDtypeStruct((S, D), A_x.dtype),
        in_specs=[pl.BlockSpec(memory_space=pl.ANY)] * 5,
        out_specs=pl.BlockSpec(memory_space=pl.ANY),
        scratch_shapes=scratch,
        compiler_params=pltpu.CompilerParams(vmem_limit_bytes=124 * 1024 * 1024),
    )(x, A_wqkv, A_wo, B_wqkv, B_wo)
    return out.reshape(A_x.shape)
```

```python
import math

import jax
import jax.numpy as jnp
from jax import lax
import jax.experimental.pallas as pl
import jax.experimental.pallas.tpu as pltpu

S = 2048
D = 640
H = 32
DH = 20
NG = 8
GD = 4 * DH
TB = 512
NB = S // TB
SB = 128
NS = TB // SB
NL = TB // 128
CK = 128
NC = S // CK
QPI = 2
LAG = 2
NSB = 4
KV = 128
SM = S - KV
STAG = (16, 48, 80, 112)
DG = 5
LN_EPS = 1e-5
QSCALE = (DH ** -0.5) * math.log2(math.e)
KV_ROWS = [(0, 144), (112, 272), (240, 400), (368, 528), (496, 640)]
AQ, AV, BQ, BK, BV, AO, BO, AK = range(8)

ORDER = []
for _g in range(NG):
    ORDER += [(BK, _g), (BQ, _g)] + ([(BV, _g - 2)] if _g >= 2 else [])
ORDER += [(BV, NG - 2), (BV, NG - 1)]

F32 = jnp.float32
BF16 = jnp.bfloat16
U32 = jnp.uint32
NN = (((1,), (0,)), ((), ()))
NT = (((1,), (1,)), ((), ()))


def _dot(a, b, dims=NN):
    return lax.dot_general(a, b, dims, precision=lax.Precision.DEFAULT,
                           preferred_element_type=F32)


def _pk(x):
    return pltpu.bitcast(x, U32)


def _up(x):
    return pltpu.bitcast(x, BF16)


def _phi(t):
    return jnp.where(t > 0, t + 1.0, jnp.exp(jnp.minimum(t, 0.0))) + 1e-6


def _layernorm(x):
    m = jnp.mean(x, axis=-1, keepdims=True)
    xc = x - m
    v = jnp.mean(xc * xc, axis=-1, keepdims=True)
    return xc * lax.rsqrt(v + LN_EPS)


def _lanes(k):
    return slice(k * 128, (k + 1) * 128)


def _kernel(x_hbm, awqkv_hbm, awo_hbm, bwqkv_hbm, bwo_hbm, out_hbm,
            xin, wsrc, obuf, sems, osems,
            x_ref, xn_ref, wt, wkt_a,
            pqt_ref, gt_ref, z_ref, mt_ref, r_ref, zmask_ref, kvmask_ref,
            k_ref, qt_ref, vt_ref, ot_ref, qb_ref, kf_ref, kb0, kb1, *s_refs):
    kbufs = (kb0, kb1)
    row8 = lax.broadcasted_iota(jnp.int32, (8, 128), 0)

    def srows(i, s):
        if isinstance(i, int):
            return pl.ds(i * TB + s * SB, SB)
        return pl.ds(pl.multiple_of(i * TB + s * SB, SB), SB)

    def cp_x(i):
        lo = 0 if i == 0 else i * TB + SB
        hi = min((i + 1) * TB + SB, S)
        return pltpu.make_async_copy(x_hbm.at[lo:hi, :], xin.at[lo:hi, :], sems.at[i])

    w_srcs = {AQ: awqkv_hbm.at[:, 0:D], AK: awqkv_hbm.at[:, D:2 * D],
              AV: awqkv_hbm.at[:, 2 * D:3 * D], AO: awo_hbm,
              BQ: bwqkv_hbm.at[:, 0:D], BK: bwqkv_hbm.at[:, D:2 * D],
              BV: bwqkv_hbm.at[:, 2 * D:3 * D], BO: bwo_hbm}

    def cp_w(m):
        return pltpu.make_async_copy(w_srcs[m], wsrc.at[m], sems.at[NB + m])

    def ln_sub(i, s):
        x = xin[srows(i, s), :].astype(F32) + x_ref[srows(i, s), :]
        return _layernorm(x).astype(BF16)

    cp_w(AK).start()
    x_ref[...] = jnp.zeros(x_ref.shape, F32)
    cp_x(0).start()
    cp_w(AQ).start()
    hr2 = lax.broadcasted_iota(jnp.int32, (H, D), 0)
    hc2 = lax.broadcasted_iota(jnp.int32, (H, D), 1) // DH
    zmask_ref[...] = (hr2 == hc2).astype(jnp.int32)
    for j, (r0, r1) in enumerate(KV_ROWS):
        hr = (lax.broadcasted_iota(jnp.int32, (160, 128), 0) + r0) // DH
        hc = (lax.broadcasted_iota(jnp.int32, (160, 128), 1) + j * 128) // DH
        kvmask_ref[j] = (hr == hc).astype(jnp.int32)
    cp_w(AK).wait()
    wkt_a[...] = _pk(wsrc[AK].T)
    gt_ref[...] = jnp.zeros(gt_ref.shape, F32)
    z_ref[...] = jnp.zeros(z_ref.shape, F32)
    s_refs[NSB - 1][...] = jnp.zeros((NL, S, 128), F32)
    s_refs[NSB - 2][:, (NC - LAG) * CK:, :] = jnp.zeros((NL, LAG * CK, 128), F32)
    ot_ref[0:QPI, 56:64, :] = jnp.zeros((QPI, 8, TB), F32)
    cp_x(0).wait()
    xn_ref[0] = _pk(ln_sub(0, 0))
    cp_w(AQ).wait()
    for i in range(1, NB):
        cp_x(i).start()
        cp_w(2 * i - 1).start()
        cp_w(2 * i).start()

    def stage_a(r):
        def body(i, c):
            for i_s in range(1, NB):
                @pl.when((r == 0) & (i == i_s))
                def _():
                    cp_x(i_s).wait()
                    cp_w(2 * i_s - 1).wait()
                    cp_w(2 * i_s).wait()

            xns = [_up(xn_ref[i & 1])] + [ln_sub(i, s) for s in range(1, NS)]
            pkts = [_phi(_dot(_up(wkt_a[...]), xn, NT)) for xn in xns]
            for m in (jnp.maximum(2 * i - 1, 0), 2 * i):
                wt[m] = _pk(wsrc[m].T)
            xn_ref[(i + 1) & 1] = _pk(ln_sub(jnp.minimum(i + 1, NB - 1), 0))
            xn0_late = _up(xn_ref[i & 1])
            z_ref[...] = (jnp.where(i > 0, z_ref[...], 0.0)
                          + (pkts[0] + pkts[1]) + (pkts[2] + pkts[3]))
            for s in range(NS):
                if s == NS // 2:
                    gt_ref[...] = _dot(
                        jnp.concatenate(pkts, axis=1),
                        jnp.concatenate([xn0_late] + xns[1:], axis=0)
                    ) + jnp.where(i > 0, gt_ref[...], 0.0)
                qt = _dot(_up(wt[AQ]), xns[s], NT)
                pqt_ref[i, :, _lanes(s)] = _pk(_phi(qt).astype(BF16))
            return c
        lax.fori_loop(0, NB, body, 0)

    def a_mid():
        z = _dot(jnp.ones((8, 128), F32), z_ref[...], NT)[0:1]
        zm = jnp.where(zmask_ref[...] > 0, z, 0.0)
        kvs = []
        for j, (r0, r1) in enumerate(KV_ROWS):
            kvj = _dot(_up(wt[AV, r0 // 2:r1 // 2, :]), gt_ref[_lanes(j), :], NT)
            kvs.append(jnp.where(kvmask_ref[j, 0:r1 - r0, :] > 0, kvj, 0.0))
        for j, (r0, r1) in enumerate(KV_ROWS):
            if j < NB:
                r_ref[j] = 1.0 / (_dot(zm, _up(pqt_ref[j])) + 1e-6)
            k0 = (r0 // 128) * 128
            k1 = -(-r1 // 128) * 128
            pads = []
            if r0 > k0:
                pads.append(jnp.zeros((r0 - k0, 128), F32))
            pads.append(kvs[j])
            if k1 > r1:
                pads.append(jnp.zeros((k1 - r1, 128), F32))
            kvj = jnp.concatenate(pads, axis=0)
            mt_ref[:, _lanes(j)] = _pk(_dot(_up(wt[AO, :, k0:k1]), kvj).astype(BF16))

    def stage_l2(i, c):
        pqns = []
        for s in range(NS):
            pq = _up(pqt_ref[i, :, _lanes(s)])
            r = r_ref[i, :, _lanes(s)]
            parts = []
            for a in range(H // 2):
                re = jnp.broadcast_to(r[2 * a:2 * a + 1], (8, SB))
                ro = jnp.broadcast_to(r[2 * a + 1:2 * a + 2], (8, SB))
                parts += [re, re, jnp.where(row8 < 4, re, ro), ro, ro]
            pqns.append((pq.astype(F32) * jnp.concatenate(parts, axis=0)).astype(BF16))
        xns = []
        for s in range(NS):
            y = x_ref[srows(i, s), :] + _dot(_up(mt_ref[...]), pqns[s]).T
            x_ref[srows(i, s), :] = y
            xns.append(_layernorm(xin[srows(i, s), :].astype(F32) + y).astype(BF16))
        zpad = jnp.zeros((8, SB), F32)
        for s in range(NS):
            ps = (s + NS - 1) % NS
            wl = jnp.concatenate(
                [wt[m, g * GD // 2:(g + 1) * GD // 2, :] for (m, g) in ORDER], axis=0)
            res = _dot(_up(wl), xns[s], NT)
            blk = {mg: res[n * GD:(n + 1) * GD] for n, mg in enumerate(ORDER)}
            krow0 = pl.ds(pl.multiple_of((i * TB + ps * SB) // 2, SB // 2), SB // 2)
            for g in range(NG):
                kt = blk[BK, g]
                qt = blk[BQ, g] * QSCALE
                vt_ref[i, g * GD:(g + 1) * GD, _lanes(ps)] = blk[BV, g]
                kparts = []
                for j in range(4):
                    r0 = (j // 2) * 40 + (16 if j % 2 else 0)
                    kparts += [kt[r0:r0 + 24], zpad]
                    if j % 2:
                        qw = [jnp.where(row8 < 4, 0.0, qt[r0:r0 + 8]), qt[r0 + 8:r0 + 24], zpad]
                    else:
                        qw = [qt[r0:r0 + 16], jnp.where(row8 < 4, qt[r0 + 16:r0 + 24], 0.0), zpad]
                    qt_ref[4 * g + j, i, :, _lanes(s)] = _pk(
                        jnp.concatenate(qw, axis=0).astype(BF16))
                kb = jnp.concatenate(kparts, axis=0).T
                k_ref[g, krow0, :] = _pk(kb.astype(BF16))
                if ps == NS - 1:
                    kf_ref[g] = kb
                    if g == 0:
                        for d in range(DH):
                            kbufs[0][d] = jnp.broadcast_to(kb[:, d:d + 1], (KV, 128))
                qb_ref[i * NS + s, g] = jnp.broadcast_to(qt.reshape(GD, 1, SB), (GD, 8, SB))
        return c

    def attention():
        NQG = NB // QPI
        NP = NG * NQG
        P = 4 * QPI
        LG = NC + LAG
        sh = NQG.bit_length() - 1
        units = SM // 16
        bounds = [16 * ((c * units + NC - 1) // NC) for c in range(NC + 1)]
        pieces = [[0] + [x - (bounds[1] - STAG[lt]) for x in bounds[1:]] + [SM]
                  for lt in range(NL)]

        def get_qm(h, j, q, lt):
            parts = []
            if j > 0:
                parts.append(jnp.zeros((32 * j, 128), BF16))
            parts.append(_up(qt_ref[h, q, :, _lanes(lt)]))
            if j < 3:
                parts.append(jnp.zeros((96 - 32 * j, 128), BF16))
            return jnp.concatenate(parts, axis=0)

        def qk(g, qm, lt, r0, r1, s_ref, mx):
            s = _dot(_up(k_ref[g, r0 // 2:r1 // 2, :]), qm)
            s_ref[lt, r0:r1, :] = s
            return jnp.maximum(mx, jnp.max(s.reshape((r1 - r0) // 8, 8, 128), axis=0))

        def build(g, j, d, kb):
            l = 32 * j + (4 if j % 2 else 0) + d
            kb[d] = jnp.broadcast_to(kf_ref[g, :, l:l + 1], (KV, 128))

        def qk_vpu(kbs, g, j, ql, lt, vi, s_ref, mx):
            s = None
            for n, d in enumerate(range(0, DH, DG)):
                t = kbs[n] * qb_ref[ql, g, j * DH + d:j * DH + d + DG]
                if s is not None:
                    t = jnp.concatenate([s[None], t], axis=0)
                s = jnp.sum(t, axis=0)
            s_ref[lt, SM + vi * 8:SM + vi * 8 + 8, :] = s
            return s if mx is None else jnp.maximum(mx, s)

        def getv(base, odd, c):
            cb, co = (c * CK) // TB, (c * CK) % TB
            v = vt_ref[cb, pl.ds(base, 24), co:co + CK]
            if odd:
                return jnp.concatenate([jnp.where(row8 < 4, 1.0, v[0:8]), v[8:24]], axis=0)
            return jnp.concatenate([v[0:16], jnp.where(row8 >= 4, 1.0, v[16:24])], axis=0)

        def pv(v, lt, rows, s_ref, m, acc):
            p = jnp.exp2(s_ref[lt, rows, :] - m).astype(BF16)
            o = _dot(v, p)
            return o if acc is None else o + acc

        def finish(base, q, lt, odd, acc):
            if not odd:
                ot_ref[q, pl.ds(base, 24), _lanes(lt)] = acc * (1.0 / acc[20:21])
                return
            oo = acc * (1.0 / acc[0:1])
            mid = jnp.where(row8 < 4, ot_ref[q, pl.ds(base, 8), _lanes(lt)], oo[0:8])
            ot_ref[q, pl.ds(base, 24), _lanes(lt)] = jnp.concatenate([mid, oo[8:24]], axis=0)

        def vbase(g, j):
            off = (j // 2) * 40 + (16 if j % 2 else 0)
            if isinstance(g, int):
                return g * GD + off
            return pl.multiple_of(g * GD + off, 8)

        def body(t, carry):
            m2, m1, acc2 = carry
            zero = pl.multiple_of(jnp.minimum(t, 0), 256)
            tp = jnp.maximum(t - 1, 0)
            g = lax.shift_right_logical(t, sh)
            gn = lax.shift_right_logical(jnp.minimum(t + 1, NP - 1), sh)
            g_prev = lax.shift_right_logical(tp, sh)
            qs = [(t & (NQG - 1)) * QPI + k for k in range(QPI)]
            qs_prev = [(tp & (NQG - 1)) * QPI + k for k in range(QPI)]
            qls = [[q * NL + lt for lt in range(NL)] for q in qs]
            crows = [pl.ds(zero + c * CK, CK) for c in range(NC)]
            krows = [pl.ds(zero + c * 8, 8) for c in range(NC)]
            ms = {-2: list(m2), -1: list(m1)}
            accs = {-2: list(acc2)}
            for n in range(P * NC):
                i, c = n // NC, n % NC
                j, q = i // QPI, qs[i % QPI]
                s_ref = s_refs[i % NSB]
                if c == 0:
                    qms = [get_qm(4 * g + j, j, q, lt) for lt in range(NL)]
                    mx = [None] * NL
                kbs = [kbufs[j % 2][d:d + DG, krows[c], :] for d in range(0, DH, DG)]
                for lt in range(NL):
                    mx[lt] = qk_vpu(kbs, g, j, qls[i % QPI][lt], lt, c, s_ref, mx[lt])
                for lt in range(NL):
                    mx[lt] = qk(g, qms[lt], lt, pieces[lt][c], pieces[lt][c + 1], s_ref, mx[lt])
                nb = (i % QPI) * NC + c
                for d in range((nb * DH) // (QPI * NC), ((nb + 1) * DH) // (QPI * NC)):
                    build(g if j < 3 else gn, (j + 1) % 4, d, kbufs[(j + 1) % 2])
                n2 = n - LG
                i2, c2 = n2 // NC, n2 % NC
                j2 = (i2 % P) // QPI
                if c2 == 0 or n == 0:
                    base2 = vbase(g_prev if i2 < 0 else g, j2)
                q2 = (qs_prev if i2 < 0 else qs)[i2 % QPI]
                v = getv(base2, j2 % 2, c2)
                acc = accs.setdefault(i2, [None] * NL)
                for lt in range(NL):
                    acc[lt] = pv(v, lt, crows[c2], s_refs[i2 % NSB], ms[i2][lt], acc[lt])
                if c2 == NC - 1:
                    for lt in range(NL):
                        finish(base2, q2, lt, j2 % 2, acc[lt])
                if c == NC - 1:
                    for lt in range(NL):
                        mx[lt] = qk(g, qms[lt], lt, pieces[lt][NC], pieces[lt][NC + 1], s_ref, mx[lt])
                    ms[i] = [jnp.max(mx[lt], axis=0, keepdims=True) for lt in range(NL)]
            return tuple(ms[P - 2]), tuple(ms[P - 1]), tuple(accs[P - 2])

        zr = tuple(jnp.zeros((1, 128), F32) for _ in range(NL))
        ones24 = tuple(jnp.ones((24, 128), F32) for _ in range(NL))
        m2, m1, acc2 = lax.fori_loop(0, NP, body, (zr, zr, ones24))

        def epilogue():
            for (i2, m, acc, c0) in ((P - 2, m2, list(acc2), NC - LAG), (P - 1, m1, [None] * NL, 0)):
                j2 = i2 // QPI
                base2 = vbase(NG - 1, j2)
                q2 = NB - QPI + i2 % QPI
                for c2 in range(c0, NC):
                    v = getv(base2, j2 % 2, c2)
                    for lt in range(NL):
                        acc[lt] = pv(v, lt, pl.ds(c2 * CK, CK), s_refs[i2 % NSB], m[lt], acc[lt])
                    if c2 == NC - 1:
                        for lt in range(NL):
                            finish(base2, q2, lt, j2 % 2, acc[lt])
                    yield
        return epilogue()

    def out_copy(i, s):
        k = i * NS + s
        return pltpu.make_async_copy(obuf.at[k * SB:(k + 1) * SB, :],
                                     out_hbm.at[k * SB:(k + 1) * SB, :], osems.at[k])

    def stage_bout(r, epi):
        @pl.when(r == 1)
        def _():
            for i in range(NB):
                for s in range(NS):
                    out_copy(i, s).wait()

        def blk(i):
            for s in range(NS):
                ot = ot_ref[i, :, _lanes(s)]
                if s == 0 and i in (0, NB - 1):
                    yy = _dot(_up(wt[BO]), ot).T
                else:
                    yy = _dot(ot.T.astype(BF16), wsrc[BO])
                if i < NB - 1:
                    for _ in range(2):
                        next(epi, None)
                y = x_ref[srows(i, s), :] + yy
                x_ref[srows(i, s), :] = y
                x = xin[srows(i, s), :].astype(F32) + y
                obuf[srows(i, s), :] = x.astype(obuf.dtype)
                out_copy(i, s).start()
                if i == 0 and s == 0:
                    xn_ref[0] = _pk(_layernorm(x).astype(BF16))
        for i in range(NB - 1):
            blk(i)

        @pl.when(r >= 0)
        def _():
            blk(NB - 1)

    def round_(r, c):
        stage_a(r)
        a_mid()
        lax.fori_loop(0, NB, stage_l2, 0)
        stage_bout(r, attention())
        return c
    lax.fori_loop(0, 2, round_, 0)
    for i in range(NB):
        for s in range(NS):
            out_copy(i, s).wait()


@jax.jit
def pallas_interleave_layers__linear_attn_block__mha_block__prompt_kernel(
    A_x: jax.Array,
    A_wqkv: jax.Array,
    A_wo: jax.Array,
    B_x: jax.Array,
    B_wqkv: jax.Array,
    B_wo: jax.Array,
):
    del B_x
    x = A_x.reshape(S, D)
    scratch = [
        pltpu.VMEM((S, D), BF16),
        pltpu.VMEM((8, D, D), BF16),
        pltpu.VMEM((S, D), BF16),
        pltpu.SemaphoreType.DMA((NB + 8,)),
        pltpu.SemaphoreType.DMA((NB * NS,)),
        pltpu.VMEM((S, D), F32),
        pltpu.VMEM((2, SB // 2, D), U32),
        pltpu.VMEM((7, D // 2, D), U32),
        pltpu.VMEM((D // 2, D), U32),
        pltpu.VMEM((NB, D // 2, TB), U32),
        pltpu.VMEM((D, D), F32),
        pltpu.VMEM((D, 128), F32),
        pltpu.VMEM((D // 2, D), U32),
        pltpu.VMEM((NB, H, TB), F32),
        pltpu.VMEM((H, D), jnp.int32),
        pltpu.VMEM((5, 160, 128), jnp.int32),
        pltpu.VMEM((NG, S // 2, 128), U32),
        pltpu.VMEM((H, NB, 16, TB), U32),
        pltpu.VMEM((NB, D, TB), F32),
        pltpu.VMEM((NB, D, TB), F32),
        pltpu.VMEM((S // 128, NG, GD, 8, 128), F32),
        pltpu.VMEM((NG, KV, 128), F32),
        pltpu.VMEM((DH, KV, 128), F32),
        pltpu.VMEM((DH, KV, 128), F32),
    ] + [pltpu.VMEM((NL, S, 128), F32) for _ in range(NSB)]
    out = pl.pallas_call(
        _kernel,
        out_shape=jax.ShapeDtypeStruct((S, D), A_x.dtype),
        in_specs=[pl.BlockSpec(memory_space=pl.ANY)] * 5,
        out_specs=pl.BlockSpec(memory_space=pl.ANY),
        scratch_shapes=scratch,
        compiler_params=pltpu.CompilerParams(vmem_limit_bytes=124 * 1024 * 1024),
    )(x, A_wqkv, A_wo, B_wqkv, B_wo)
    return out.reshape(A_x.shape)
```
